```python
import jax
import jax.numpy as jnp

def _softmax(x, axis=-1):
    return jax.nn.softmax(x, axis=axis)

def _gelu(x):
    return jax.nn.gelu(x, approximate=True)

def _silu(x):
    return jax.nn.silu(x)

def _sigmoid(x):
    return jax.nn.sigmoid(x)

def _layernorm(x, axis=-1, eps=1e-05):
    m = jnp.mean(x, axis=axis, keepdims=True)
    v = jnp.var(x, axis=axis, keepdims=True)
    return (x - m) / jnp.sqrt(v + eps)

def _scatter_add(tgt, idx, src, axis=0):
    return tgt.at[idx].add(src)

def _segment_sum(src, seg, n):
    return jax.ops.segment_sum(src, seg, n)

class _Rng:

    def __init__(self, key):
        self._k = key

    def _next(self):
        self._k, sub = jax.random.split(self._k)
        return sub

    def normal(self, shape):
        return jax.random.normal(self._next(), shape, dtype=jnp.bfloat16)

    def randint(self, lo, hi, shape):
        return jax.random.randint(self._next(), shape, lo, hi, dtype=jnp.int32)

    def uniform(self, shape, lo=0.0, hi=1.0):
        return jax.random.uniform(self._next(), shape, jnp.bfloat16, lo, hi)

    def permutation(self, n):
        return jax.random.permutation(self._next(), n)
kernel_name = 'concat_heads__softmax_full_mha__memory_aug_recurrent_mem_tr__prompt'

def setup_inputs():
    _rng = _Rng(jax.random.key(int.from_bytes(__import__("os").urandom(4), "little")))
    _w = lambda a: (lambda t: t.astype(jnp.bfloat16) if jnp.issubdtype(t.dtype, jnp.floating) else t)(jnp.asarray(a))

    def _A_setup():
        B, S, D = (1, 2048, 1024)
        return {'x': _w((lambda *s: _rng.normal(s) * 0.05)(B, S, D)), 'wqkv': _w((lambda *s: _rng.normal(s) * 0.05)(D, 3 * D)), 'wo': _w((lambda *s: _rng.normal(s) * 0.05)(D, D))}
    _A_in = _A_setup()

    def _B_setup():
        B, S, Dm = (1, 2048, 1024)
        H, Dh = (32, 128)
        M, seg = (8, 32)
        seg = min(seg, S)
        S = S // seg * seg
        return {'x': _w((lambda *s: _rng.normal(s) * 0.05)(B, S, Dm)), 'mem0': _w((lambda *s: _rng.normal(s) * 0.05)(B, M, Dm)), 'Wq': _w((lambda *s: _rng.normal(s) * 0.05)(Dm, H, Dh) * Dm ** (-0.5)), 'Wk': _w((lambda *s: _rng.normal(s) * 0.05)(Dm, H, Dh) * Dm ** (-0.5)), 'Wv': _w((lambda *s: _rng.normal(s) * 0.05)(Dm, H, Dh) * Dm ** (-0.5)), 'Wo': _w((lambda *s: _rng.normal(s) * 0.05)(H, Dh, Dm) * (H * Dh) ** (-0.5)), 'seg_len': seg}
    _B_in = _B_setup()
    return {'A_x': _A_in['x'], 'A_wqkv': _A_in['wqkv'], 'A_wo': _A_in['wo'], 'B_x': _B_in['x'], 'B_mem0': _B_in['mem0'], 'B_Wq': _B_in['Wq'], 'B_Wk': _B_in['Wk'], 'B_Wv': _B_in['Wv'], 'B_Wo': _B_in['Wo'], 'B_seg_len': _B_in['seg_len']}

def reference(A_x, A_wqkv, A_wo, B_x, B_mem0, B_Wq, B_Wk, B_Wv, B_Wo, B_seg_len):

    def _A_ref(x, wqkv, wo):
        B, S, D = x.shape
        H = 32
        Dh = D // H
        qkv = (lambda x, *d: x.transpose(*d))((x @ wqkv).reshape(B, S, 3, H, Dh), 2, 0, 3, 1, 4)
        q, k, v = (qkv[0], qkv[1], qkv[2])
        scale = Dh ** (-0.5)
        scores = jnp.einsum('bhqd,bhkd->bhqk', q, k) * scale
        p = _softmax(scores, axis=-1)
        o = jnp.einsum('bhqk,bhkd->bhqd', p, v)
        return (lambda x, *d: x.transpose(*d))(o, 0, 2, 1, 3).reshape(B, S, D) @ wo

    def _B_ref(x, mem0, Wq, Wk, Wv, Wo, seg_len):
        B, S, Dm = x.shape
        H, Dh = (Wq.shape[1], Wq.shape[2])
        M = mem0.shape[1]
        scale = Dh ** (-0.5)
        n_seg = S // seg_len
        L = M + seg_len
        idx = jnp.arange(L)
        mask = (idx[:, None] < M) | (idx[:, None] >= idx[None, :])
        mem = mem0
        outs = []
        for s in range(n_seg):
            xs = x[:, s * seg_len:(s + 1) * seg_len, :].copy()
            h = jnp.concatenate([mem, xs], axis=1)
            q = jnp.einsum('btd,dhe->bhte', h, Wq)
            k = jnp.einsum('btd,dhe->bhte', h, Wk)
            v = jnp.einsum('btd,dhe->bhte', h, Wv)
            scores = jnp.einsum('bhqe,bhke->bhqk', q, k) * scale
            scores = jnp.where(mask[None, None], scores, -1000000000.0)
            p = _softmax(scores, axis=-1)
            o = jnp.einsum('bhqk,bhke->bhqe', p, v)
            o = jnp.einsum('bhte,hed->btd', o, Wo)
            mem = o[:, :M, :].copy()
            outs.append(o[:, M:, :])
        return jnp.concatenate(outs, axis=1)
    a = _A_ref(A_x, A_wqkv, A_wo)
    b = _B_ref(B_x, B_mem0, B_Wq, B_Wk, B_Wv, B_Wo, B_seg_len)
    return jnp.concatenate([a, b], axis=-1)
```

```python
import functools

import jax
import jax.numpy as jnp
from jax import lax
import jax.experimental.pallas as pl
import jax.experimental.pallas.tpu as pltpu

bf16 = jnp.bfloat16
f32 = jnp.float32
u32 = jnp.uint32

S = 2048
D = 1024
HA = 32
DHA = 32
HB = 32
DHB = 128
MEM = 8
SEG = 32
LOG2E = 1.4426950408889634
LAG = 8


def _dot(a, b):
    return jnp.dot(a, b, preferred_element_type=f32)


def _dot_t(a, b):
    return lax.dot_general(a, b, (((1,), (1,)), ((), ())), preferred_element_type=f32)


def _bc(x):
    return pltpu.bitcast(x, bf16)


def _kernel(ax_hbm, awqkv_hbm, awo_hbm, bx_hbm, bmem_hbm, bwq_hbm, bwk_hbm, bwv_hbm, bwo_hbm,
            out_hbm,
            xa, wqkv, awo, wT, kbuf, qT, vT, sa, sb, obuf, outa,
            xb, mem0, raw, wq, wk, wv, wo, outb, cq, ck, cv, co,
            sem_a, sem_b, sem_raw, sem_wo, sem_out):
    cp_x = pltpu.make_async_copy(ax_hbm, xa, sem_a.at[0])
    cp_w = pltpu.make_async_copy(awqkv_hbm, wqkv, sem_a.at[1])
    cp_x.start()
    cp_w.start()
    cp_x.wait()
    cp_w.wait()

    cp_awo = pltpu.make_async_copy(awo_hbm, awo, sem_a.at[2])
    cp_awo.start()
    cp_raw = []
    for i, w_hbm in enumerate((bwq_hbm, bwk_hbm, bwv_hbm)):
        w32 = w_hbm.bitcast(u32)
        for hp in range(HB // 2):
            cp = pltpu.make_async_copy(w32.at[:, hp, :], raw.at[i, hp], sem_raw.at[i * 16 + hp])
            cp.start()
            cp_raw.append(cp)
    cp_wo = []
    for n in range(D // 128):
        cp = pltpu.make_async_copy(bwo_hbm.at[:, pl.ds(n * 128, 128)], wo.at[n], sem_wo.at[n])
        cp.start()
        cp_wo.append(cp)
    cp_xb = pltpu.make_async_copy(bx_hbm, xb, sem_b.at[0])
    cp_mem = pltpu.make_async_copy(bmem_hbm, mem0, sem_b.at[1])
    cp_xb.start()
    cp_mem.start()

    RC = 256

    def kproj(c, carry):
        r0 = pl.multiple_of(c * RC, RC)
        x = xa[pl.ds(r0, RC), :]
        for g in range(8):
            w = wqkv[:, D + g * 128:D + (g + 1) * 128]
            kbuf[g, pl.ds(r0, RC), :] = _dot(x, w).astype(bf16)
        return carry

    lax.fori_loop(0, S // RC, kproj, 0)

    def wtrans(kt, carry):
        r0 = pl.multiple_of(kt * 128, 128)
        for i, c0 in enumerate((0, 2 * D)):
            for n in range(8):
                t = wqkv[pl.ds(r0, 128), c0 + n * 128:c0 + (n + 1) * 128]
                wT[kt, i * D + n * 128:i * D + (n + 1) * 128, :] = t.T
        return carry

    lax.fori_loop(0, 8, wtrans, 0)

    wT32 = wT.bitcast(u32)
    qscale = (DHA ** -0.5) * LOG2E

    def qvproj(j, carry):
        t0 = pl.multiple_of(j * 128, 128)
        xs = [xa[pl.ds(t0, 128), kt * 128:(kt + 1) * 128] for kt in range(8)]
        for c in range(2 * D // RC):
            acc = None
            for kt in range(8):
                lhs = _bc(wT32[kt, c * RC // 2:(c + 1) * RC // 2, :])
                r = _dot_t(lhs, xs[kt])
                acc = r if acc is None else acc + r
            if c * RC < D:
                for gg in range(RC // 128):
                    qT[(c * RC) // 128 + gg, j] = (acc[gg * 128:(gg + 1) * 128] * qscale).astype(bf16)
            else:
                h0 = (c * RC - D) // DHA
                for hh in range(RC // DHA):
                    vT[h0 + hh, j] = acc[hh * DHA:(hh + 1) * DHA].astype(bf16)
        return carry

    lax.fori_loop(0, S // 128, qvproj, 0)

    k32 = kbuf.bitcast(u32)
    q32 = qT.bitcast(u32)
    v32 = vT.bitcast(u32)
    NK = S // 128

    def q_tile(g, j, hh):
        q = _bc(q32[g, j, hh * 16:(hh + 1) * 16, :])
        parts = []
        if hh > 0:
            parts.append(jnp.zeros((hh * DHA, 128), bf16))
        parts.append(q)
        if hh < 3:
            parts.append(jnp.zeros(((3 - hh) * DHA, 128), bf16))
        return jnp.concatenate(parts, axis=0) if len(parts) > 1 else q

    def qk_tile(g, qm, c, s_w):
        k = _bc(k32[g, c * 64:(c + 1) * 64, :])
        s = _dot(k, qm)
        s_w[c * 128:(c + 1) * 128, :] = s
        return jnp.max(s.reshape(16, 8, 128), axis=0)

    def half(g, j, hh, gn, qn, s_w, s_r, m, zero):
        h = g * 4 + hh
        m8 = l = acc = None
        for c in range(NK + LAG):
            if c < NK:
                mt = qk_tile(gn, qn, c, s_w)
                m8 = mt if m8 is None else jnp.maximum(m8, mt)
            if c >= LAG:
                t = c - LAG
                if zero is None:
                    s = s_r[t * 128:(t + 1) * 128, :]
                else:
                    s = s_r[pl.ds(pl.multiple_of(zero + t * 128, 128), 128), :]
                p = jnp.exp2(s - m)
                lt = jnp.sum(p.reshape(16, 8, 128), axis=0)
                l = lt if l is None else l + lt
                pv = _dot(_bc(v32[h, t]), p.astype(bf16))
                acc = pv if acc is None else acc + pv
        o = acc * (1.0 / jnp.sum(l, axis=0, keepdims=True))
        return o, jnp.max(m8, axis=0, keepdims=True)

    q0 = q_tile(0, 0, 0)
    m8 = None
    for c in range(NK):
        mt = qk_tile(0, q0, c, sa)
        m8 = mt if m8 is None else jnp.maximum(m8, mt)
    m_first = jnp.max(m8, axis=0, keepdims=True)

    NIT = 64

    def a2_body(it, m):
        g = it // 8
        jj = it % 8
        zero = (it * (it + 1)) & 1
        outs = []
        for r in range(8):
            j = 2 * jj + r // 4
            hh = r % 4
            s_r, s_w = (sa, sb) if r % 2 == 0 else (sb, sa)
            if r < 7:
                gn = g
                qn = q_tile(g, 2 * jj + (r + 1) // 4, (r + 1) % 4)
            else:
                itn = jnp.minimum(it + 1, NIT - 1)
                gn = itn // 8
                qn = q_tile(gn, 2 * (itn % 8), 0)
            o, m = half(g, j, hh, gn, qn, s_w, s_r, m, None if r == 0 else zero)
            outs.append(o)
            if hh == 3:
                ot = jnp.concatenate(outs, axis=0)
                outs = []
                obuf[g, pl.ds(pl.multiple_of(j * 128, 128), 128), :] = ot.T.astype(bf16)
        return m

    lax.fori_loop(0, NIT, a2_body, m_first)

    cp_awo.wait()

    def oproj(c, carry):
        r0 = pl.multiple_of(c * RC, RC)
        o = jnp.concatenate([obuf[g, pl.ds(r0, RC), :] for g in range(8)], axis=1)
        outa[pl.ds(r0, RC), :] = _dot(o, awo[...]).astype(bf16)
        return carry

    lax.fori_loop(0, S // RC, oproj, 0)
    cp_outa = pltpu.make_async_copy(outa, out_hbm.at[:, pl.ds(0, D)], sem_out.at[0])
    cp_outa.start()

    for cp in cp_raw:
        cp.wait()

    def repack(i, carry):
        for wi, dst in enumerate((wq, wk, wv)):
            for hp in range(HB // 2):
                for jb in range(2):
                    base = pl.multiple_of(i * 32, 32) + jb * 16
                    ve = raw[wi, hp, pl.ds(base, 8, stride=2), :]
                    vo = raw[wi, hp, pl.ds(base + 1, 8, stride=2), :]
                    lo = (ve & jnp.uint32(0xFFFF)) | (vo << 16)
                    hi = (ve >> 16) | (vo & jnp.uint32(0xFFFF0000))
                    r = pl.ds(pl.multiple_of(i * 16, 16) + jb * 8, 8)
                    dst[2 * hp, r, :] = lo
                    dst[2 * hp + 1, r, :] = hi
        return carry

    lax.fori_loop(0, D // 32, repack, 0)

    for cp in cp_wo:
        cp.wait()
    cp_xb.wait()
    cp_mem.wait()
    wo32 = wo.bitcast(u32)
    bscale = DHB ** -0.5
    row = lax.broadcasted_iota(jnp.int32, (48, 48), 0)
    col = lax.broadcasted_iota(jnp.int32, (48, 48), 1)
    mask = (col < MEM + SEG) & ((row < MEM) | (row >= col))
    LQ, LP = 1, 3

    def qk_soft(q, k):
        s = _dot_t(q, k)
        s = jnp.where(mask, s * bscale, -1e9)
        m = jnp.max(s, axis=-1, keepdims=True)
        p = jnp.exp(s - m)
        l = jnp.sum(p, axis=-1, keepdims=True)
        return (p / l).astype(bf16)

    def step(hmat, assemble, finish_o):
        qs, ks, vs, ps, o_list = {}, {}, {}, {}, [None] * HB
        accs = [None] * 8

        def do_proj(h):
            qs[h] = assemble(cq, h, _dot(hmat, _bc(wq[h])))
            ks[h] = assemble(ck, h, _dot(hmat, _bc(wk[h])))
            vs[h] = assemble(cv, h, _dot(hmat, _bc(wv[h])))

        def do_wo(g):
            og = jnp.concatenate(o_list[4 * g:4 * g + 4], axis=1)
            for n in range(8):
                r = _dot(og, _bc(wo32[n, g * 256:(g + 1) * 256, :]))
                accs[n] = r if accs[n] is None else accs[n] + r

        g_next = 0
        for i in range(HB + LP):
            if i < HB:
                do_proj(i)
            else:
                do_wo(g_next)
                g_next += 1
            if 0 <= i - LQ < HB:
                ps[i - LQ] = qk_soft(qs.pop(i - LQ), ks.pop(i - LQ))
            if 0 <= i - LP < HB:
                h = i - LP
                o_list[h] = finish_o(h, _dot(ps.pop(h), vs.pop(h)))
        while g_next < 8:
            do_wo(g_next)
            g_next += 1
        return jnp.concatenate(accs, axis=1)

    def dstep(d, mem):
        base = pl.multiple_of(d * 64, 64)
        ha = jnp.concatenate([mem, xb[pl.ds(base, 40), :].astype(f32)], axis=0).astype(bf16)

        def asm_a(cref, h, v):
            cref[h] = v[40:48]
            return v.astype(bf16)

        def fin_a(h, o):
            co[h] = o[32:40]
            return o[0:32].astype(bf16)

        y = step(ha, asm_a, fin_a).astype(bf16)
        outb[pl.ds(base, 24), :] = y[8:32]
        mem1 = y[0:8].astype(f32)
        hb = jnp.concatenate([mem1, xb[pl.ds(base + 40, 24), :].astype(f32)], axis=0).astype(bf16)
        z8 = jnp.zeros((8, DHB), f32)

        def asm_b(cref, h, v):
            return jnp.concatenate([v[0:8], cref[h], v[8:32], z8], axis=0).astype(bf16)

        def fin_b(h, o):
            return jnp.concatenate([o[0:8], co[h], o[8:40]], axis=0).astype(bf16)

        y = step(hb, asm_b, fin_b).astype(bf16)
        outb[pl.ds(base + 24, 40), :] = y[8:48]
        return y[0:8].astype(f32)

    lax.fori_loop(0, S // (2 * SEG), dstep, mem0[...].astype(f32))

    cp_outb = pltpu.make_async_copy(outb, out_hbm.at[:, pl.ds(D, D)], sem_out.at[1])
    cp_outb.start()
    cp_outa.wait()
    cp_outb.wait()


@functools.partial(jax.jit, static_argnames=("B_seg_len",))
def pallas_concat_heads__softmax_full_mha__memory_aug_recurrent_mem_tr__prompt_kernel(
    A_x: jax.Array,
    A_wqkv: jax.Array,
    A_wo: jax.Array,
    B_x: jax.Array,
    B_mem0: jax.Array,
    B_Wq: jax.Array,
    B_Wk: jax.Array,
    B_Wv: jax.Array,
    B_Wo: jax.Array,
    B_seg_len: int,
):
    assert A_x.shape == (1, S, D) and B_x.shape == (1, S, D) and B_mem0.shape == (1, MEM, D)
    assert B_Wq.shape == (D, HB, DHB) and B_Wo.shape == (HB, DHB, D) and B_seg_len == SEG
    any_spec = pl.BlockSpec(memory_space=pl.ANY)
    scratch = [
        pltpu.VMEM((S, D), bf16),
        pltpu.VMEM((D, 3 * D), bf16),
        pltpu.VMEM((D, D), bf16),
        pltpu.VMEM((8, 2 * D, 128), bf16),
        pltpu.VMEM((8, S, 128), bf16),
        pltpu.VMEM((8, 16, 128, 128), bf16),
        pltpu.VMEM((HA, 16, DHA, 128), bf16),
        pltpu.VMEM((S, 128), f32),
        pltpu.VMEM((S, 128), f32),
        pltpu.VMEM((8, S, 128), bf16),
        pltpu.VMEM((S, D), bf16),
        pltpu.VMEM((S, D), bf16),
        pltpu.VMEM((MEM, D), bf16),
        pltpu.VMEM((3, HB // 2, D, 128), u32),
        pltpu.VMEM((HB, D // 2, 128), u32),
        pltpu.VMEM((HB, D // 2, 128), u32),
        pltpu.VMEM((HB, D // 2, 128), u32),
        pltpu.VMEM((8, HB * DHB, 128), bf16),
        pltpu.VMEM((S, D), bf16),
        pltpu.VMEM((HB, 8, 128), f32),
        pltpu.VMEM((HB, 8, 128), f32),
        pltpu.VMEM((HB, 8, 128), f32),
        pltpu.VMEM((HB, 8, 128), f32),
        pltpu.SemaphoreType.DMA((3,)),
        pltpu.SemaphoreType.DMA((2,)),
        pltpu.SemaphoreType.DMA((48,)),
        pltpu.SemaphoreType.DMA((8,)),
        pltpu.SemaphoreType.DMA((2,)),
    ]
    out = pl.pallas_call(
        _kernel,
        out_shape=jax.ShapeDtypeStruct((S, 2 * D), bf16),
        in_specs=[any_spec] * 9,
        out_specs=any_spec,
        scratch_shapes=scratch,
        compiler_params=pltpu.CompilerParams(vmem_limit_bytes=124 * 1024 * 1024),
        name="mha_rmt_fused",
    )(A_x.reshape(S, D), A_wqkv, A_wo, B_x.reshape(S, D), B_mem0.reshape(MEM, D),
      B_Wq, B_Wk, B_Wv, B_Wo.reshape(HB * DHB, D))
    return out.reshape(1, S, 2 * D)
```

```python
import functools

import jax
import jax.numpy as jnp
from jax import lax
import jax.experimental.pallas as pl
import jax.experimental.pallas.tpu as pltpu

bf16 = jnp.bfloat16
f32 = jnp.float32
u32 = jnp.uint32

S = 2048
D = 1024
HA = 32
DHA = 32
HB = 32
DHB = 128
MEM = 8
SEG = 32
LOG2E = 1.4426950408889634
A2_JU = 8
PROJ_U = 2
HIDE_REPACK = True
LAG = 8


def _dot(a, b):
    return jnp.dot(a, b, preferred_element_type=f32)


def _dot_t(a, b):
    return lax.dot_general(a, b, (((1,), (1,)), ((), ())), preferred_element_type=f32)


def _bc(x):
    return pltpu.bitcast(x, bf16)


def _kernel(ax_hbm, awqkv_hbm, awo_hbm, bx_hbm, bmem_hbm, bwq_hbm, bwk_hbm, bwv_hbm, bwo_hbm,
            out_hbm,
            xa, wqkv, awo, kbuf, qT, vT, sa, sb, obuf, outa,
            xb, mem0, raw, wq, wk, wv, wo, outb, cq, ck, cv, co,
            sem_a, sem_x, sem_b, sem_raw, sem_wo, sem_out, sem_ob):
    RC = 256
    NXC = S // RC
    cp_wk = pltpu.make_async_copy(awqkv_hbm.at[:, pl.ds(D, D)], wqkv.at[:, pl.ds(D, D)], sem_a.at[0])
    cp_x = [pltpu.make_async_copy(ax_hbm.at[pl.ds(c * RC, RC), :], xa.at[pl.ds(c * RC, RC), :], sem_x.at[c])
            for c in range(NXC)]
    cp_wq = pltpu.make_async_copy(awqkv_hbm.at[:, pl.ds(0, D)], wqkv.at[:, pl.ds(0, D)], sem_a.at[1])
    cp_wv = pltpu.make_async_copy(awqkv_hbm.at[:, pl.ds(2 * D, D)], wqkv.at[:, pl.ds(2 * D, D)], sem_a.at[3])
    cp_x[0].start()
    cp_wk.start()
    for c in range(1, NXC):
        cp_x[c].start()
    cp_wq.start()
    cp_wv.start()
    cp_wk.wait()

    cp_awo = pltpu.make_async_copy(awo_hbm, awo, sem_a.at[2])
    cp_awo.start()
    cp_raw = []
    for i, w_hbm in enumerate((bwq_hbm, bwk_hbm, bwv_hbm)):
        w32 = w_hbm.bitcast(u32)
        for hp in range(HB // 2):
            cp = pltpu.make_async_copy(w32.at[:, hp, :], raw.at[i, hp], sem_raw.at[i * 16 + hp])
            cp.start()
            cp_raw.append(cp)
    cp_wo = []
    for n in range(D // 128):
        cp = pltpu.make_async_copy(bwo_hbm.at[:, pl.ds(n * 128, 128)], wo.at[n], sem_wo.at[n])
        cp.start()
        cp_wo.append(cp)
    cp_xb = pltpu.make_async_copy(bx_hbm, xb, sem_b.at[0])
    cp_mem = pltpu.make_async_copy(bmem_hbm, mem0, sem_b.at[1])
    cp_xb.start()
    cp_mem.start()

    qscale = (DHA ** -0.5) * LOG2E

    def kproj(i, carry):
        for cc in range(PROJ_U):
            c = i * PROJ_U + cc
            r0 = pl.multiple_of(c * RC, RC)
            pltpu.make_async_copy(ax_hbm.at[pl.ds(r0, RC), :], xa.at[pl.ds(r0, RC), :], sem_x.at[c]).wait()
        for cc in range(PROJ_U):
            r0 = pl.multiple_of((i * PROJ_U + cc) * RC, RC)
            x = xa[pl.ds(r0, RC), :]
            for g in range(8):
                w = wqkv[:, D + g * 128:D + (g + 1) * 128]
                kbuf[g, pl.ds(r0, RC), :] = _dot(x, w).astype(bf16)
        return carry

    lax.fori_loop(0, NXC // PROJ_U, kproj, 0)
    cp_wq.wait()
    cp_wv.wait()

    def qvproj(c, carry):
        r0 = pl.multiple_of(c * RC, RC)
        x = xa[pl.ds(r0, RC), :]
        for g in range(8):
            q = _dot(x, wqkv[:, g * 128:(g + 1) * 128]) * qscale
            v = _dot(x, wqkv[:, 2 * D + g * 128:2 * D + (g + 1) * 128])
            for jj in range(RC // 128):
                j = c * (RC // 128) + jj
                qT[g, j] = q[jj * 128:(jj + 1) * 128].T.astype(bf16)
                vt = v[jj * 128:(jj + 1) * 128].T.astype(bf16)
                for hh in range(4):
                    vT[g * 4 + hh, j] = vt[hh * DHA:(hh + 1) * DHA]
        return carry

    lax.fori_loop(0, NXC, qvproj, 0)

    k32 = kbuf.bitcast(u32)
    q32 = qT.bitcast(u32)
    v32 = vT.bitcast(u32)
    NK = S // 128

    def q_tile(g, j, hh):
        q = _bc(q32[g, j, hh * 16:(hh + 1) * 16, :])
        parts = []
        if hh > 0:
            parts.append(jnp.zeros((hh * DHA, 128), bf16))
        parts.append(q)
        if hh < 3:
            parts.append(jnp.zeros(((3 - hh) * DHA, 128), bf16))
        return jnp.concatenate(parts, axis=0) if len(parts) > 1 else q

    def qk_tile(g, qm, c, s_w):
        k = _bc(k32[g, c * 64:(c + 1) * 64, :])
        s = _dot(k, qm)
        s_w[c * 128:(c + 1) * 128, :] = s
        return jnp.max(s.reshape(16, 8, 128), axis=0)

    def half(g, j, hh, gn, qn, s_w, s_r, m, zero):
        h = g * 4 + hh
        m8 = l = acc = None
        for c in range(NK + LAG):
            if c < NK:
                mt = qk_tile(gn, qn, c, s_w)
                m8 = mt if m8 is None else jnp.maximum(m8, mt)
            if c >= LAG:
                t = c - LAG
                if zero is None:
                    s = s_r[t * 128:(t + 1) * 128, :]
                else:
                    s = s_r[pl.ds(pl.multiple_of(zero + t * 128, 128), 128), :]
                p = jnp.exp2(s - m)
                lt = jnp.sum(p.reshape(16, 8, 128), axis=0)
                l = lt if l is None else l + lt
                pv = _dot(_bc(v32[h, t]), p.astype(bf16))
                acc = pv if acc is None else acc + pv
        o = acc * (1.0 / jnp.sum(l, axis=0, keepdims=True))
        return o, jnp.max(m8, axis=0, keepdims=True)

    q0 = q_tile(0, 0, 0)
    m8 = None
    for c in range(NK):
        mt = qk_tile(0, q0, c, sa)
        m8 = mt if m8 is None else jnp.maximum(m8, mt)
    m_first = jnp.max(m8, axis=0, keepdims=True)

    for cp in cp_raw:
        cp.wait()

    def repack(i, nblk):
        for wi, dst in enumerate((wq, wk, wv)):
            for hp in range(HB // 2):
                for jb in range(nblk):
                    base = pl.multiple_of(i * (16 * nblk), 16 * nblk) + jb * 16
                    ve = raw[wi, hp, pl.ds(base, 8, stride=2), :]
                    vo = raw[wi, hp, pl.ds(base + 1, 8, stride=2), :]
                    lo = (ve & jnp.uint32(0xFFFF)) | (vo << 16)
                    hi = (ve >> 16) | (vo & jnp.uint32(0xFFFF0000))
                    r = pl.ds(pl.multiple_of(i * (8 * nblk), 8 * nblk) + jb * 8, 8)
                    dst[2 * hp, r, :] = lo
                    dst[2 * hp + 1, r, :] = hi

    JU = A2_JU
    NJ = 16 // JU
    NIT = 8 * NJ
    NR = 4 * JU

    def a2_body(it, m):
        g = it // NJ
        jj = it % NJ
        zero = (it * (it + 1)) & 1
        outs = []
        for r in range(NR):
            j = JU * jj + r // 4
            hh = r % 4
            s_r, s_w = (sa, sb) if r % 2 == 0 else (sb, sa)
            if r < NR - 1:
                gn = g
                qn = q_tile(g, JU * jj + (r + 1) // 4, (r + 1) % 4)
            else:
                itn = jnp.minimum(it + 1, NIT - 1)
                gn = itn // NJ
                qn = q_tile(gn, JU * (itn % NJ), 0)
            o, m = half(g, j, hh, gn, qn, s_w, s_r, m, None if r == 0 else zero)
            outs.append(o)
            if hh == 3:
                ot = jnp.concatenate(outs, axis=0)
                outs = []
                obuf[g, pl.ds(pl.multiple_of(j * 128, 128), 128), :] = ot.T.astype(bf16)
        if HIDE_REPACK:
            repack(it, D // 16 // NIT)
        return m

    lax.fori_loop(0, NIT, a2_body, m_first)

    cp_awo.wait()

    def oproj(i, carry):
        for cc in range(PROJ_U):
            r0 = pl.multiple_of((i * PROJ_U + cc) * RC, RC)
            o = jnp.concatenate([obuf[g, pl.ds(r0, RC), :] for g in range(8)], axis=1)
            outa[pl.ds(r0, RC), :] = _dot(o, awo[...]).astype(bf16)
        return carry

    lax.fori_loop(0, NXC // PROJ_U, oproj, 0)
    cp_outa = pltpu.make_async_copy(outa, out_hbm.at[:, pl.ds(0, D)], sem_out.at[0])
    cp_outa.start()

    if not HIDE_REPACK:
        lax.fori_loop(0, D // 32, lambda i, c: (repack(i, 2), c)[1], 0)

    for cp in cp_wo:
        cp.wait()
    cp_xb.wait()
    cp_mem.wait()
    wo32 = wo.bitcast(u32)
    bscale = DHB ** -0.5
    row = lax.broadcasted_iota(jnp.int32, (48, 48), 0)
    col = lax.broadcasted_iota(jnp.int32, (48, 48), 1)
    mask = (col < MEM + SEG) & ((row < MEM) | (row >= col))
    LQ, LP = 1, 3

    def qk_soft(q, k):
        s = _dot_t(q, k)
        s = jnp.where(mask, s * bscale, -1e9)
        m = jnp.max(s, axis=-1, keepdims=True)
        p = jnp.exp(s - m)
        l = jnp.sum(p, axis=-1, keepdims=True)
        return (p / l).astype(bf16)

    def step(hmat, assemble, finish_o):
        qs, ks, vs, ps, o_list = {}, {}, {}, {}, [None] * HB
        accs = [None] * 8

        def do_proj(h):
            qs[h] = assemble(cq, h, _dot(hmat, _bc(wq[h])))
            ks[h] = assemble(ck, h, _dot(hmat, _bc(wk[h])))
            vs[h] = assemble(cv, h, _dot(hmat, _bc(wv[h])))

        def do_wo(g):
            og = jnp.concatenate(o_list[4 * g:4 * g + 4], axis=1)
            for n in range(8):
                r = _dot(og, _bc(wo32[n, g * 256:(g + 1) * 256, :]))
                accs[n] = r if accs[n] is None else accs[n] + r

        g_next = 0
        for i in range(HB + LP):
            if i < HB:
                do_proj(i)
            else:
                do_wo(g_next)
                g_next += 1
            if 0 <= i - LQ < HB:
                ps[i - LQ] = qk_soft(qs.pop(i - LQ), ks.pop(i - LQ))
            if 0 <= i - LP < HB:
                h = i - LP
                o_list[h] = finish_o(h, _dot(ps.pop(h), vs.pop(h)))
        while g_next < 8:
            do_wo(g_next)
            g_next += 1
        return jnp.concatenate(accs, axis=1)

    def dstep(d, mem):
        base = pl.multiple_of(d * 64, 64)
        ha = jnp.concatenate([mem, xb[pl.ds(base, 40), :].astype(f32)], axis=0).astype(bf16)

        def asm_a(cref, h, v):
            cref[h] = v[40:48]
            return v.astype(bf16)

        def fin_a(h, o):
            co[h] = o[32:40]
            return o[0:32].astype(bf16)

        y = step(ha, asm_a, fin_a).astype(bf16)
        outb[pl.ds(base, 24), :] = y[8:32]
        mem1 = y[0:8].astype(f32)
        hb = jnp.concatenate([mem1, xb[pl.ds(base + 40, 24), :].astype(f32)], axis=0).astype(bf16)
        z8 = jnp.zeros((8, DHB), f32)

        def asm_b(cref, h, v):
            return jnp.concatenate([v[0:8], cref[h], v[8:32], z8], axis=0).astype(bf16)

        def fin_b(h, o):
            return jnp.concatenate([o[0:8], co[h], o[8:40]], axis=0).astype(bf16)

        y = step(hb, asm_b, fin_b).astype(bf16)
        outb[pl.ds(base + 24, 40), :] = y[8:48]
        rows = pl.ds(base, 64)
        pltpu.make_async_copy(outb.at[rows, :], out_hbm.at[rows, pl.ds(D, D)], sem_ob.at[d]).start()
        return y[0:8].astype(f32)

    lax.fori_loop(0, S // (2 * SEG), dstep, mem0[...].astype(f32))

    cp_outa.wait()

    def wait_out(d, carry):
        rows = pl.ds(pl.multiple_of(d * 64, 64), 64)
        pltpu.make_async_copy(outb.at[rows, :], out_hbm.at[rows, pl.ds(D, D)], sem_ob.at[d]).wait()
        return carry

    lax.fori_loop(0, S // (2 * SEG), wait_out, 0)


@functools.partial(jax.jit, static_argnames=("B_seg_len",))
def pallas_concat_heads__softmax_full_mha__memory_aug_recurrent_mem_tr__prompt_kernel(
    A_x: jax.Array,
    A_wqkv: jax.Array,
    A_wo: jax.Array,
    B_x: jax.Array,
    B_mem0: jax.Array,
    B_Wq: jax.Array,
    B_Wk: jax.Array,
    B_Wv: jax.Array,
    B_Wo: jax.Array,
    B_seg_len: int,
):
    assert A_x.shape == (1, S, D) and B_x.shape == (1, S, D) and B_mem0.shape == (1, MEM, D)
    assert B_Wq.shape == (D, HB, DHB) and B_Wo.shape == (HB, DHB, D) and B_seg_len == SEG
    any_spec = pl.BlockSpec(memory_space=pl.ANY)
    scratch = [
        pltpu.VMEM((S, D), bf16),
        pltpu.VMEM((D, 3 * D), bf16),
        pltpu.VMEM((D, D), bf16),
        pltpu.VMEM((8, S, 128), bf16),
        pltpu.VMEM((8, 16, 128, 128), bf16),
        pltpu.VMEM((HA, 16, DHA, 128), bf16),
        pltpu.VMEM((S, 128), f32),
        pltpu.VMEM((S, 128), f32),
        pltpu.VMEM((8, S, 128), bf16),
        pltpu.VMEM((S, D), bf16),
        pltpu.VMEM((S, D), bf16),
        pltpu.VMEM((MEM, D), bf16),
        pltpu.VMEM((3, HB // 2, D, 128), u32),
        pltpu.VMEM((HB, D // 2, 128), u32),
        pltpu.VMEM((HB, D // 2, 128), u32),
        pltpu.VMEM((HB, D // 2, 128), u32),
        pltpu.VMEM((8, HB * DHB, 128), bf16),
        pltpu.VMEM((S, D), bf16),
        pltpu.VMEM((HB, 8, 128), f32),
        pltpu.VMEM((HB, 8, 128), f32),
        pltpu.VMEM((HB, 8, 128), f32),
        pltpu.VMEM((HB, 8, 128), f32),
        pltpu.SemaphoreType.DMA((4,)),
        pltpu.SemaphoreType.DMA((8,)),
        pltpu.SemaphoreType.DMA((2,)),
        pltpu.SemaphoreType.DMA((48,)),
        pltpu.SemaphoreType.DMA((8,)),
        pltpu.SemaphoreType.DMA((1,)),
        pltpu.SemaphoreType.DMA((32,)),
    ]
    out = pl.pallas_call(
        _kernel,
        out_shape=jax.ShapeDtypeStruct((S, 2 * D), bf16),
        in_specs=[any_spec] * 9,
        out_specs=any_spec,
        scratch_shapes=scratch,
        compiler_params=pltpu.CompilerParams(vmem_limit_bytes=124 * 1024 * 1024),
        name="mha_rmt_fused",
    )(A_x.reshape(S, D), A_wqkv, A_wo, B_x.reshape(S, D), B_mem0.reshape(MEM, D),
      B_Wq, B_Wk, B_Wv, B_Wo.reshape(HB * DHB, D))
    return out.reshape(1, S, 2 * D)
```

```python
import functools

import jax
import jax.numpy as jnp
from jax import lax
import jax.experimental.pallas as pl
import jax.experimental.pallas.tpu as pltpu

bf16 = jnp.bfloat16
f32 = jnp.float32
u32 = jnp.uint32

S = 2048
D = 1024
HA = 32
DHA = 32
HB = 32
DHB = 128
MEM = 8
SEG = 32
LOG2E = 1.4426950408889634
A2_JU = 8
KP_U = 2
QV_U = 4
PROJ_U = 2
B_LQ = 3
B_LP = 6
LAG = 8


def _dot(a, b):
    return jnp.dot(a, b, preferred_element_type=f32)


def _dot_t(a, b):
    return lax.dot_general(a, b, (((1,), (1,)), ((), ())), preferred_element_type=f32)


def _bc(x):
    return pltpu.bitcast(x, bf16)


def _kernel(ax_hbm, awqkv_hbm, awo_hbm, bx_hbm, bmem_hbm, bwq_hbm, bwk_hbm, bwv_hbm, bwo_hbm,
            out_hbm,
            xa, wqkv, awo, kbuf, qT, vT, sa, sb, obuf, outa,
            xb, mem0, raw, wq, wk, wv, wo, outb, cq, ck, cv, co,
            sem_a, sem_x, sem_b, sem_raw, sem_wo, sem_out, sem_ob):
    RC = 256
    NXC = S // RC
    cp_wk = pltpu.make_async_copy(awqkv_hbm.at[:, pl.ds(D, D)], wqkv.at[:, pl.ds(D, D)], sem_a.at[0])
    cp_x = [pltpu.make_async_copy(ax_hbm.at[pl.ds(c * RC, RC), :], xa.at[pl.ds(c * RC, RC), :], sem_x.at[c])
            for c in range(NXC)]
    cp_wq = pltpu.make_async_copy(awqkv_hbm.at[:, pl.ds(0, D)], wqkv.at[:, pl.ds(0, D)], sem_a.at[1])
    cp_wv = pltpu.make_async_copy(awqkv_hbm.at[:, pl.ds(2 * D, D)], wqkv.at[:, pl.ds(2 * D, D)], sem_a.at[3])
    cp_wk.start()
    for c in range(KP_U):
        cp_x[c].start()
    cp_wk.wait()
    for c in range(KP_U, NXC):
        cp_x[c].start()
    cp_wq.start()
    cp_wv.start()


    qscale = (DHA ** -0.5) * LOG2E

    def kproj(i, carry):
        for cc in range(KP_U):
            c = i * KP_U + cc
            r0 = pl.multiple_of(c * RC, RC)
            pltpu.make_async_copy(ax_hbm.at[pl.ds(r0, RC), :], xa.at[pl.ds(r0, RC), :], sem_x.at[c]).wait()
        for cc in range(KP_U):
            r0 = pl.multiple_of((i * KP_U + cc) * RC, RC)
            x = xa[pl.ds(r0, RC), :]
            for g in range(8):
                w = wqkv[:, D + g * 128:D + (g + 1) * 128]
                kbuf[g, pl.ds(r0, RC), :] = _dot(x, w).astype(bf16)
        return carry

    lax.fori_loop(0, NXC // KP_U, kproj, 0)
    cp_wq.wait()
    cp_wv.wait()

    def qvproj(i, carry):
        for cc in range(QV_U):
            c = i * QV_U + cc
            r0 = pl.multiple_of(c * RC, RC)
            x = xa[pl.ds(r0, RC), :]
            for g in range(8):
                q = _dot(x, wqkv[:, g * 128:(g + 1) * 128]) * qscale
                v = _dot(x, wqkv[:, 2 * D + g * 128:2 * D + (g + 1) * 128])
                for jj in range(RC // 128):
                    j = c * (RC // 128) + jj
                    qT[g, j] = q[jj * 128:(jj + 1) * 128].T.astype(bf16)
                    vt = v[jj * 128:(jj + 1) * 128].T.astype(bf16)
                    for hh in range(4):
                        vT[g * 4 + hh, j] = vt[hh * DHA:(hh + 1) * DHA]
        return carry

    lax.fori_loop(0, NXC // QV_U, qvproj, 0)

    k32 = kbuf.bitcast(u32)
    q32 = qT.bitcast(u32)
    v32 = vT.bitcast(u32)
    NK = S // 128

    def q_tile(g, j, hh):
        q = _bc(q32[g, j, hh * 16:(hh + 1) * 16, :])
        parts = []
        if hh > 0:
            parts.append(jnp.zeros((hh * DHA, 128), bf16))
        parts.append(q)
        if hh < 3:
            parts.append(jnp.zeros(((3 - hh) * DHA, 128), bf16))
        return jnp.concatenate(parts, axis=0) if len(parts) > 1 else q

    def qk_tile(g, qm, c, s_w):
        k = _bc(k32[g, c * 64:(c + 1) * 64, :])
        s = _dot(k, qm)
        s_w[c * 128:(c + 1) * 128, :] = s
        return jnp.max(s.reshape(16, 8, 128), axis=0)

    def half(g, j, hh, gn, qn, s_w, s_r, m, zero):
        h = g * 4 + hh
        m8 = l = acc = None
        for c in range(NK + LAG):
            if c < NK:
                mt = qk_tile(gn, qn, c, s_w)
                m8 = mt if m8 is None else jnp.maximum(m8, mt)
            if c >= LAG:
                t = c - LAG
                if zero is None:
                    s = s_r[t * 128:(t + 1) * 128, :]
                else:
                    s = s_r[pl.ds(pl.multiple_of(zero + t * 128, 128), 128), :]
                p = jnp.exp2(s - m)
                lt = jnp.sum(p.reshape(16, 8, 128), axis=0)
                l = lt if l is None else l + lt
                pv = _dot(_bc(v32[h, t]), p.astype(bf16))
                acc = pv if acc is None else acc + pv
        o = acc * (1.0 / jnp.sum(l, axis=0, keepdims=True))
        return o, jnp.max(m8, axis=0, keepdims=True)

    q0 = q_tile(0, 0, 0)
    m8 = None
    for c in range(NK):
        mt = qk_tile(0, q0, c, sa)
        m8 = mt if m8 is None else jnp.maximum(m8, mt)
    m_first = jnp.max(m8, axis=0, keepdims=True)

    cp_awo = pltpu.make_async_copy(awo_hbm, awo, sem_a.at[2])
    cp_raw = []
    for i, w_hbm in enumerate((bwq_hbm, bwk_hbm, bwv_hbm)):
        w32 = w_hbm.bitcast(u32)
        for hp in range(HB // 2):
            cp_raw.append(pltpu.make_async_copy(w32.at[:, hp, :], raw.at[i, hp], sem_raw.at[i * 16 + hp]))
    cp_wo = [pltpu.make_async_copy(bwo_hbm.at[:, pl.ds(n * 128, 128)], wo.at[n], sem_wo.at[n])
             for n in range(D // 128)]
    cp_xb = pltpu.make_async_copy(bx_hbm, xb, sem_b.at[0])
    cp_mem = pltpu.make_async_copy(bmem_hbm, mem0, sem_b.at[1])

    def repack(i, nblk):
        for wi, dst in enumerate((wq, wk, wv)):
            for hp in range(HB // 2):
                for jb in range(nblk):
                    base = pl.multiple_of(i * (16 * nblk), 16 * nblk) + jb * 16
                    ve = raw[wi, hp, pl.ds(base, 8, stride=2), :]
                    vo = raw[wi, hp, pl.ds(base + 1, 8, stride=2), :]
                    lo = (ve & jnp.uint32(0xFFFF)) | (vo << 16)
                    hi = (ve >> 16) | (vo & jnp.uint32(0xFFFF0000))
                    r = pl.ds(pl.multiple_of(i * (8 * nblk), 8 * nblk) + jb * 8, 8)
                    dst[2 * hp, r, :] = lo
                    dst[2 * hp + 1, r, :] = hi

    JU = A2_JU
    NJ = 16 // JU
    NIT = 8 * NJ
    NR = 4 * JU

    def a2_body(it, m):
        g = it // NJ
        jj = it % NJ

        @pl.when(it == 1)
        def _():
            cp_awo.start()
            for cp in cp_raw:
                cp.start()

        @pl.when(it == 4)
        def _():
            for cp in cp_wo:
                cp.start()
            cp_xb.start()
            cp_mem.start()

        zero = (it * (it + 1)) & 1
        outs = []
        for r in range(NR):
            j = JU * jj + r // 4
            hh = r % 4
            s_r, s_w = (sa, sb) if r % 2 == 0 else (sb, sa)
            if r < NR - 1:
                gn = g
                qn = q_tile(g, JU * jj + (r + 1) // 4, (r + 1) % 4)
            else:
                itn = jnp.minimum(it + 1, NIT - 1)
                gn = itn // NJ
                qn = q_tile(gn, JU * (itn % NJ), 0)
            o, m = half(g, j, hh, gn, qn, s_w, s_r, m, None if r == 0 else zero)
            outs.append(o)
            if hh == 3:
                ot = jnp.concatenate(outs, axis=0)
                outs = []
                obuf[g, pl.ds(pl.multiple_of(j * 128, 128), 128), :] = ot.T.astype(bf16)
        return m

    lax.fori_loop(0, NIT, a2_body, m_first)

    cp_awo.wait()
    for cp in cp_raw:
        cp.wait()

    def oproj(i, carry):
        repack(i, (D // 16) // (NXC // PROJ_U))
        for cc in range(PROJ_U):
            r0 = pl.multiple_of((i * PROJ_U + cc) * RC, RC)
            o = jnp.concatenate([obuf[g, pl.ds(r0, RC), :] for g in range(8)], axis=1)
            outa[pl.ds(r0, RC), :] = _dot(o, awo[...]).astype(bf16)
        return carry

    lax.fori_loop(0, NXC // PROJ_U, oproj, 0)
    cp_outa = pltpu.make_async_copy(outa, out_hbm.at[:, pl.ds(0, D)], sem_out.at[0])
    cp_outa.start()

    for cp in cp_wo:
        cp.wait()
    cp_xb.wait()
    cp_mem.wait()
    wo32 = wo.bitcast(u32)
    bscale = DHB ** -0.5
    row = lax.broadcasted_iota(jnp.int32, (48, 48), 0)
    col = lax.broadcasted_iota(jnp.int32, (48, 48), 1)
    mask = (col < MEM + SEG) & ((row < MEM) | (row >= col))
    LQ, LP = B_LQ, B_LP

    def qk_soft(q, k):
        s = _dot_t(q, k)
        s = jnp.where(mask, s * bscale, -1e9)
        m = jnp.max(s, axis=-1, keepdims=True)
        p = jnp.exp(s - m)
        l = jnp.sum(p, axis=-1, keepdims=True)
        return (p / l).astype(bf16)

    def step(hmat, assemble, finish_o):
        qs, ks, vs, ps, o_list = {}, {}, {}, {}, [None] * HB
        accs = [None] * 8

        def do_proj(h):
            qs[h] = assemble(cq, h, _dot(hmat, _bc(wq[h])))
            ks[h] = assemble(ck, h, _dot(hmat, _bc(wk[h])))
            vs[h] = assemble(cv, h, _dot(hmat, _bc(wv[h])))

        def do_wo(g):
            og = jnp.concatenate(o_list[4 * g:4 * g + 4], axis=1)
            for n in range(8):
                r = _dot(og, _bc(wo32[n, g * 256:(g + 1) * 256, :]))
                accs[n] = r if accs[n] is None else accs[n] + r

        g_next = 0
        for i in range(HB + LP):
            if i < HB:
                do_proj(i)
            else:
                do_wo(g_next)
                g_next += 1
            if 0 <= i - LQ < HB:
                ps[i - LQ] = qk_soft(qs.pop(i - LQ), ks.pop(i - LQ))
            if 0 <= i - LP < HB:
                h = i - LP
                o_list[h] = finish_o(h, _dot(ps.pop(h), vs.pop(h)))
        while g_next < 8:
            do_wo(g_next)
            g_next += 1
        return jnp.concatenate(accs, axis=1)

    def dstep(d, mem):
        base = pl.multiple_of(d * 64, 64)
        ha = jnp.concatenate([mem, xb[pl.ds(base, 40), :].astype(f32)], axis=0).astype(bf16)

        def asm_a(cref, h, v):
            cref[h] = v[40:48]
            return v.astype(bf16)

        def fin_a(h, o):
            co[h] = o[32:40]
            return o[0:32].astype(bf16)

        y = step(ha, asm_a, fin_a).astype(bf16)
        outb[pl.ds(base, 24), :] = y[8:32]
        mem1 = y[0:8].astype(f32)
        hb = jnp.concatenate([mem1, xb[pl.ds(base + 40, 24), :].astype(f32)], axis=0).astype(bf16)
        z8 = jnp.zeros((8, DHB), f32)

        def asm_b(cref, h, v):
            return jnp.concatenate([v[0:8], cref[h], v[8:32], z8], axis=0).astype(bf16)

        def fin_b(h, o):
            return jnp.concatenate([o[0:8], co[h], o[8:40]], axis=0).astype(bf16)

        y = step(hb, asm_b, fin_b).astype(bf16)
        outb[pl.ds(base + 24, 40), :] = y[8:48]
        rows = pl.ds(base, 64)
        pltpu.make_async_copy(outb.at[rows, :], out_hbm.at[rows, pl.ds(D, D)], sem_ob.at[d]).start()
        return y[0:8].astype(f32)

    lax.fori_loop(0, S // (2 * SEG), dstep, mem0[...].astype(f32))

    cp_outa.wait()

    def wait_out(d, carry):
        rows = pl.ds(pl.multiple_of(d * 64, 64), 64)
        pltpu.make_async_copy(outb.at[rows, :], out_hbm.at[rows, pl.ds(D, D)], sem_ob.at[d]).wait()
        return carry

    lax.fori_loop(0, S // (2 * SEG), wait_out, 0)


@functools.partial(jax.jit, static_argnames=("B_seg_len",))
def pallas_concat_heads__softmax_full_mha__memory_aug_recurrent_mem_tr__prompt_kernel(
    A_x: jax.Array,
    A_wqkv: jax.Array,
    A_wo: jax.Array,
    B_x: jax.Array,
    B_mem0: jax.Array,
    B_Wq: jax.Array,
    B_Wk: jax.Array,
    B_Wv: jax.Array,
    B_Wo: jax.Array,
    B_seg_len: int,
):
    assert A_x.shape == (1, S, D) and B_x.shape == (1, S, D) and B_mem0.shape == (1, MEM, D)
    assert B_Wq.shape == (D, HB, DHB) and B_Wo.shape == (HB, DHB, D) and B_seg_len == SEG
    any_spec = pl.BlockSpec(memory_space=pl.ANY)
    scratch = [
        pltpu.VMEM((S, D), bf16),
        pltpu.VMEM((D, 3 * D), bf16),
        pltpu.VMEM((D, D), bf16),
        pltpu.VMEM((8, S, 128), bf16),
        pltpu.VMEM((8, 16, 128, 128), bf16),
        pltpu.VMEM((HA, 16, DHA, 128), bf16),
        pltpu.VMEM((S, 128), f32),
        pltpu.VMEM((S, 128), f32),
        pltpu.VMEM((8, S, 128), bf16),
        pltpu.VMEM((S, D), bf16),
        pltpu.VMEM((S, D), bf16),
        pltpu.VMEM((MEM, D), bf16),
        pltpu.VMEM((3, HB // 2, D, 128), u32),
        pltpu.VMEM((HB, D // 2, 128), u32),
        pltpu.VMEM((HB, D // 2, 128), u32),
        pltpu.VMEM((HB, D // 2, 128), u32),
        pltpu.VMEM((8, HB * DHB, 128), bf16),
        pltpu.VMEM((S, D), bf16),
        pltpu.VMEM((HB, 8, 128), f32),
        pltpu.VMEM((HB, 8, 128), f32),
        pltpu.VMEM((HB, 8, 128), f32),
        pltpu.VMEM((HB, 8, 128), f32),
        pltpu.SemaphoreType.DMA((4,)),
        pltpu.SemaphoreType.DMA((8,)),
        pltpu.SemaphoreType.DMA((2,)),
        pltpu.SemaphoreType.DMA((48,)),
        pltpu.SemaphoreType.DMA((8,)),
        pltpu.SemaphoreType.DMA((1,)),
        pltpu.SemaphoreType.DMA((32,)),
    ]
    out = pl.pallas_call(
        _kernel,
        out_shape=jax.ShapeDtypeStruct((S, 2 * D), bf16),
        in_specs=[any_spec] * 9,
        out_specs=any_spec,
        scratch_shapes=scratch,
        compiler_params=pltpu.CompilerParams(vmem_limit_bytes=124 * 1024 * 1024),
        name="mha_rmt_fused",
    )(A_x.reshape(S, D), A_wqkv, A_wo, B_x.reshape(S, D), B_mem0.reshape(MEM, D),
      B_Wq, B_Wk, B_Wv, B_Wo.reshape(HB * DHB, D))
    return out.reshape(1, S, 2 * D)
```

```python
import functools

import jax
import jax.numpy as jnp
from jax import lax
import jax.experimental.pallas as pl
import jax.experimental.pallas.tpu as pltpu

bf16 = jnp.bfloat16
f32 = jnp.float32
u32 = jnp.uint32

S = 2048
D = 1024
HA = 32
DHA = 32
HB = 32
DHB = 128
MEM = 8
SEG = 32
LOG2E = 1.4426950408889634
A2_JU = 8
KP_U = 2
QV_U = 4
PROJ_U = 2
B_WG = 1
B_LQ = 2
B_LP = 6
LAG = 8


def _dot(a, b):
    return jnp.dot(a, b, preferred_element_type=f32)


def _dot_t(a, b):
    return lax.dot_general(a, b, (((1,), (1,)), ((), ())), preferred_element_type=f32)


def _bc(x):
    return pltpu.bitcast(x, bf16)


def _kernel(ax_hbm, awqkv_hbm, awo_hbm, bx_hbm, bmem_hbm, bwq_hbm, bwk_hbm, bwv_hbm, bwo_hbm,
            out_hbm,
            xa, wqkv, awo, kbuf, qT, vT, sa, sb, obuf, outa,
            xb, mem0, raw, wq, wk, wv, wo, outb, cq, ck, cv, co,
            sem_a, sem_x, sem_b, sem_raw, sem_wo, sem_out, sem_ob):
    RC = 256
    NXC = S // RC
    cp_wk = pltpu.make_async_copy(awqkv_hbm.at[:, pl.ds(D, D)], wqkv.at[:, pl.ds(D, D)], sem_a.at[0])
    cp_x = [pltpu.make_async_copy(ax_hbm.at[pl.ds(c * RC, RC), :], xa.at[pl.ds(c * RC, RC), :], sem_x.at[c])
            for c in range(NXC)]
    cp_wq = pltpu.make_async_copy(awqkv_hbm.at[:, pl.ds(0, D)], wqkv.at[:, pl.ds(0, D)], sem_a.at[1])
    cp_wv = pltpu.make_async_copy(awqkv_hbm.at[:, pl.ds(2 * D, D)], wqkv.at[:, pl.ds(2 * D, D)], sem_a.at[3])
    cp_wk.start()
    for c in range(KP_U):
        cp_x[c].start()
    cp_wk.wait()
    for c in range(KP_U, NXC):
        cp_x[c].start()
    cp_wq.start()
    cp_wv.start()


    qscale = (DHA ** -0.5) * LOG2E

    def kproj(i, carry):
        for cc in range(KP_U):
            c = i * KP_U + cc
            r0 = pl.multiple_of(c * RC, RC)
            pltpu.make_async_copy(ax_hbm.at[pl.ds(r0, RC), :], xa.at[pl.ds(r0, RC), :], sem_x.at[c]).wait()
        for cc in range(KP_U):
            r0 = pl.multiple_of((i * KP_U + cc) * RC, RC)
            x = xa[pl.ds(r0, RC), :]
            for g in range(8):
                w = wqkv[:, D + g * 128:D + (g + 1) * 128]
                kbuf[g, pl.ds(r0, RC), :] = _dot(x, w).astype(bf16)
        return carry

    lax.fori_loop(0, NXC // KP_U, kproj, 0)
    cp_wq.wait()
    cp_wv.wait()

    def qvproj(i, carry):
        for cc in range(QV_U):
            c = i * QV_U + cc
            r0 = pl.multiple_of(c * RC, RC)
            x = xa[pl.ds(r0, RC), :]
            for g in range(8):
                q = _dot(x, wqkv[:, g * 128:(g + 1) * 128]) * qscale
                v = _dot(x, wqkv[:, 2 * D + g * 128:2 * D + (g + 1) * 128])
                for jj in range(RC // 128):
                    j = c * (RC // 128) + jj
                    qT[g, j] = q[jj * 128:(jj + 1) * 128].T.astype(bf16)
                    vt = v[jj * 128:(jj + 1) * 128].T.astype(bf16)
                    for hh in range(4):
                        vT[g * 4 + hh, j] = vt[hh * DHA:(hh + 1) * DHA]
        return carry

    lax.fori_loop(0, NXC // QV_U, qvproj, 0)

    k32 = kbuf.bitcast(u32)
    q32 = qT.bitcast(u32)
    v32 = vT.bitcast(u32)
    NK = S // 128

    def q_tile(g, j, hh):
        q = _bc(q32[g, j, hh * 16:(hh + 1) * 16, :])
        parts = []
        if hh > 0:
            parts.append(jnp.zeros((hh * DHA, 128), bf16))
        parts.append(q)
        if hh < 3:
            parts.append(jnp.zeros(((3 - hh) * DHA, 128), bf16))
        return jnp.concatenate(parts, axis=0) if len(parts) > 1 else q

    def qk_tile(g, qm, c, s_w):
        k = _bc(k32[g, c * 64:(c + 1) * 64, :])
        s = _dot(k, qm)
        s_w[c * 128:(c + 1) * 128, :] = s
        return jnp.max(s.reshape(16, 8, 128), axis=0)

    def half(g, j, hh, gn, qn, s_w, s_r, m, zero):
        h = g * 4 + hh
        m8 = l = acc = None
        for c in range(NK + LAG):
            if c < NK:
                mt = qk_tile(gn, qn, c, s_w)
                m8 = mt if m8 is None else jnp.maximum(m8, mt)
            if c >= LAG:
                t = c - LAG
                if zero is None:
                    s = s_r[t * 128:(t + 1) * 128, :]
                else:
                    s = s_r[pl.ds(pl.multiple_of(zero + t * 128, 128), 128), :]
                p = jnp.exp2(s - m)
                lt = jnp.sum(p.reshape(16, 8, 128), axis=0)
                l = lt if l is None else l + lt
                pv = _dot(_bc(v32[h, t]), p.astype(bf16))
                acc = pv if acc is None else acc + pv
        o = acc * (1.0 / jnp.sum(l, axis=0, keepdims=True))
        return o, jnp.max(m8, axis=0, keepdims=True)

    q0 = q_tile(0, 0, 0)
    m8 = None
    for c in range(NK):
        mt = qk_tile(0, q0, c, sa)
        m8 = mt if m8 is None else jnp.maximum(m8, mt)
    m_first = jnp.max(m8, axis=0, keepdims=True)

    cp_awo = pltpu.make_async_copy(awo_hbm, awo, sem_a.at[2])
    cp_raw = []
    for i, w_hbm in enumerate((bwq_hbm, bwk_hbm, bwv_hbm)):
        w32 = w_hbm.bitcast(u32)
        for hp in range(HB // 2):
            cp_raw.append(pltpu.make_async_copy(w32.at[:, hp, :], raw.at[i, hp], sem_raw.at[i * 16 + hp]))
    cp_wo = [pltpu.make_async_copy(bwo_hbm.at[:, pl.ds(n * 128, 128)], wo.at[n], sem_wo.at[n])
             for n in range(D // 128)]
    cp_xb = pltpu.make_async_copy(bx_hbm, xb, sem_b.at[0])
    cp_mem = pltpu.make_async_copy(bmem_hbm, mem0, sem_b.at[1])

    def repack(i, nblk):
        for wi, dst in enumerate((wq, wk, wv)):
            for hp in range(HB // 2):
                for jb in range(nblk):
                    base = pl.multiple_of(i * (16 * nblk), 16 * nblk) + jb * 16
                    ve = raw[wi, hp, pl.ds(base, 8, stride=2), :]
                    vo = raw[wi, hp, pl.ds(base + 1, 8, stride=2), :]
                    lo = (ve & jnp.uint32(0xFFFF)) | (vo << 16)
                    hi = (ve >> 16) | (vo & jnp.uint32(0xFFFF0000))
                    r = pl.ds(pl.multiple_of(i * (8 * nblk), 8 * nblk) + jb * 8, 8)
                    dst[2 * hp, r, :] = lo
                    dst[2 * hp + 1, r, :] = hi

    JU = A2_JU
    NJ = 16 // JU
    NIT = 8 * NJ
    NR = 4 * JU

    def a2_body(it, m):
        g = it // NJ
        jj = it % NJ

        @pl.when(it == 1)
        def _():
            cp_awo.start()
            for cp in cp_raw:
                cp.start()

        @pl.when(it == 4)
        def _():
            for cp in cp_wo:
                cp.start()
            cp_xb.start()
            cp_mem.start()

        zero = (it * (it + 1)) & 1
        outs = []
        for r in range(NR):
            j = JU * jj + r // 4
            hh = r % 4
            s_r, s_w = (sa, sb) if r % 2 == 0 else (sb, sa)
            if r < NR - 1:
                gn = g
                qn = q_tile(g, JU * jj + (r + 1) // 4, (r + 1) % 4)
            else:
                itn = jnp.minimum(it + 1, NIT - 1)
                gn = itn // NJ
                qn = q_tile(gn, JU * (itn % NJ), 0)
            o, m = half(g, j, hh, gn, qn, s_w, s_r, m, None if r == 0 else zero)
            outs.append(o)
            if hh == 3:
                ot = jnp.concatenate(outs, axis=0)
                outs = []
                obuf[g, pl.ds(pl.multiple_of(j * 128, 128), 128), :] = ot.T.astype(bf16)
        return m

    lax.fori_loop(0, NIT, a2_body, m_first)

    cp_awo.wait()
    for cp in cp_raw:
        cp.wait()

    def oproj(i, carry):
        repack(i, (D // 16) // (NXC // PROJ_U))
        for cc in range(PROJ_U):
            r0 = pl.multiple_of((i * PROJ_U + cc) * RC, RC)
            o = jnp.concatenate([obuf[g, pl.ds(r0, RC), :] for g in range(8)], axis=1)
            outa[pl.ds(r0, RC), :] = _dot(o, awo[...]).astype(bf16)
        return carry

    lax.fori_loop(0, NXC // PROJ_U, oproj, 0)
    cp_outa = pltpu.make_async_copy(outa, out_hbm.at[:, pl.ds(0, D)], sem_out.at[0])
    cp_outa.start()

    for cp in cp_wo:
        cp.wait()
    cp_xb.wait()
    cp_mem.wait()
    wo32 = wo.bitcast(u32)
    bscale = DHB ** -0.5
    L = MEM + SEG
    row = lax.broadcasted_iota(jnp.int32, (2 * L, 2 * L), 0)
    col = lax.broadcasted_iota(jnp.int32, (2 * L, 2 * L), 1)
    same = (row < L) == (col < L)
    r_in = jnp.where(row < L, row, row - L)
    c_in = jnp.where(col < L, col, col - L)
    keep = same & ((r_in < MEM) | (r_in >= c_in))
    fill = jnp.where(same, -1e9, -jnp.inf).astype(f32)
    LQ, LP = B_LQ, B_LP
    NP = HB // 2

    def qk_soft(q, k):
        s = _dot_t(q, k)
        s = jnp.where(keep, s * bscale, fill)
        m = jnp.max(s, axis=-1, keepdims=True)
        p = jnp.exp(s - m)
        l = jnp.sum(p, axis=-1, keepdims=True)
        return (p / l).astype(bf16)

    def step(hmat, blocks, finish_o):
        qs, ks, vs, ps, o_list = {}, {}, {}, {}, [None] * HB
        accs = [None] * 8

        def do_proj(pr):
            parts = {}
            for h in (2 * pr, 2 * pr + 1):
                for name, w, cref in (("q", wq, cq), ("k", wk, ck), ("v", wv, cv)):
                    parts[name, h] = blocks(cref, h, _dot(hmat, _bc(w[h])))
            for name, dst in (("q", qs), ("k", ks), ("v", vs)):
                dst[pr] = jnp.concatenate([parts[name, 2 * pr], parts[name, 2 * pr + 1]], axis=0).astype(bf16)

        def do_wo(g):
            og = jnp.concatenate(o_list[4 * g:4 * g + 4], axis=1)
            for n in range(8):
                r = _dot(og, _bc(wo32[n, g * 256:(g + 1) * 256, :]))
                accs[n] = r if accs[n] is None else accs[n] + r

        g_next = 0
        for i in range(NP + LP):
            if i < NP:
                do_proj(i)
            else:
                for _ in range(B_WG):
                    do_wo(g_next)
                    g_next += 1
            if 0 <= i - LQ < NP:
                ps[i - LQ] = qk_soft(qs.pop(i - LQ), ks.pop(i - LQ))
            if 0 <= i - LP < NP:
                pr = i - LP
                o = _dot(ps.pop(pr), vs.pop(pr))
                o_list[2 * pr] = finish_o(2 * pr, o[0:L])
                o_list[2 * pr + 1] = finish_o(2 * pr + 1, o[L:2 * L])
        while g_next < 8:
            do_wo(g_next)
            g_next += 1
        return jnp.concatenate(accs, axis=1)

    def dstep(d, mem):
        base = pl.multiple_of(d * 64, 64)
        ha = jnp.concatenate([mem, xb[pl.ds(base, 40), :].astype(f32)], axis=0).astype(bf16)

        def blk_a(cref, h, v):
            cref[h] = v[40:48]
            return v[0:40]

        def fin_a(h, o):
            co[h] = o[32:40]
            return o[0:32].astype(bf16)

        y = step(ha, blk_a, fin_a).astype(bf16)
        outb[pl.ds(base, 24), :] = y[8:32]
        mem1 = y[0:8].astype(f32)
        hb = jnp.concatenate([mem1, xb[pl.ds(base + 40, 24), :].astype(f32)], axis=0).astype(bf16)

        def asm_b(cref, h, v):
            return jnp.concatenate([v[0:8], cref[h], v[8:32]], axis=0)

        def fin_b(h, o):
            return jnp.concatenate([o[0:8], co[h], o[8:40]], axis=0).astype(bf16)

        y = step(hb, asm_b, fin_b).astype(bf16)
        outb[pl.ds(base + 24, 40), :] = y[8:48]
        rows = pl.ds(base, 64)
        pltpu.make_async_copy(outb.at[rows, :], out_hbm.at[rows, pl.ds(D, D)], sem_ob.at[d]).start()
        return y[0:8].astype(f32)

    lax.fori_loop(0, S // (2 * SEG), dstep, mem0[...].astype(f32))

    cp_outa.wait()

    def wait_out(d, carry):
        rows = pl.ds(pl.multiple_of(d * 64, 64), 64)
        pltpu.make_async_copy(outb.at[rows, :], out_hbm.at[rows, pl.ds(D, D)], sem_ob.at[d]).wait()
        return carry

    lax.fori_loop(0, S // (2 * SEG), wait_out, 0)


@functools.partial(jax.jit, static_argnames=("B_seg_len",))
def pallas_concat_heads__softmax_full_mha__memory_aug_recurrent_mem_tr__prompt_kernel(
    A_x: jax.Array,
    A_wqkv: jax.Array,
    A_wo: jax.Array,
    B_x: jax.Array,
    B_mem0: jax.Array,
    B_Wq: jax.Array,
    B_Wk: jax.Array,
    B_Wv: jax.Array,
    B_Wo: jax.Array,
    B_seg_len: int,
):
    assert A_x.shape == (1, S, D) and B_x.shape == (1, S, D) and B_mem0.shape == (1, MEM, D)
    assert B_Wq.shape == (D, HB, DHB) and B_Wo.shape == (HB, DHB, D) and B_seg_len == SEG
    any_spec = pl.BlockSpec(memory_space=pl.ANY)
    scratch = [
        pltpu.VMEM((S, D), bf16),
        pltpu.VMEM((D, 3 * D), bf16),
        pltpu.VMEM((D, D), bf16),
        pltpu.VMEM((8, S, 128), bf16),
        pltpu.VMEM((8, 16, 128, 128), bf16),
        pltpu.VMEM((HA, 16, DHA, 128), bf16),
        pltpu.VMEM((S, 128), f32),
        pltpu.VMEM((S, 128), f32),
        pltpu.VMEM((8, S, 128), bf16),
        pltpu.VMEM((S, D), bf16),
        pltpu.VMEM((S, D), bf16),
        pltpu.VMEM((MEM, D), bf16),
        pltpu.VMEM((3, HB // 2, D, 128), u32),
        pltpu.VMEM((HB, D // 2, 128), u32),
        pltpu.VMEM((HB, D // 2, 128), u32),
        pltpu.VMEM((HB, D // 2, 128), u32),
        pltpu.VMEM((8, HB * DHB, 128), bf16),
        pltpu.VMEM((S, D), bf16),
        pltpu.VMEM((HB, 8, 128), f32),
        pltpu.VMEM((HB, 8, 128), f32),
        pltpu.VMEM((HB, 8, 128), f32),
        pltpu.VMEM((HB, 8, 128), f32),
        pltpu.SemaphoreType.DMA((4,)),
        pltpu.SemaphoreType.DMA((8,)),
        pltpu.SemaphoreType.DMA((2,)),
        pltpu.SemaphoreType.DMA((48,)),
        pltpu.SemaphoreType.DMA((8,)),
        pltpu.SemaphoreType.DMA((1,)),
        pltpu.SemaphoreType.DMA((32,)),
    ]
    out = pl.pallas_call(
        _kernel,
        out_shape=jax.ShapeDtypeStruct((S, 2 * D), bf16),
        in_specs=[any_spec] * 9,
        out_specs=any_spec,
        scratch_shapes=scratch,
        compiler_params=pltpu.CompilerParams(vmem_limit_bytes=124 * 1024 * 1024),
        name="mha_rmt_fused",
    )(A_x.reshape(S, D), A_wqkv, A_wo, B_x.reshape(S, D), B_mem0.reshape(MEM, D),
      B_Wq, B_Wk, B_Wv, B_Wo.reshape(HB * DHB, D))
    return out.reshape(1, S, 2 * D)
```

```python
import functools

import jax
import jax.numpy as jnp
from jax import lax
import jax.experimental.pallas as pl
import jax.experimental.pallas.tpu as pltpu

bf16 = jnp.bfloat16
f32 = jnp.float32
u32 = jnp.uint32

S = 2048
D = 1024
HA = 32
DHA = 32
HB = 32
DHB = 128
MEM = 8
SEG = 32
LOG2E = 1.4426950408889634
A2_JU = 8
KP_U = 2
QV_U = 4
PROJ_U = 2
B_WG = 1
B_LQ = 2
B_LP = 6
LAG = 9


def _dot(a, b):
    return jnp.dot(a, b, preferred_element_type=f32)


def _dot_t(a, b):
    return lax.dot_general(a, b, (((1,), (1,)), ((), ())), preferred_element_type=f32)


def _bc(x):
    return pltpu.bitcast(x, bf16)


def _kernel(ax_hbm, awqkv_hbm, awo_hbm, bx_hbm, bmem_hbm, bwq_hbm, bwk_hbm, bwv_hbm, bwo_hbm,
            out_hbm,
            xa, wqkv, awo, kbuf, qT, vT, sa, sb, obuf, outa,
            xb, mem0, raw, wq, wk, wv, wo, outb, cq, ck, cv, co,
            sem_a, sem_x, sem_b, sem_raw, sem_wo, sem_out, sem_ob):
    RC = 256
    NXC = S // RC
    cp_wk = pltpu.make_async_copy(awqkv_hbm.at[:, pl.ds(D, D)], wqkv.at[:, pl.ds(D, D)], sem_a.at[0])
    cp_x = [pltpu.make_async_copy(ax_hbm.at[pl.ds(c * RC, RC), :], xa.at[pl.ds(c * RC, RC), :], sem_x.at[c])
            for c in range(NXC)]
    cp_wq = pltpu.make_async_copy(awqkv_hbm.at[:, pl.ds(0, D)], wqkv.at[:, pl.ds(0, D)], sem_a.at[1])
    cp_wv = pltpu.make_async_copy(awqkv_hbm.at[:, pl.ds(2 * D, D)], wqkv.at[:, pl.ds(2 * D, D)], sem_a.at[3])
    cp_wk.start()
    for c in range(KP_U):
        cp_x[c].start()
    cp_wk.wait()
    for c in range(KP_U, NXC):
        cp_x[c].start()


    qscale = (DHA ** -0.5) * LOG2E

    def kproj(i, carry):
        @pl.when(i == 1)
        def _():
            cp_wq.start()
            cp_wv.start()

        for cc in range(KP_U):
            c = i * KP_U + cc
            r0 = pl.multiple_of(c * RC, RC)
            pltpu.make_async_copy(ax_hbm.at[pl.ds(r0, RC), :], xa.at[pl.ds(r0, RC), :], sem_x.at[c]).wait()
        for cc in range(KP_U):
            r0 = pl.multiple_of((i * KP_U + cc) * RC, RC)
            x = xa[pl.ds(r0, RC), :]
            for g in range(8):
                w = wqkv[:, D + g * 128:D + (g + 1) * 128]
                kbuf[g, pl.ds(r0, RC), :] = _dot(x, w).astype(bf16)
        return carry

    lax.fori_loop(0, NXC // KP_U, kproj, 0)
    cp_wq.wait()
    cp_wv.wait()

    def qvproj(i, carry):
        for cc in range(QV_U):
            c = i * QV_U + cc
            r0 = pl.multiple_of(c * RC, RC)
            x = xa[pl.ds(r0, RC), :]
            for g in range(8):
                q = _dot(x, wqkv[:, g * 128:(g + 1) * 128]) * qscale
                v = _dot(x, wqkv[:, 2 * D + g * 128:2 * D + (g + 1) * 128])
                for jj in range(RC // 128):
                    j = c * (RC // 128) + jj
                    qT[g, j] = q[jj * 128:(jj + 1) * 128].T.astype(bf16)
                    vt = v[jj * 128:(jj + 1) * 128].T.astype(bf16)
                    for hh in range(4):
                        vT[g * 4 + hh, j] = vt[hh * DHA:(hh + 1) * DHA]
        return carry

    lax.fori_loop(0, NXC // QV_U, qvproj, 0)

    k32 = kbuf.bitcast(u32)
    q32 = qT.bitcast(u32)
    v32 = vT.bitcast(u32)
    NK = S // 128

    def q_tile(g, j, hh):
        q = _bc(q32[g, j, hh * 16:(hh + 1) * 16, :])
        parts = []
        if hh > 0:
            parts.append(jnp.zeros((hh * DHA, 128), bf16))
        parts.append(q)
        if hh < 3:
            parts.append(jnp.zeros(((3 - hh) * DHA, 128), bf16))
        return jnp.concatenate(parts, axis=0) if len(parts) > 1 else q

    def qk_tile(g, qm, c, s_w):
        k = _bc(k32[g, c * 64:(c + 1) * 64, :])
        s = _dot(k, qm)
        s_w[c * 128:(c + 1) * 128, :] = s
        return jnp.max(s.reshape(16, 8, 128), axis=0)

    def half(g, hh, gn, qn, s_w, s_r, m8_cur, zero):
        h = g * 4 + hh
        m = jnp.max(m8_cur, axis=0, keepdims=True)
        m8 = l = acc = None
        for c in range(NK + LAG):
            if c < NK:
                mt = qk_tile(gn, qn, c, s_w)
                m8 = mt if m8 is None else jnp.maximum(m8, mt)
            if c >= LAG:
                t = c - LAG
                if zero is None:
                    s = s_r[t * 128:(t + 1) * 128, :]
                else:
                    s = s_r[pl.ds(pl.multiple_of(zero + t * 128, 128), 128), :]
                p = jnp.exp2(s - m)
                lt = jnp.sum(p.reshape(16, 8, 128), axis=0)
                l = lt if l is None else l + lt
                pv = _dot(_bc(v32[h, t]), p.astype(bf16))
                acc = pv if acc is None else acc + pv
        return acc, l, m8

    q0 = q_tile(0, 0, 0)
    m8 = None
    for c in range(NK):
        mt = qk_tile(0, q0, c, sa)
        m8 = mt if m8 is None else jnp.maximum(m8, mt)
    m8_first = m8

    cp_awo = pltpu.make_async_copy(awo_hbm, awo, sem_a.at[2])
    cp_raw = []
    for i, w_hbm in enumerate((bwq_hbm, bwk_hbm, bwv_hbm)):
        w32 = w_hbm.bitcast(u32)
        for hp in range(HB // 2):
            cp_raw.append(pltpu.make_async_copy(w32.at[:, hp, :], raw.at[i, hp], sem_raw.at[i * 16 + hp]))
    cp_wo = [pltpu.make_async_copy(bwo_hbm.at[:, pl.ds(n * 128, 128)], wo.at[n], sem_wo.at[n])
             for n in range(D // 128)]
    cp_xb = pltpu.make_async_copy(bx_hbm, xb, sem_b.at[0])
    cp_mem = pltpu.make_async_copy(bmem_hbm, mem0, sem_b.at[1])

    def repack(i, nblk):
        for wi, dst in enumerate((wq, wk, wv)):
            for hp in range(HB // 2):
                for jb in range(nblk):
                    base = pl.multiple_of(i * (16 * nblk), 16 * nblk) + jb * 16
                    ve = raw[wi, hp, pl.ds(base, 8, stride=2), :]
                    vo = raw[wi, hp, pl.ds(base + 1, 8, stride=2), :]
                    lo = (ve & jnp.uint32(0xFFFF)) | (vo << 16)
                    hi = (ve >> 16) | (vo & jnp.uint32(0xFFFF0000))
                    r = pl.ds(pl.multiple_of(i * (8 * nblk), 8 * nblk) + jb * 8, 8)
                    dst[2 * hp, r, :] = lo
                    dst[2 * hp + 1, r, :] = hi

    JU = A2_JU
    NJ = 16 // JU
    NIT = 8 * NJ
    NR = 4 * JU

    def normalise(acc, l):
        return acc * (1.0 / jnp.sum(l, axis=0, keepdims=True))

    def store_tile(it, outs):
        ot = jnp.concatenate(outs, axis=0)
        g = it // NJ
        j = JU * (it % NJ) + (JU - 1)
        obuf[g, pl.ds(pl.multiple_of(j * 128, 128), 128), :] = ot.T.astype(bf16)

    def a2_body(it, carry):
        m8, prev_outs, prev_acc, prev_l = carry
        g = it // NJ
        jj = it % NJ

        @pl.when(it == 1)
        def _():
            cp_awo.start()
            for cp in cp_raw:
                cp.start()

        @pl.when(it == 4)
        def _():
            for cp in cp_wo:
                cp.start()
            cp_xb.start()
            cp_mem.start()

        store_tile(jnp.maximum(it - 1, 0), list(prev_outs) + [normalise(prev_acc, prev_l)])

        zero = (it * (it + 1)) & 1
        outs = []
        for r in range(NR):
            j = JU * jj + r // 4
            hh = r % 4
            s_r, s_w = (sa, sb) if r % 2 == 0 else (sb, sa)
            if r < NR - 1:
                gn = g
                qn = q_tile(g, JU * jj + (r + 1) // 4, (r + 1) % 4)
            else:
                itn = jnp.minimum(it + 1, NIT - 1)
                gn = itn // NJ
                qn = q_tile(gn, JU * (itn % NJ), 0)
            acc, l, m8 = half(g, hh, gn, qn, s_w, s_r, m8, None if r == 0 else zero)
            if r == NR - 1:
                return m8, tuple(outs), acc, l
            outs.append(normalise(acc, l))
            if hh == 3:
                ot = jnp.concatenate(outs, axis=0)
                outs = []
                obuf[g, pl.ds(pl.multiple_of(j * 128, 128), 128), :] = ot.T.astype(bf16)

    z32 = jnp.zeros((DHA, 128), f32)
    _, last_outs, last_acc, last_l = lax.fori_loop(
        0, NIT, a2_body, (m8_first, (z32, z32, z32), z32, jnp.ones((8, 128), f32)))
    store_tile(jnp.int32(NIT - 1), list(last_outs) + [normalise(last_acc, last_l)])

    cp_awo.wait()
    for cp in cp_raw:
        cp.wait()

    def oproj(i, carry):
        repack(i, (D // 16) // (NXC // PROJ_U))
        for cc in range(PROJ_U):
            r0 = pl.multiple_of((i * PROJ_U + cc) * RC, RC)
            o = jnp.concatenate([obuf[g, pl.ds(r0, RC), :] for g in range(8)], axis=1)
            outa[pl.ds(r0, RC), :] = _dot(o, awo[...]).astype(bf16)
        return carry

    lax.fori_loop(0, NXC // PROJ_U, oproj, 0)
    cp_outa = pltpu.make_async_copy(outa, out_hbm.at[:, pl.ds(0, D)], sem_out.at[0])
    cp_outa.start()

    for cp in cp_wo:
        cp.wait()
    cp_xb.wait()
    cp_mem.wait()
    wo32 = wo.bitcast(u32)
    bscale = DHB ** -0.5
    L = MEM + SEG
    row = lax.broadcasted_iota(jnp.int32, (2 * L, 2 * L), 0)
    col = lax.broadcasted_iota(jnp.int32, (2 * L, 2 * L), 1)
    same = (row < L) == (col < L)
    r_in = jnp.where(row < L, row, row - L)
    c_in = jnp.where(col < L, col, col - L)
    keep = same & ((r_in < MEM) | (r_in >= c_in))
    fill = jnp.where(same, -1e9, -jnp.inf).astype(f32)
    LQ, LP = B_LQ, B_LP
    NP = HB // 2

    def qk_soft(q, k):
        s = _dot_t(q, k)
        s = jnp.where(keep, s * bscale, fill)
        m = jnp.max(s, axis=-1, keepdims=True)
        p = jnp.exp(s - m)
        l = jnp.sum(p, axis=-1, keepdims=True)
        return (p / l).astype(bf16)

    def step(hmat, blocks, finish_o):
        qs, ks, vs, ps, o_list = {}, {}, {}, {}, [None] * HB
        accs = [None] * 8

        def do_proj(pr):
            parts = {}
            for h in (2 * pr, 2 * pr + 1):
                for name, w, cref in (("q", wq, cq), ("k", wk, ck), ("v", wv, cv)):
                    parts[name, h] = blocks(cref, h, _dot(hmat, _bc(w[h])))
            for name, dst in (("q", qs), ("k", ks), ("v", vs)):
                dst[pr] = jnp.concatenate([parts[name, 2 * pr], parts[name, 2 * pr + 1]], axis=0).astype(bf16)

        def do_wo(g):
            og = jnp.concatenate(o_list[4 * g:4 * g + 4], axis=1)
            for n in range(8):
                r = _dot(og, _bc(wo32[n, g * 256:(g + 1) * 256, :]))
                accs[n] = r if accs[n] is None else accs[n] + r

        g_next = 0
        for i in range(NP + LP):
            if i < NP:
                do_proj(i)
            else:
                for _ in range(B_WG):
                    do_wo(g_next)
                    g_next += 1
            if 0 <= i - LQ < NP:
                ps[i - LQ] = qk_soft(qs.pop(i - LQ), ks.pop(i - LQ))
            if 0 <= i - LP < NP:
                pr = i - LP
                o = _dot(ps.pop(pr), vs.pop(pr))
                o_list[2 * pr] = finish_o(2 * pr, o[0:L])
                o_list[2 * pr + 1] = finish_o(2 * pr + 1, o[L:2 * L])
        while g_next < 8:
            do_wo(g_next)
            g_next += 1
        return jnp.concatenate(accs, axis=1)

    def dstep(d, mem):
        base = pl.multiple_of(d * 64, 64)
        ha = jnp.concatenate([mem, xb[pl.ds(base, 40), :].astype(f32)], axis=0).astype(bf16)

        def blk_a(cref, h, v):
            cref[h] = v[40:48]
            return v[0:40]

        def fin_a(h, o):
            co[h] = o[32:40]
            return o[0:32].astype(bf16)

        y = step(ha, blk_a, fin_a).astype(bf16)
        outb[pl.ds(base, 24), :] = y[8:32]
        mem1 = y[0:8].astype(f32)
        hb = jnp.concatenate([mem1, xb[pl.ds(base + 40, 24), :].astype(f32)], axis=0).astype(bf16)

        def asm_b(cref, h, v):
            return jnp.concatenate([v[0:8], cref[h], v[8:32]], axis=0)

        def fin_b(h, o):
            return jnp.concatenate([o[0:8], co[h], o[8:40]], axis=0).astype(bf16)

        y = step(hb, asm_b, fin_b).astype(bf16)
        outb[pl.ds(base + 24, 40), :] = y[8:48]
        rows = pl.ds(base, 64)
        pltpu.make_async_copy(outb.at[rows, :], out_hbm.at[rows, pl.ds(D, D)], sem_ob.at[d]).start()
        return y[0:8].astype(f32)

    lax.fori_loop(0, S // (2 * SEG), dstep, mem0[...].astype(f32))

    cp_outa.wait()

    def wait_out(d, carry):
        rows = pl.ds(pl.multiple_of(d * 64, 64), 64)
        pltpu.make_async_copy(outb.at[rows, :], out_hbm.at[rows, pl.ds(D, D)], sem_ob.at[d]).wait()
        return carry

    lax.fori_loop(0, S // (2 * SEG), wait_out, 0)


@functools.partial(jax.jit, static_argnames=("B_seg_len",))
def pallas_concat_heads__softmax_full_mha__memory_aug_recurrent_mem_tr__prompt_kernel(
    A_x: jax.Array,
    A_wqkv: jax.Array,
    A_wo: jax.Array,
    B_x: jax.Array,
    B_mem0: jax.Array,
    B_Wq: jax.Array,
    B_Wk: jax.Array,
    B_Wv: jax.Array,
    B_Wo: jax.Array,
    B_seg_len: int,
):
    assert A_x.shape == (1, S, D) and B_x.shape == (1, S, D) and B_mem0.shape == (1, MEM, D)
    assert B_Wq.shape == (D, HB, DHB) and B_Wo.shape == (HB, DHB, D) and B_seg_len == SEG
    any_spec = pl.BlockSpec(memory_space=pl.ANY)
    scratch = [
        pltpu.VMEM((S, D), bf16),
        pltpu.VMEM((D, 3 * D), bf16),
        pltpu.VMEM((D, D), bf16),
        pltpu.VMEM((8, S, 128), bf16),
        pltpu.VMEM((8, 16, 128, 128), bf16),
        pltpu.VMEM((HA, 16, DHA, 128), bf16),
        pltpu.VMEM((S, 128), f32),
        pltpu.VMEM((S, 128), f32),
        pltpu.VMEM((8, S, 128), bf16),
        pltpu.VMEM((S, D), bf16),
        pltpu.VMEM((S, D), bf16),
        pltpu.VMEM((MEM, D), bf16),
        pltpu.VMEM((3, HB // 2, D, 128), u32),
        pltpu.VMEM((HB, D // 2, 128), u32),
        pltpu.VMEM((HB, D // 2, 128), u32),
        pltpu.VMEM((HB, D // 2, 128), u32),
        pltpu.VMEM((8, HB * DHB, 128), bf16),
        pltpu.VMEM((S, D), bf16),
        pltpu.VMEM((HB, 8, 128), f32),
        pltpu.VMEM((HB, 8, 128), f32),
        pltpu.VMEM((HB, 8, 128), f32),
        pltpu.VMEM((HB, 8, 128), f32),
        pltpu.SemaphoreType.DMA((4,)),
        pltpu.SemaphoreType.DMA((8,)),
        pltpu.SemaphoreType.DMA((2,)),
        pltpu.SemaphoreType.DMA((48,)),
        pltpu.SemaphoreType.DMA((8,)),
        pltpu.SemaphoreType.DMA((1,)),
        pltpu.SemaphoreType.DMA((32,)),
    ]
    out = pl.pallas_call(
        _kernel,
        out_shape=jax.ShapeDtypeStruct((S, 2 * D), bf16),
        in_specs=[any_spec] * 9,
        out_specs=any_spec,
        scratch_shapes=scratch,
        compiler_params=pltpu.CompilerParams(vmem_limit_bytes=124 * 1024 * 1024),
        name="mha_rmt_fused",
    )(A_x.reshape(S, D), A_wqkv, A_wo, B_x.reshape(S, D), B_mem0.reshape(MEM, D),
      B_Wq, B_Wk, B_Wv, B_Wo.reshape(HB * DHB, D))
    return out.reshape(1, S, 2 * D)
```

```python
import functools

import jax
import jax.numpy as jnp
from jax import lax
import jax.experimental.pallas as pl
import jax.experimental.pallas.tpu as pltpu

bf16 = jnp.bfloat16
f32 = jnp.float32
u32 = jnp.uint32

S = 2048
D = 1024
HA = 32
DHA = 32
HB = 32
DHB = 128
MEM = 8
SEG = 32
LOG2E = 1.4426950408889634
A2_JU = 8
W_SPLIT = 1
KP_U = 2
QV_U = 4
PROJ_U = 2
B_WG = 1
B_LQ = 2
B_LP = 6
A2_PV_FIRST = False
LAG = 9


def _dot(a, b):
    return jnp.dot(a, b, preferred_element_type=f32)


def _dot_t(a, b):
    return lax.dot_general(a, b, (((1,), (1,)), ((), ())), preferred_element_type=f32)


def _bc(x):
    return pltpu.bitcast(x, bf16)


def _kernel(ax_hbm, awqkv_hbm, awo_hbm, bx_hbm, bmem_hbm, bwq_hbm, bwk_hbm, bwv_hbm, bwo_hbm,
            out_hbm,
            xa, wqkv, awo, kbuf, qT, vT, sa, sb, obuf, outa,
            xb, mem0, raw, wq, wk, wv, wo, outb, cq, ck, cv, co,
            sem_w, sem_a, sem_x, sem_b, sem_raw, sem_wo, sem_out, sem_ob):
    RC = 256
    NXC = S // RC
    WS = W_SPLIT

    def w_copies(col0, sem0):
        rows = D // WS
        return [pltpu.make_async_copy(awqkv_hbm.at[pl.ds(i * rows, rows), pl.ds(col0, D)],
                                      wqkv.at[pl.ds(i * rows, rows), pl.ds(col0, D)], sem_w.at[sem0 + i])
                for i in range(WS)]

    cp_wk = w_copies(D, 0)
    cp_wq = w_copies(0, WS)
    cp_wv = w_copies(2 * D, 2 * WS)
    cp_x = [pltpu.make_async_copy(ax_hbm.at[pl.ds(c * RC, RC), :], xa.at[pl.ds(c * RC, RC), :], sem_x.at[c])
            for c in range(NXC)]
    for cp in cp_wk:
        cp.start()
    for c in range(KP_U):
        cp_x[c].start()
    for cp in cp_wk:
        cp.wait()
    for c in range(KP_U, 2 * KP_U):
        cp_x[c].start()

    qscale = (DHA ** -0.5) * LOG2E

    def kproj(i, carry):
        for it in range(1, NXC // KP_U):
            @pl.when(i == it)
            def _():
                for c in range((it + 1) * KP_U, min((it + 2) * KP_U, NXC)):
                    cp_x[c].start()
                if it == 1:
                    for cp in cp_wq:
                        cp.start()
                if it == min(2, NXC // KP_U - 1):
                    for cp in cp_wv:
                        cp.start()

        for cc in range(KP_U):
            c = i * KP_U + cc
            r0 = pl.multiple_of(c * RC, RC)
            pltpu.make_async_copy(ax_hbm.at[pl.ds(r0, RC), :], xa.at[pl.ds(r0, RC), :], sem_x.at[c]).wait()
        for cc in range(KP_U):
            r0 = pl.multiple_of((i * KP_U + cc) * RC, RC)
            x = xa[pl.ds(r0, RC), :]
            for g in range(8):
                w = wqkv[:, D + g * 128:D + (g + 1) * 128]
                kbuf[g, pl.ds(r0, RC), :] = _dot(x, w).astype(bf16)
        return carry

    lax.fori_loop(0, NXC // KP_U, kproj, 0)
    for cp in cp_wq + cp_wv:
        cp.wait()

    def qvproj(i, carry):
        for cc in range(QV_U):
            c = i * QV_U + cc
            r0 = pl.multiple_of(c * RC, RC)
            x = xa[pl.ds(r0, RC), :]
            for g in range(8):
                q = _dot(x, wqkv[:, g * 128:(g + 1) * 128]) * qscale
                v = _dot(x, wqkv[:, 2 * D + g * 128:2 * D + (g + 1) * 128])
                for jj in range(RC // 128):
                    j = c * (RC // 128) + jj
                    qT[g, j] = q[jj * 128:(jj + 1) * 128].T.astype(bf16)
                    vt = v[jj * 128:(jj + 1) * 128].T.astype(bf16)
                    for hh in range(4):
                        vT[g * 4 + hh, j] = vt[hh * DHA:(hh + 1) * DHA]
        return carry

    lax.fori_loop(0, NXC // QV_U, qvproj, 0)

    k32 = kbuf.bitcast(u32)
    q32 = qT.bitcast(u32)
    v32 = vT.bitcast(u32)
    NK = S // 128

    def q_tile(g, j, hh):
        q = _bc(q32[g, j, hh * 16:(hh + 1) * 16, :])
        parts = []
        if hh > 0:
            parts.append(jnp.zeros((hh * DHA, 128), bf16))
        parts.append(q)
        if hh < 3:
            parts.append(jnp.zeros(((3 - hh) * DHA, 128), bf16))
        return jnp.concatenate(parts, axis=0) if len(parts) > 1 else q

    def qk_tile(g, qm, c, s_w):
        k = _bc(k32[g, c * 64:(c + 1) * 64, :])
        s = _dot(k, qm)
        s_w[c * 128:(c + 1) * 128, :] = s
        return jnp.max(s.reshape(16, 8, 128), axis=0)

    def half(g, hh, gn, qn, s_w, s_r, m8_cur, zero):
        h = g * 4 + hh
        m = jnp.max(m8_cur, axis=0, keepdims=True)
        st = {"m8": None, "l": None, "acc": None}

        def do_qk(c):
            mt = qk_tile(gn, qn, c, s_w)
            st["m8"] = mt if st["m8"] is None else jnp.maximum(st["m8"], mt)

        def do_pv(t):
            if zero is None:
                s = s_r[t * 128:(t + 1) * 128, :]
            else:
                s = s_r[pl.ds(pl.multiple_of(zero + t * 128, 128), 128), :]
            p = jnp.exp2(s - m)
            lt = jnp.sum(p.reshape(16, 8, 128), axis=0)
            st["l"] = lt if st["l"] is None else st["l"] + lt
            pv = _dot(_bc(v32[h, t]), p.astype(bf16))
            st["acc"] = pv if st["acc"] is None else st["acc"] + pv

        for c in range(NK + LAG):
            if A2_PV_FIRST and c >= LAG:
                do_pv(c - LAG)
            if c < NK:
                do_qk(c)
            if not A2_PV_FIRST and c >= LAG:
                do_pv(c - LAG)
        m8, l, acc = st["m8"], st["l"], st["acc"]
        return acc, l, m8

    q0 = q_tile(0, 0, 0)
    m8 = None
    for c in range(NK):
        mt = qk_tile(0, q0, c, sa)
        m8 = mt if m8 is None else jnp.maximum(m8, mt)
    m8_first = m8

    cp_awo = pltpu.make_async_copy(awo_hbm, awo, sem_a.at[2])
    cp_raw = []
    for i, w_hbm in enumerate((bwq_hbm, bwk_hbm, bwv_hbm)):
        w32 = w_hbm.bitcast(u32)
        for hp in range(HB // 2):
            cp_raw.append(pltpu.make_async_copy(w32.at[:, hp, :], raw.at[i, hp], sem_raw.at[i * 16 + hp]))
    cp_wo = [pltpu.make_async_copy(bwo_hbm.at[:, pl.ds(n * 128, 128)], wo.at[n], sem_wo.at[n])
             for n in range(D // 128)]
    cp_xb = pltpu.make_async_copy(bx_hbm, xb, sem_b.at[0])
    cp_mem = pltpu.make_async_copy(bmem_hbm, mem0, sem_b.at[1])

    def repack(i, nblk):
        for wi, dst in enumerate((wq, wk, wv)):
            for hp in range(HB // 2):
                for jb in range(nblk):
                    base = pl.multiple_of(i * (16 * nblk), 16 * nblk) + jb * 16
                    ve = raw[wi, hp, pl.ds(base, 8, stride=2), :]
                    vo = raw[wi, hp, pl.ds(base + 1, 8, stride=2), :]
                    lo = (ve & jnp.uint32(0xFFFF)) | (vo << 16)
                    hi = (ve >> 16) | (vo & jnp.uint32(0xFFFF0000))
                    r = pl.ds(pl.multiple_of(i * (8 * nblk), 8 * nblk) + jb * 8, 8)
                    dst[2 * hp, r, :] = lo
                    dst[2 * hp + 1, r, :] = hi

    JU = A2_JU
    NJ = 16 // JU
    NIT = 8 * NJ
    NR = 4 * JU

    def normalise(acc, l):
        return acc * (1.0 / jnp.sum(l, axis=0, keepdims=True))

    def store_tile(it, outs):
        ot = jnp.concatenate(outs, axis=0)
        g = it // NJ
        j = JU * (it % NJ) + (JU - 1)
        obuf[g, pl.ds(pl.multiple_of(j * 128, 128), 128), :] = ot.T.astype(bf16)

    def a2_body(it, carry):
        m8, prev_outs, prev_acc, prev_l = carry
        g = it // NJ
        jj = it % NJ

        @pl.when(it == 1)
        def _():
            cp_awo.start()
            for cp in cp_raw:
                cp.start()

        @pl.when(it == 4)
        def _():
            for cp in cp_wo:
                cp.start()
            cp_xb.start()
            cp_mem.start()

        store_tile(jnp.maximum(it - 1, 0), list(prev_outs) + [normalise(prev_acc, prev_l)])

        zero = (it * (it + 1)) & 1
        outs = []
        for r in range(NR):
            j = JU * jj + r // 4
            hh = r % 4
            s_r, s_w = (sa, sb) if r % 2 == 0 else (sb, sa)
            if r < NR - 1:
                gn = g
                qn = q_tile(g, JU * jj + (r + 1) // 4, (r + 1) % 4)
            else:
                itn = jnp.minimum(it + 1, NIT - 1)
                gn = itn // NJ
                qn = q_tile(gn, JU * (itn % NJ), 0)
            acc, l, m8 = half(g, hh, gn, qn, s_w, s_r, m8, None if r == 0 else zero)
            if r == NR - 1:
                return m8, tuple(outs), acc, l
            outs.append(normalise(acc, l))
            if hh == 3:
                ot = jnp.concatenate(outs, axis=0)
                outs = []
                obuf[g, pl.ds(pl.multiple_of(j * 128, 128), 128), :] = ot.T.astype(bf16)

    z32 = jnp.zeros((DHA, 128), f32)
    _, last_outs, last_acc, last_l = lax.fori_loop(
        0, NIT, a2_body, (m8_first, (z32, z32, z32), z32, jnp.ones((8, 128), f32)))
    store_tile(jnp.int32(NIT - 1), list(last_outs) + [normalise(last_acc, last_l)])

    cp_awo.wait()
    for cp in cp_raw:
        cp.wait()

    def oproj(i, carry):
        repack(i, (D // 16) // (NXC // PROJ_U))
        for cc in range(PROJ_U):
            r0 = pl.multiple_of((i * PROJ_U + cc) * RC, RC)
            o = jnp.concatenate([obuf[g, pl.ds(r0, RC), :] for g in range(8)], axis=1)
            outa[pl.ds(r0, RC), :] = _dot(o, awo[...]).astype(bf16)
        return carry

    lax.fori_loop(0, NXC // PROJ_U, oproj, 0)
    cp_outa = pltpu.make_async_copy(outa, out_hbm.at[:, pl.ds(0, D)], sem_out.at[0])
    cp_outa.start()

    for cp in cp_wo:
        cp.wait()
    cp_xb.wait()
    cp_mem.wait()
    wo32 = wo.bitcast(u32)
    bscale = DHB ** -0.5
    L = MEM + SEG
    row = lax.broadcasted_iota(jnp.int32, (2 * L, 2 * L), 0)
    col = lax.broadcasted_iota(jnp.int32, (2 * L, 2 * L), 1)
    same = (row < L) == (col < L)
    r_in = jnp.where(row < L, row, row - L)
    c_in = jnp.where(col < L, col, col - L)
    keep = same & ((r_in < MEM) | (r_in >= c_in))
    fill = jnp.where(same, -1e9, -jnp.inf).astype(f32)
    LQ, LP = B_LQ, B_LP
    NP = HB // 2

    def qk_soft(q, k):
        s = _dot_t(q, k)
        s = jnp.where(keep, s * bscale, fill)
        m = jnp.max(s, axis=-1, keepdims=True)
        p = jnp.exp(s - m)
        l = jnp.sum(p, axis=-1, keepdims=True)
        return (p / l).astype(bf16)

    def step(hmat, blocks, finish_o):
        qs, ks, vs, ps, o_list = {}, {}, {}, {}, [None] * HB
        accs = [None] * 8

        def do_proj(pr):
            parts = {}
            for h in (2 * pr, 2 * pr + 1):
                for name, w, cref in (("q", wq, cq), ("k", wk, ck), ("v", wv, cv)):
                    parts[name, h] = blocks(cref, h, _dot(hmat, _bc(w[h])))
            for name, dst in (("q", qs), ("k", ks), ("v", vs)):
                dst[pr] = jnp.concatenate([parts[name, 2 * pr], parts[name, 2 * pr + 1]], axis=0).astype(bf16)

        def do_wo(g):
            og = jnp.concatenate(o_list[4 * g:4 * g + 4], axis=1)
            for n in range(8):
                r = _dot(og, _bc(wo32[n, g * 256:(g + 1) * 256, :]))
                accs[n] = r if accs[n] is None else accs[n] + r

        g_next = 0
        for i in range(NP + LP):
            if i < NP:
                do_proj(i)
            else:
                for _ in range(B_WG):
                    do_wo(g_next)
                    g_next += 1
            if 0 <= i - LQ < NP:
                ps[i - LQ] = qk_soft(qs.pop(i - LQ), ks.pop(i - LQ))
            if 0 <= i - LP < NP:
                pr = i - LP
                o = _dot(ps.pop(pr), vs.pop(pr))
                o_list[2 * pr] = finish_o(2 * pr, o[0:L])
                o_list[2 * pr + 1] = finish_o(2 * pr + 1, o[L:2 * L])
        while g_next < 8:
            do_wo(g_next)
            g_next += 1
        return jnp.concatenate(accs, axis=1)

    def dstep(d, mem):
        base = pl.multiple_of(d * 64, 64)
        ha = jnp.concatenate([mem, xb[pl.ds(base, 40), :].astype(f32)], axis=0).astype(bf16)

        def blk_a(cref, h, v):
            cref[h] = v[40:48]
            return v[0:40]

        def fin_a(h, o):
            co[h] = o[32:40]
            return o[0:32].astype(bf16)

        y = step(ha, blk_a, fin_a).astype(bf16)
        outb[pl.ds(base, 24), :] = y[8:32]
        mem1 = y[0:8].astype(f32)
        hb = jnp.concatenate([mem1, xb[pl.ds(base + 40, 24), :].astype(f32)], axis=0).astype(bf16)

        def asm_b(cref, h, v):
            return jnp.concatenate([v[0:8], cref[h], v[8:32]], axis=0)

        def fin_b(h, o):
            return jnp.concatenate([o[0:8], co[h], o[8:40]], axis=0).astype(bf16)

        y = step(hb, asm_b, fin_b).astype(bf16)
        outb[pl.ds(base + 24, 40), :] = y[8:48]
        rows = pl.ds(base, 64)
        pltpu.make_async_copy(outb.at[rows, :], out_hbm.at[rows, pl.ds(D, D)], sem_ob.at[d]).start()
        return y[0:8].astype(f32)

    lax.fori_loop(0, S // (2 * SEG), dstep, mem0[...].astype(f32))

    cp_outa.wait()

    def wait_out(d, carry):
        rows = pl.ds(pl.multiple_of(d * 64, 64), 64)
        pltpu.make_async_copy(outb.at[rows, :], out_hbm.at[rows, pl.ds(D, D)], sem_ob.at[d]).wait()
        return carry

    lax.fori_loop(0, S // (2 * SEG), wait_out, 0)


@functools.partial(jax.jit, static_argnames=("B_seg_len",))
def pallas_concat_heads__softmax_full_mha__memory_aug_recurrent_mem_tr__prompt_kernel(
    A_x: jax.Array,
    A_wqkv: jax.Array,
    A_wo: jax.Array,
    B_x: jax.Array,
    B_mem0: jax.Array,
    B_Wq: jax.Array,
    B_Wk: jax.Array,
    B_Wv: jax.Array,
    B_Wo: jax.Array,
    B_seg_len: int,
):
    assert A_x.shape == (1, S, D) and B_x.shape == (1, S, D) and B_mem0.shape == (1, MEM, D)
    assert B_Wq.shape == (D, HB, DHB) and B_Wo.shape == (HB, DHB, D) and B_seg_len == SEG
    any_spec = pl.BlockSpec(memory_space=pl.ANY)
    scratch = [
        pltpu.VMEM((S, D), bf16),
        pltpu.VMEM((D, 3 * D), bf16),
        pltpu.VMEM((D, D), bf16),
        pltpu.VMEM((8, S, 128), bf16),
        pltpu.VMEM((8, 16, 128, 128), bf16),
        pltpu.VMEM((HA, 16, DHA, 128), bf16),
        pltpu.VMEM((S, 128), f32),
        pltpu.VMEM((S, 128), f32),
        pltpu.VMEM((8, S, 128), bf16),
        pltpu.VMEM((S, D), bf16),
        pltpu.VMEM((S, D), bf16),
        pltpu.VMEM((MEM, D), bf16),
        pltpu.VMEM((3, HB // 2, D, 128), u32),
        pltpu.VMEM((HB, D // 2, 128), u32),
        pltpu.VMEM((HB, D // 2, 128), u32),
        pltpu.VMEM((HB, D // 2, 128), u32),
        pltpu.VMEM((8, HB * DHB, 128), bf16),
        pltpu.VMEM((S, D), bf16),
        pltpu.VMEM((HB, 8, 128), f32),
        pltpu.VMEM((HB, 8, 128), f32),
        pltpu.VMEM((HB, 8, 128), f32),
        pltpu.VMEM((HB, 8, 128), f32),
        pltpu.SemaphoreType.DMA((3 * W_SPLIT,)),
        pltpu.SemaphoreType.DMA((3,)),
        pltpu.SemaphoreType.DMA((8,)),
        pltpu.SemaphoreType.DMA((2,)),
        pltpu.SemaphoreType.DMA((48,)),
        pltpu.SemaphoreType.DMA((8,)),
        pltpu.SemaphoreType.DMA((1,)),
        pltpu.SemaphoreType.DMA((32,)),
    ]
    out = pl.pallas_call(
        _kernel,
        out_shape=jax.ShapeDtypeStruct((S, 2 * D), bf16),
        in_specs=[any_spec] * 9,
        out_specs=any_spec,
        scratch_shapes=scratch,
        compiler_params=pltpu.CompilerParams(vmem_limit_bytes=124 * 1024 * 1024),
        name="mha_rmt_fused",
    )(A_x.reshape(S, D), A_wqkv, A_wo, B_x.reshape(S, D), B_mem0.reshape(MEM, D),
      B_Wq, B_Wk, B_Wv, B_Wo.reshape(HB * DHB, D))
    return out.reshape(1, S, 2 * D)
```

```python
import functools

import jax
import jax.numpy as jnp
from jax import lax
import jax.experimental.pallas as pl
import jax.experimental.pallas.tpu as pltpu

bf16 = jnp.bfloat16
f32 = jnp.float32
u32 = jnp.uint32

S = 2048
D = 1024
HA = 32
DHA = 32
HB = 32
DHB = 128
MEM = 8
SEG = 32
LOG2E = 1.4426950408889634
A2_JU = 8
QV_U = 4
PROJ_U = 2
B_U = 2
B_WG = 1
B_LQ = 2
B_LP = 6
A2_PV_FIRST = False
LAG = 9


def _dot(a, b):
    return jnp.dot(a, b, preferred_element_type=f32)


def _dot_t(a, b):
    return lax.dot_general(a, b, (((1,), (1,)), ((), ())), preferred_element_type=f32)


def _bc(x):
    return pltpu.bitcast(x, bf16)


def _kernel(ax_hbm, awqkv_hbm, awo_hbm, bx_hbm, bmem_hbm, bwq_hbm, bwk_hbm, bwv_hbm, bwo_hbm,
            out_hbm,
            xa, wqkv, awo, kbuf, qT, vT, sa, sb, obuf, outa,
            xb, mem0, raw, wq, wk, wv, wo, outb, cq, ck, cv, co,
            sem_w, sem_a, sem_x, sem_b, sem_raw, sem_wo, sem_out, sem_ob):
    RC = 256
    NXC = S // RC
    def w_copy(col0, ncol, sem):
        return pltpu.make_async_copy(awqkv_hbm.at[:, pl.ds(col0, ncol)], wqkv.at[:, pl.ds(col0, ncol)], sem)

    cp_wk0 = w_copy(D, D // 2, sem_w.at[0])
    cp_wk1 = w_copy(D + D // 2, D // 2, sem_w.at[1])
    cp_wq = w_copy(0, D, sem_w.at[2])
    cp_wv = w_copy(2 * D, D, sem_w.at[3])
    cp_x = [pltpu.make_async_copy(ax_hbm.at[pl.ds(c * RC, RC), :], xa.at[pl.ds(c * RC, RC), :], sem_x.at[c])
            for c in range(NXC)]
    cp_wk0.start(priority=0)
    cp_x[0].start(priority=0)
    cp_x[1].start(priority=0)
    cp_wk1.start(priority=1)

    qscale = (DHA ** -0.5) * LOG2E

    def kproj_chunks(r0s, groups):
        for r0 in r0s:
            x = xa[pl.ds(r0, RC), :]
            for g in groups:
                w = wqkv[:, D + g * 128:D + (g + 1) * 128]
                kbuf[g, pl.ds(r0, RC), :] = _dot(x, w).astype(bf16)

    cp_wk0.wait()
    cp_x[0].wait()
    cp_x[1].wait()
    kproj_chunks((0, RC), range(0, 4))
    cp_wk1.wait()
    for c in range(2, NXC):
        cp_x[c].start(priority=0)
    cp_wq.start(priority=1)
    cp_wv.start(priority=1)
    kproj_chunks((0, RC), range(4, 8))

    def kproj(i, carry):
        r0s = [pl.multiple_of((2 * i + cc) * RC, RC) for cc in range(2)]
        for cc in range(2):
            pltpu.make_async_copy(ax_hbm.at[pl.ds(r0s[cc], RC), :], xa.at[pl.ds(r0s[cc], RC), :],
                                  sem_x.at[2 * i + cc]).wait()
        kproj_chunks(r0s, range(8))
        return carry

    lax.fori_loop(1, NXC // 2, kproj, 0)
    cp_wq.wait()
    cp_wv.wait()

    def qvproj(i, carry):
        for cc in range(QV_U):
            c = i * QV_U + cc
            r0 = pl.multiple_of(c * RC, RC)
            x = xa[pl.ds(r0, RC), :]
            for g in range(8):
                q = _dot(x, wqkv[:, g * 128:(g + 1) * 128]) * qscale
                v = _dot(x, wqkv[:, 2 * D + g * 128:2 * D + (g + 1) * 128])
                for jj in range(RC // 128):
                    j = c * (RC // 128) + jj
                    qT[g, j] = q[jj * 128:(jj + 1) * 128].T.astype(bf16)
                    vt = v[jj * 128:(jj + 1) * 128].T.astype(bf16)
                    for hh in range(4):
                        vT[g * 4 + hh, j] = vt[hh * DHA:(hh + 1) * DHA]
        return carry

    lax.fori_loop(0, NXC // QV_U, qvproj, 0)

    k32 = kbuf.bitcast(u32)
    q32 = qT.bitcast(u32)
    v32 = vT.bitcast(u32)
    NK = S // 128

    def q_tile(g, j, hh):
        q = _bc(q32[g, j, hh * 16:(hh + 1) * 16, :])
        parts = []
        if hh > 0:
            parts.append(jnp.zeros((hh * DHA, 128), bf16))
        parts.append(q)
        if hh < 3:
            parts.append(jnp.zeros(((3 - hh) * DHA, 128), bf16))
        return jnp.concatenate(parts, axis=0) if len(parts) > 1 else q

    def qk_tile(g, qm, c, s_w):
        k = _bc(k32[g, c * 64:(c + 1) * 64, :])
        s = _dot(k, qm)
        s_w[c * 128:(c + 1) * 128, :] = s
        return jnp.max(s.reshape(16, 8, 128), axis=0)

    def half(g, hh, gn, qn, s_w, s_r, m8_cur, zero):
        h = g * 4 + hh
        m = jnp.max(m8_cur, axis=0, keepdims=True)
        st = {"m8": None, "l": None, "acc": None}

        def do_qk(c):
            mt = qk_tile(gn, qn, c, s_w)
            st["m8"] = mt if st["m8"] is None else jnp.maximum(st["m8"], mt)

        def do_pv(t):
            if zero is None:
                s = s_r[t * 128:(t + 1) * 128, :]
            else:
                s = s_r[pl.ds(pl.multiple_of(zero + t * 128, 128), 128), :]
            p = jnp.exp2(s - m)
            lt = jnp.sum(p.reshape(16, 8, 128), axis=0)
            st["l"] = lt if st["l"] is None else st["l"] + lt
            pv = _dot(_bc(v32[h, t]), p.astype(bf16))
            st["acc"] = pv if st["acc"] is None else st["acc"] + pv

        for c in range(NK + LAG):
            if A2_PV_FIRST and c >= LAG:
                do_pv(c - LAG)
            if c < NK:
                do_qk(c)
            if not A2_PV_FIRST and c >= LAG:
                do_pv(c - LAG)
        m8, l, acc = st["m8"], st["l"], st["acc"]
        return acc, l, m8

    q0 = q_tile(0, 0, 0)
    m8 = None
    for c in range(NK):
        mt = qk_tile(0, q0, c, sa)
        m8 = mt if m8 is None else jnp.maximum(m8, mt)
    m8_first = m8

    cp_awo = pltpu.make_async_copy(awo_hbm, awo, sem_a.at[2])
    cp_raw = []
    for i, w_hbm in enumerate((bwq_hbm, bwk_hbm, bwv_hbm)):
        w32 = w_hbm.bitcast(u32)
        for hp in range(HB // 2):
            cp_raw.append(pltpu.make_async_copy(w32.at[:, hp, :], raw.at[i, hp], sem_raw.at[i * 16 + hp]))
    cp_wo = [pltpu.make_async_copy(bwo_hbm.at[:, pl.ds(n * 128, 128)], wo.at[n], sem_wo.at[n])
             for n in range(D // 128)]
    cp_xb = pltpu.make_async_copy(bx_hbm, xb, sem_b.at[0])
    cp_mem = pltpu.make_async_copy(bmem_hbm, mem0, sem_b.at[1])

    def repack(i, nblk):
        for wi, dst in enumerate((wq, wk, wv)):
            for hp in range(HB // 2):
                for jb in range(nblk):
                    base = pl.multiple_of(i * (16 * nblk), 16 * nblk) + jb * 16
                    ve = raw[wi, hp, pl.ds(base, 8, stride=2), :]
                    vo = raw[wi, hp, pl.ds(base + 1, 8, stride=2), :]
                    lo = (ve & jnp.uint32(0xFFFF)) | (vo << 16)
                    hi = (ve >> 16) | (vo & jnp.uint32(0xFFFF0000))
                    r = pl.ds(pl.multiple_of(i * (8 * nblk), 8 * nblk) + jb * 8, 8)
                    dst[2 * hp, r, :] = lo
                    dst[2 * hp + 1, r, :] = hi

    JU = A2_JU
    NJ = 16 // JU
    NIT = 8 * NJ
    NR = 4 * JU

    def normalise(acc, l):
        return acc * (1.0 / jnp.sum(l, axis=0, keepdims=True))

    def store_tile(it, outs):
        ot = jnp.concatenate(outs, axis=0)
        g = it // NJ
        j = JU * (it % NJ) + (JU - 1)
        obuf[g, pl.ds(pl.multiple_of(j * 128, 128), 128), :] = ot.T.astype(bf16)

    def a2_body(it, carry):
        m8, prev_outs, prev_acc, prev_l = carry
        g = it // NJ
        jj = it % NJ

        @pl.when(it == 1)
        def _():
            cp_awo.start()
            for cp in cp_raw:
                cp.start()

        @pl.when(it == 4)
        def _():
            for cp in cp_wo:
                cp.start()
            cp_xb.start()
            cp_mem.start()

        store_tile(jnp.maximum(it - 1, 0), list(prev_outs) + [normalise(prev_acc, prev_l)])

        zero = (it * (it + 1)) & 1
        outs = []
        for r in range(NR):
            j = JU * jj + r // 4
            hh = r % 4
            s_r, s_w = (sa, sb) if r % 2 == 0 else (sb, sa)
            if r < NR - 1:
                gn = g
                qn = q_tile(g, JU * jj + (r + 1) // 4, (r + 1) % 4)
            else:
                itn = jnp.minimum(it + 1, NIT - 1)
                gn = itn // NJ
                qn = q_tile(gn, JU * (itn % NJ), 0)
            acc, l, m8 = half(g, hh, gn, qn, s_w, s_r, m8, None if r == 0 else zero)
            if r == NR - 1:
                return m8, tuple(outs), acc, l
            outs.append(normalise(acc, l))
            if hh == 3:
                ot = jnp.concatenate(outs, axis=0)
                outs = []
                obuf[g, pl.ds(pl.multiple_of(j * 128, 128), 128), :] = ot.T.astype(bf16)

    z32 = jnp.zeros((DHA, 128), f32)
    _, last_outs, last_acc, last_l = lax.fori_loop(
        0, NIT, a2_body, (m8_first, (z32, z32, z32), z32, jnp.ones((8, 128), f32)))
    store_tile(jnp.int32(NIT - 1), list(last_outs) + [normalise(last_acc, last_l)])

    cp_awo.wait()
    for cp in cp_raw:
        cp.wait()

    def oproj(i, carry):
        repack(i, (D // 16) // (NXC // PROJ_U))
        for cc in range(PROJ_U):
            r0 = pl.multiple_of((i * PROJ_U + cc) * RC, RC)
            o = jnp.concatenate([obuf[g, pl.ds(r0, RC), :] for g in range(8)], axis=1)
            outa[pl.ds(r0, RC), :] = _dot(o, awo[...]).astype(bf16)
        return carry

    lax.fori_loop(0, NXC // PROJ_U, oproj, 0)
    cp_outa = pltpu.make_async_copy(outa, out_hbm.at[:, pl.ds(0, D)], sem_out.at[0])
    cp_outa.start()

    for cp in cp_wo:
        cp.wait()
    cp_xb.wait()
    cp_mem.wait()
    wo32 = wo.bitcast(u32)
    bscale = DHB ** -0.5
    L = MEM + SEG
    row = lax.broadcasted_iota(jnp.int32, (2 * L, 2 * L), 0)
    col = lax.broadcasted_iota(jnp.int32, (2 * L, 2 * L), 1)
    same = (row < L) == (col < L)
    r_in = jnp.where(row < L, row, row - L)
    c_in = jnp.where(col < L, col, col - L)
    keep = same & ((r_in < MEM) | (r_in >= c_in))
    fill = jnp.where(same, -1e9, -jnp.inf).astype(f32)
    LQ, LP = B_LQ, B_LP
    NP = HB // 2

    def qk_soft(q, k):
        s = _dot_t(q, k)
        s = jnp.where(keep, s * bscale, fill)
        m = jnp.max(s, axis=-1, keepdims=True)
        p = jnp.exp(s - m)
        l = jnp.sum(p, axis=-1, keepdims=True)
        return (p / l).astype(bf16)

    def step(hmat, blocks, finish_o):
        qs, ks, vs, ps, o_list = {}, {}, {}, {}, [None] * HB
        accs = [None] * 8

        def do_proj(pr):
            parts = {}
            for h in (2 * pr, 2 * pr + 1):
                for name, w, cref in (("q", wq, cq), ("k", wk, ck), ("v", wv, cv)):
                    parts[name, h] = blocks(cref, h, _dot(hmat, _bc(w[h])))
            for name, dst in (("q", qs), ("k", ks), ("v", vs)):
                dst[pr] = jnp.concatenate([parts[name, 2 * pr], parts[name, 2 * pr + 1]], axis=0).astype(bf16)

        def do_wo(g):
            og = jnp.concatenate(o_list[4 * g:4 * g + 4], axis=1)
            for n in range(8):
                r = _dot(og, _bc(wo32[n, g * 256:(g + 1) * 256, :]))
                accs[n] = r if accs[n] is None else accs[n] + r

        g_next = 0
        for i in range(NP + LP):
            if i < NP:
                do_proj(i)
            else:
                for _ in range(B_WG):
                    do_wo(g_next)
                    g_next += 1
            if 0 <= i - LQ < NP:
                ps[i - LQ] = qk_soft(qs.pop(i - LQ), ks.pop(i - LQ))
            if 0 <= i - LP < NP:
                pr = i - LP
                o = _dot(ps.pop(pr), vs.pop(pr))
                o_list[2 * pr] = finish_o(2 * pr, o[0:L])
                o_list[2 * pr + 1] = finish_o(2 * pr + 1, o[L:2 * L])
        while g_next < 8:
            do_wo(g_next)
            g_next += 1
        return jnp.concatenate(accs, axis=1)

    def dstep(d, mem):
        base = pl.multiple_of(d * 64, 64)
        ha = jnp.concatenate([mem, xb[pl.ds(base, 40), :].astype(f32)], axis=0).astype(bf16)

        def blk_a(cref, h, v):
            cref[h] = v[40:48]
            return v[0:40]

        def fin_a(h, o):
            co[h] = o[32:40]
            return o[0:32].astype(bf16)

        y = step(ha, blk_a, fin_a).astype(bf16)
        outb[pl.ds(base, 24), :] = y[8:32]
        mem1 = y[0:8].astype(f32)
        hb = jnp.concatenate([mem1, xb[pl.ds(base + 40, 24), :].astype(f32)], axis=0).astype(bf16)

        def asm_b(cref, h, v):
            return jnp.concatenate([v[0:8], cref[h], v[8:32]], axis=0)

        def fin_b(h, o):
            return jnp.concatenate([o[0:8], co[h], o[8:40]], axis=0).astype(bf16)

        y = step(hb, asm_b, fin_b).astype(bf16)
        outb[pl.ds(base + 24, 40), :] = y[8:48]
        rows = pl.ds(base, 64)
        pltpu.make_async_copy(outb.at[rows, :], out_hbm.at[rows, pl.ds(D, D)], sem_ob.at[d]).start()
        return y[0:8].astype(f32)

    def dstep_n(i, mem):
        for r in range(B_U):
            mem = dstep(i * B_U + r, mem)
        return mem

    lax.fori_loop(0, S // (2 * SEG) // B_U, dstep_n, mem0[...].astype(f32))

    cp_outa.wait()

    def wait_out(d, carry):
        rows = pl.ds(pl.multiple_of(d * 64, 64), 64)
        pltpu.make_async_copy(outb.at[rows, :], out_hbm.at[rows, pl.ds(D, D)], sem_ob.at[d]).wait()
        return carry

    lax.fori_loop(0, S // (2 * SEG), wait_out, 0)


@functools.partial(jax.jit, static_argnames=("B_seg_len",))
def pallas_concat_heads__softmax_full_mha__memory_aug_recurrent_mem_tr__prompt_kernel(
    A_x: jax.Array,
    A_wqkv: jax.Array,
    A_wo: jax.Array,
    B_x: jax.Array,
    B_mem0: jax.Array,
    B_Wq: jax.Array,
    B_Wk: jax.Array,
    B_Wv: jax.Array,
    B_Wo: jax.Array,
    B_seg_len: int,
):
    assert A_x.shape == (1, S, D) and B_x.shape == (1, S, D) and B_mem0.shape == (1, MEM, D)
    assert B_Wq.shape == (D, HB, DHB) and B_Wo.shape == (HB, DHB, D) and B_seg_len == SEG
    any_spec = pl.BlockSpec(memory_space=pl.ANY)
    scratch = [
        pltpu.VMEM((S, D), bf16),
        pltpu.VMEM((D, 3 * D), bf16),
        pltpu.VMEM((D, D), bf16),
        pltpu.VMEM((8, S, 128), bf16),
        pltpu.VMEM((8, 16, 128, 128), bf16),
        pltpu.VMEM((HA, 16, DHA, 128), bf16),
        pltpu.VMEM((S, 128), f32),
        pltpu.VMEM((S, 128), f32),
        pltpu.VMEM((8, S, 128), bf16),
        pltpu.VMEM((S, D), bf16),
        pltpu.VMEM((S, D), bf16),
        pltpu.VMEM((MEM, D), bf16),
        pltpu.VMEM((3, HB // 2, D, 128), u32),
        pltpu.VMEM((HB, D // 2, 128), u32),
        pltpu.VMEM((HB, D // 2, 128), u32),
        pltpu.VMEM((HB, D // 2, 128), u32),
        pltpu.VMEM((8, HB * DHB, 128), bf16),
        pltpu.VMEM((S, D), bf16),
        pltpu.VMEM((HB, 8, 128), f32),
        pltpu.VMEM((HB, 8, 128), f32),
        pltpu.VMEM((HB, 8, 128), f32),
        pltpu.VMEM((HB, 8, 128), f32),
        pltpu.SemaphoreType.DMA((4,)),
        pltpu.SemaphoreType.DMA((3,)),
        pltpu.SemaphoreType.DMA((8,)),
        pltpu.SemaphoreType.DMA((2,)),
        pltpu.SemaphoreType.DMA((48,)),
        pltpu.SemaphoreType.DMA((8,)),
        pltpu.SemaphoreType.DMA((1,)),
        pltpu.SemaphoreType.DMA((32,)),
    ]
    out = pl.pallas_call(
        _kernel,
        out_shape=jax.ShapeDtypeStruct((S, 2 * D), bf16),
        in_specs=[any_spec] * 9,
        out_specs=any_spec,
        scratch_shapes=scratch,
        compiler_params=pltpu.CompilerParams(vmem_limit_bytes=124 * 1024 * 1024),
        name="mha_rmt_fused",
    )(A_x.reshape(S, D), A_wqkv, A_wo, B_x.reshape(S, D), B_mem0.reshape(MEM, D),
      B_Wq, B_Wk, B_Wv, B_Wo.reshape(HB * DHB, D))
    return out.reshape(1, S, 2 * D)
```

```python
import functools

import jax
import jax.numpy as jnp
from jax import lax
import jax.experimental.pallas as pl
import jax.experimental.pallas.tpu as pltpu

bf16 = jnp.bfloat16
f32 = jnp.float32
u32 = jnp.uint32

S = 2048
D = 1024
HA = 32
DHA = 32
HB = 32
DHB = 128
MEM = 8
SEG = 32
LOG2E = 1.4426950408889634
A2_JU = 8
QV_U = 4
RP_G = 4
PROJ_U = 2
B_U = 2
B_WG = 1
B_LQ = 2
B_LP = 6
A2_PV_FIRST = False
LAG = 9


def _dot(a, b):
    return jnp.dot(a, b, preferred_element_type=f32)


def _dot_t(a, b):
    return lax.dot_general(a, b, (((1,), (1,)), ((), ())), preferred_element_type=f32)


def _bc(x):
    return pltpu.bitcast(x, bf16)


def _kernel(ax_hbm, awqkv_hbm, awo_hbm, bx_hbm, bmem_hbm, bwq_hbm, bwk_hbm, bwv_hbm, bwo_hbm,
            out_hbm,
            xa, wqkv, awo, kbuf, qT, vT, sa, sb, obuf, outa,
            xb, mem0, wbuf, wo, outb, cq, ck, cv, co,
            sem_w, sem_a, sem_x, sem_b, sem_raw, sem_wo, sem_out, sem_ob):
    RC = 256
    NXC = S // RC
    def w_copy(col0, ncol, sem):
        return pltpu.make_async_copy(awqkv_hbm.at[:, pl.ds(col0, ncol)], wqkv.at[:, pl.ds(col0, ncol)], sem)

    cp_wk0 = w_copy(D, D // 2, sem_w.at[0])
    cp_wk1 = w_copy(D + D // 2, D // 2, sem_w.at[1])
    cp_wq = w_copy(0, D, sem_w.at[2])
    cp_wv = w_copy(2 * D, D, sem_w.at[3])
    cp_x = [pltpu.make_async_copy(ax_hbm.at[pl.ds(c * RC, RC), :], xa.at[pl.ds(c * RC, RC), :], sem_x.at[c])
            for c in range(NXC)]
    cp_wk0.start(priority=0)
    cp_x[0].start(priority=0)
    cp_x[1].start(priority=0)
    cp_wk1.start(priority=1)

    qscale = (DHA ** -0.5) * LOG2E

    def kproj_chunks(r0s, groups):
        for r0 in r0s:
            x = xa[pl.ds(r0, RC), :]
            for g in groups:
                w = wqkv[:, D + g * 128:D + (g + 1) * 128]
                kbuf[g, pl.ds(r0, RC), :] = _dot(x, w).astype(bf16)

    cp_wk0.wait()
    cp_x[0].wait()
    cp_x[1].wait()
    kproj_chunks((0, RC), range(0, 4))
    cp_wk1.wait()
    for c in range(2, NXC):
        cp_x[c].start(priority=0)
    cp_wq.start(priority=1)
    cp_wv.start(priority=1)
    kproj_chunks((0, RC), range(4, 8))

    def kproj(i, carry):
        r0s = [pl.multiple_of((2 * i + cc) * RC, RC) for cc in range(2)]
        for cc in range(2):
            pltpu.make_async_copy(ax_hbm.at[pl.ds(r0s[cc], RC), :], xa.at[pl.ds(r0s[cc], RC), :],
                                  sem_x.at[2 * i + cc]).wait()
        kproj_chunks(r0s, range(8))
        return carry

    lax.fori_loop(1, NXC // 2, kproj, 0)
    cp_wq.wait()
    cp_wv.wait()

    def qvproj(i, carry):
        for cc in range(QV_U):
            c = i * QV_U + cc
            r0 = pl.multiple_of(c * RC, RC)
            x = xa[pl.ds(r0, RC), :]
            for g in range(8):
                q = _dot(x, wqkv[:, g * 128:(g + 1) * 128]) * qscale
                v = _dot(x, wqkv[:, 2 * D + g * 128:2 * D + (g + 1) * 128])
                for jj in range(RC // 128):
                    j = c * (RC // 128) + jj
                    qT[g, j] = q[jj * 128:(jj + 1) * 128].T.astype(bf16)
                    vt = v[jj * 128:(jj + 1) * 128].T.astype(bf16)
                    for hh in range(4):
                        vT[g * 4 + hh, j] = vt[hh * DHA:(hh + 1) * DHA]
        return carry

    lax.fori_loop(0, NXC // QV_U, qvproj, 0)

    k32 = kbuf.bitcast(u32)
    q32 = qT.bitcast(u32)
    v32 = vT.bitcast(u32)
    NK = S // 128

    def q_tile(g, j, hh):
        q = _bc(q32[g, j, hh * 16:(hh + 1) * 16, :])
        parts = []
        if hh > 0:
            parts.append(jnp.zeros((hh * DHA, 128), bf16))
        parts.append(q)
        if hh < 3:
            parts.append(jnp.zeros(((3 - hh) * DHA, 128), bf16))
        return jnp.concatenate(parts, axis=0) if len(parts) > 1 else q

    def qk_tile(g, qm, c, s_w):
        k = _bc(k32[g, c * 64:(c + 1) * 64, :])
        s = _dot(k, qm)
        s_w[c * 128:(c + 1) * 128, :] = s
        return jnp.max(s.reshape(16, 8, 128), axis=0)

    def half(g, hh, gn, qn, s_w, s_r, m8_cur, zero):
        h = g * 4 + hh
        m = jnp.max(m8_cur, axis=0, keepdims=True)
        st = {"m8": None, "l": None, "acc": None}

        def do_qk(c):
            mt = qk_tile(gn, qn, c, s_w)
            st["m8"] = mt if st["m8"] is None else jnp.maximum(st["m8"], mt)

        def do_pv(t):
            if zero is None:
                s = s_r[t * 128:(t + 1) * 128, :]
            else:
                s = s_r[pl.ds(pl.multiple_of(zero + t * 128, 128), 128), :]
            p = jnp.exp2(s - m)
            lt = jnp.sum(p.reshape(16, 8, 128), axis=0)
            st["l"] = lt if st["l"] is None else st["l"] + lt
            pv = _dot(_bc(v32[h, t]), p.astype(bf16))
            st["acc"] = pv if st["acc"] is None else st["acc"] + pv

        for c in range(NK + LAG):
            if A2_PV_FIRST and c >= LAG:
                do_pv(c - LAG)
            if c < NK:
                do_qk(c)
            if not A2_PV_FIRST and c >= LAG:
                do_pv(c - LAG)
        m8, l, acc = st["m8"], st["l"], st["acc"]
        return acc, l, m8

    q0 = q_tile(0, 0, 0)
    m8 = None
    for c in range(NK):
        mt = qk_tile(0, q0, c, sa)
        m8 = mt if m8 is None else jnp.maximum(m8, mt)
    m8_first = m8

    cp_awo = pltpu.make_async_copy(awo_hbm, awo, sem_a.at[2])
    cp_raw = []
    for i, w_hbm in enumerate((bwq_hbm, bwk_hbm, bwv_hbm)):
        w32 = w_hbm.bitcast(u32)
        for hp in range(HB // 2):
            cp_raw.append(pltpu.make_async_copy(w32.at[:, hp, :], wbuf.at[i, pl.ds(hp * D, D), :],
                                                sem_raw.at[i * 16 + hp]))
    cp_wo = [pltpu.make_async_copy(bwo_hbm.at[:, pl.ds(n * 128, 128)], wo.at[n], sem_wo.at[n])
             for n in range(D // 128)]
    cp_xb = pltpu.make_async_copy(bx_hbm, xb, sem_b.at[0])
    cp_mem = pltpu.make_async_copy(bmem_hbm, mem0, sem_b.at[1])

    def repack_group(units):
        vals = []
        for wi, hp, blk in units:
            base = pl.multiple_of(hp * D + blk * 16, 16)
            vals.append((wbuf[wi, pl.ds(base, 8, stride=2), :], wbuf[wi, pl.ds(base + 1, 8, stride=2), :]))
        for (wi, hp, blk), (ve, vo) in zip(units, vals):
            r = pl.multiple_of(2 * hp * (D // 2) + blk * 8, 8)
            wbuf[3 + wi, pl.ds(r, 8), :] = (ve & jnp.uint32(0xFFFF)) | (vo << 16)
            wbuf[3 + wi, pl.ds(r + D // 2, 8), :] = (ve >> 16) | (vo & jnp.uint32(0xFFFF0000))

    JU = A2_JU
    NJ = 16 // JU
    NIT = 8 * NJ
    NR = 4 * JU

    def normalise(acc, l):
        return acc * (1.0 / jnp.sum(l, axis=0, keepdims=True))

    def store_tile(it, outs):
        ot = jnp.concatenate(outs, axis=0)
        g = it // NJ
        j = JU * (it % NJ) + (JU - 1)
        obuf[g, pl.ds(pl.multiple_of(j * 128, 128), 128), :] = ot.T.astype(bf16)

    def a2_body(it, carry):
        m8, prev_outs, prev_acc, prev_l = carry
        g = it // NJ
        jj = it % NJ

        @pl.when(it == 1)
        def _():
            cp_awo.start()
            for cp in cp_raw:
                cp.start()

        @pl.when(it == 4)
        def _():
            for cp in cp_wo:
                cp.start()
            cp_xb.start()
            cp_mem.start()

        store_tile(jnp.maximum(it - 1, 0), list(prev_outs) + [normalise(prev_acc, prev_l)])

        zero = (it * (it + 1)) & 1
        outs = []
        for r in range(NR):
            j = JU * jj + r // 4
            hh = r % 4
            s_r, s_w = (sa, sb) if r % 2 == 0 else (sb, sa)
            if r < NR - 1:
                gn = g
                qn = q_tile(g, JU * jj + (r + 1) // 4, (r + 1) % 4)
            else:
                itn = jnp.minimum(it + 1, NIT - 1)
                gn = itn // NJ
                qn = q_tile(gn, JU * (itn % NJ), 0)
            acc, l, m8 = half(g, hh, gn, qn, s_w, s_r, m8, None if r == 0 else zero)
            if r == NR - 1:
                return m8, tuple(outs), acc, l
            outs.append(normalise(acc, l))
            if hh == 3:
                ot = jnp.concatenate(outs, axis=0)
                outs = []
                obuf[g, pl.ds(pl.multiple_of(j * 128, 128), 128), :] = ot.T.astype(bf16)

    z32 = jnp.zeros((DHA, 128), f32)
    _, last_outs, last_acc, last_l = lax.fori_loop(
        0, NIT, a2_body, (m8_first, (z32, z32, z32), z32, jnp.ones((8, 128), f32)))
    store_tile(jnp.int32(NIT - 1), list(last_outs) + [normalise(last_acc, last_l)])

    cp_awo.wait()
    for cp in cp_raw:
        cp.wait()

    NOI = NXC // PROJ_U
    RBLK = (D // 16) // NOI

    def oproj(i, carry):
        units = [(wi, hp, jb) for jb in range(RBLK) for wi in range(3) for hp in range(HB // 2)]
        per_dot = -(-len(units) // (PROJ_U * 8))
        for cc in range(PROJ_U):
            r0 = pl.multiple_of((i * PROJ_U + cc) * RC, RC)
            o = jnp.concatenate([obuf[g, pl.ds(r0, RC), :] for g in range(8)], axis=1)
            for n in range(8):
                outa[pl.ds(r0, RC), n * 128:(n + 1) * 128] = _dot(o, awo[:, n * 128:(n + 1) * 128]).astype(bf16)
                mine, units = units[:per_dot], units[per_dot:]
                for q0 in range(0, len(mine), RP_G):
                    repack_group([(wi, hp, i * RBLK + jb) for wi, hp, jb in mine[q0:q0 + RP_G]])
        return carry

    lax.fori_loop(0, NOI, oproj, 0)
    cp_outa = pltpu.make_async_copy(outa, out_hbm.at[:, pl.ds(0, D)], sem_out.at[0])
    cp_outa.start()

    for cp in cp_wo:
        cp.wait()
    cp_xb.wait()
    cp_mem.wait()
    wo32 = wo.bitcast(u32)
    bscale = DHB ** -0.5
    L = MEM + SEG
    row = lax.broadcasted_iota(jnp.int32, (2 * L, 2 * L), 0)
    col = lax.broadcasted_iota(jnp.int32, (2 * L, 2 * L), 1)
    same = (row < L) == (col < L)
    r_in = jnp.where(row < L, row, row - L)
    c_in = jnp.where(col < L, col, col - L)
    keep = same & ((r_in < MEM) | (r_in >= c_in))
    fill = jnp.where(same, -1e9, -jnp.inf).astype(f32)
    LQ, LP = B_LQ, B_LP
    NP = HB // 2

    def qk_soft(q, k):
        s = _dot_t(q, k)
        s = jnp.where(keep, s * bscale, fill)
        m = jnp.max(s, axis=-1, keepdims=True)
        p = jnp.exp(s - m)
        l = jnp.sum(p, axis=-1, keepdims=True)
        return (p / l).astype(bf16)

    def step(hmat, blocks, finish_o):
        qs, ks, vs, ps, o_list = {}, {}, {}, {}, [None] * HB
        accs = [None] * 8

        def do_proj(pr):
            parts = {}
            for h in (2 * pr, 2 * pr + 1):
                for name, wi, cref in (("q", 3, cq), ("k", 4, ck), ("v", 5, cv)):
                    parts[name, h] = blocks(cref, h, _dot(hmat, _bc(wbuf[wi, h * (D // 2):(h + 1) * (D // 2), :])))
            for name, dst in (("q", qs), ("k", ks), ("v", vs)):
                dst[pr] = jnp.concatenate([parts[name, 2 * pr], parts[name, 2 * pr + 1]], axis=0).astype(bf16)

        def do_wo(g):
            og = jnp.concatenate(o_list[4 * g:4 * g + 4], axis=1)
            for n in range(8):
                r = _dot(og, _bc(wo32[n, g * 256:(g + 1) * 256, :]))
                accs[n] = r if accs[n] is None else accs[n] + r

        g_next = 0
        for i in range(NP + LP):
            if i < NP:
                do_proj(i)
            else:
                for _ in range(B_WG):
                    do_wo(g_next)
                    g_next += 1
            if 0 <= i - LQ < NP:
                ps[i - LQ] = qk_soft(qs.pop(i - LQ), ks.pop(i - LQ))
            if 0 <= i - LP < NP:
                pr = i - LP
                o = _dot(ps.pop(pr), vs.pop(pr))
                o_list[2 * pr] = finish_o(2 * pr, o[0:L])
                o_list[2 * pr + 1] = finish_o(2 * pr + 1, o[L:2 * L])
        while g_next < 8:
            do_wo(g_next)
            g_next += 1
        return jnp.concatenate(accs, axis=1)

    def dstep(d, mem):
        base = pl.multiple_of(d * 64, 64)
        ha = jnp.concatenate([mem, xb[pl.ds(base, 40), :].astype(f32)], axis=0).astype(bf16)

        def blk_a(cref, h, v):
            cref[h] = v[40:48]
            return v[0:40]

        def fin_a(h, o):
            co[h] = o[32:40]
            return o[0:32].astype(bf16)

        y = step(ha, blk_a, fin_a).astype(bf16)
        outb[pl.ds(base, 24), :] = y[8:32]
        mem1 = y[0:8].astype(f32)
        hb = jnp.concatenate([mem1, xb[pl.ds(base + 40, 24), :].astype(f32)], axis=0).astype(bf16)

        def asm_b(cref, h, v):
            return jnp.concatenate([v[0:8], cref[h], v[8:32]], axis=0)

        def fin_b(h, o):
            return jnp.concatenate([o[0:8], co[h], o[8:40]], axis=0).astype(bf16)

        y = step(hb, asm_b, fin_b).astype(bf16)
        outb[pl.ds(base + 24, 40), :] = y[8:48]
        rows = pl.ds(base, 64)
        pltpu.make_async_copy(outb.at[rows, :], out_hbm.at[rows, pl.ds(D, D)], sem_ob.at[d]).start()
        return y[0:8].astype(f32)

    def dstep_n(i, mem):
        for r in range(B_U):
            mem = dstep(i * B_U + r, mem)
        return mem

    lax.fori_loop(0, S // (2 * SEG) // B_U, dstep_n, mem0[...].astype(f32))

    cp_outa.wait()

    def wait_out(d, carry):
        rows = pl.ds(pl.multiple_of(d * 64, 64), 64)
        pltpu.make_async_copy(outb.at[rows, :], out_hbm.at[rows, pl.ds(D, D)], sem_ob.at[d]).wait()
        return carry

    lax.fori_loop(0, S // (2 * SEG), wait_out, 0)


@functools.partial(jax.jit, static_argnames=("B_seg_len",))
def pallas_concat_heads__softmax_full_mha__memory_aug_recurrent_mem_tr__prompt_kernel(
    A_x: jax.Array,
    A_wqkv: jax.Array,
    A_wo: jax.Array,
    B_x: jax.Array,
    B_mem0: jax.Array,
    B_Wq: jax.Array,
    B_Wk: jax.Array,
    B_Wv: jax.Array,
    B_Wo: jax.Array,
    B_seg_len: int,
):
    assert A_x.shape == (1, S, D) and B_x.shape == (1, S, D) and B_mem0.shape == (1, MEM, D)
    assert B_Wq.shape == (D, HB, DHB) and B_Wo.shape == (HB, DHB, D) and B_seg_len == SEG
    any_spec = pl.BlockSpec(memory_space=pl.ANY)
    scratch = [
        pltpu.VMEM((S, D), bf16),
        pltpu.VMEM((D, 3 * D), bf16),
        pltpu.VMEM((D, D), bf16),
        pltpu.VMEM((8, S, 128), bf16),
        pltpu.VMEM((8, 16, 128, 128), bf16),
        pltpu.VMEM((HA, 16, DHA, 128), bf16),
        pltpu.VMEM((S, 128), f32),
        pltpu.VMEM((S, 128), f32),
        pltpu.VMEM((8, S, 128), bf16),
        pltpu.VMEM((S, D), bf16),
        pltpu.VMEM((S, D), bf16),
        pltpu.VMEM((MEM, D), bf16),
        pltpu.VMEM((6, HB * D // 2, 128), u32),
        pltpu.VMEM((8, HB * DHB, 128), bf16),
        pltpu.VMEM((S, D), bf16),
        pltpu.VMEM((HB, 8, 128), f32),
        pltpu.VMEM((HB, 8, 128), f32),
        pltpu.VMEM((HB, 8, 128), f32),
        pltpu.VMEM((HB, 8, 128), f32),
        pltpu.SemaphoreType.DMA((4,)),
        pltpu.SemaphoreType.DMA((3,)),
        pltpu.SemaphoreType.DMA((8,)),
        pltpu.SemaphoreType.DMA((2,)),
        pltpu.SemaphoreType.DMA((48,)),
        pltpu.SemaphoreType.DMA((8,)),
        pltpu.SemaphoreType.DMA((1,)),
        pltpu.SemaphoreType.DMA((32,)),
    ]
    out = pl.pallas_call(
        _kernel,
        out_shape=jax.ShapeDtypeStruct((S, 2 * D), bf16),
        in_specs=[any_spec] * 9,
        out_specs=any_spec,
        scratch_shapes=scratch,
        compiler_params=pltpu.CompilerParams(vmem_limit_bytes=124 * 1024 * 1024),
        name="mha_rmt_fused",
    )(A_x.reshape(S, D), A_wqkv, A_wo, B_x.reshape(S, D), B_mem0.reshape(MEM, D),
      B_Wq, B_Wk, B_Wv, B_Wo.reshape(HB * DHB, D))
    return out.reshape(1, S, 2 * D)
```

```python
import functools

import jax
import jax.numpy as jnp
from jax import lax
import jax.experimental.pallas as pl
import jax.experimental.pallas.tpu as pltpu

bf16 = jnp.bfloat16
f32 = jnp.float32
u32 = jnp.uint32

S = 2048
D = 1024
HA = 32
DHA = 32
HB = 32
DHB = 128
MEM = 8
SEG = 32
LOG2E = 1.4426950408889634
A2_JU = 8
QV_U = 4
RP_G = 4
PROJ_U = 2
B_U = 2
B_SPLIT = 1
B_KSPLIT = ((0, 128), (128, 256), (256, 384), (384, 512), (512, 1024))
B_WG = 1
B_LQ = 2
B_LP = 6
A2_PV_FIRST = False
LAG = 9


def _dot(a, b):
    return jnp.dot(a, b, preferred_element_type=f32)


def _dot_t(a, b):
    return lax.dot_general(a, b, (((1,), (1,)), ((), ())), preferred_element_type=f32)


def _bc(x):
    return pltpu.bitcast(x, bf16)


def _kernel(ax_hbm, awqkv_hbm, awo_hbm, bx_hbm, bmem_hbm, bwq_hbm, bwk_hbm, bwv_hbm, bwo_hbm,
            out_hbm,
            xa, wqkv, awo, kbuf, qT, vT, sa, sb, obuf, outa,
            xb, mem0, wbuf, wo, outb, cq, ck, cv, co,
            sem_w, sem_a, sem_x, sem_b, sem_raw, sem_wo, sem_out, sem_ob):
    RC = 256
    NXC = S // RC
    def w_copy(col0, ncol, sem):
        return pltpu.make_async_copy(awqkv_hbm.at[:, pl.ds(col0, ncol)], wqkv.at[:, pl.ds(col0, ncol)], sem)

    cp_wk0 = w_copy(D, D // 2, sem_w.at[0])
    cp_wk1 = w_copy(D + D // 2, D // 2, sem_w.at[1])
    cp_wq = w_copy(0, D, sem_w.at[2])
    cp_wv = w_copy(2 * D, D, sem_w.at[3])
    cp_x = [pltpu.make_async_copy(ax_hbm.at[pl.ds(c * RC, RC), :], xa.at[pl.ds(c * RC, RC), :], sem_x.at[c])
            for c in range(NXC)]
    cp_wk0.start(priority=0)
    cp_x[0].start(priority=0)
    cp_x[1].start(priority=0)
    cp_wk1.start(priority=1)

    qscale = (DHA ** -0.5) * LOG2E

    def kproj_chunks(r0s, groups):
        for r0 in r0s:
            x = xa[pl.ds(r0, RC), :]
            for g in groups:
                w = wqkv[:, D + g * 128:D + (g + 1) * 128]
                kbuf[g, pl.ds(r0, RC), :] = _dot(x, w).astype(bf16)

    cp_wk0.wait()
    cp_x[0].wait()
    cp_x[1].wait()
    kproj_chunks((0, RC), range(0, 4))
    cp_wk1.wait()
    for c in range(2, NXC):
        cp_x[c].start(priority=0)
    cp_wq.start(priority=1)
    cp_wv.start(priority=1)
    kproj_chunks((0, RC), range(4, 8))

    def kproj(i, carry):
        r0s = [pl.multiple_of((2 * i + cc) * RC, RC) for cc in range(2)]
        for cc in range(2):
            pltpu.make_async_copy(ax_hbm.at[pl.ds(r0s[cc], RC), :], xa.at[pl.ds(r0s[cc], RC), :],
                                  sem_x.at[2 * i + cc]).wait()
        kproj_chunks(r0s, range(8))
        return carry

    lax.fori_loop(1, NXC // 2, kproj, 0)
    cp_wq.wait()
    cp_wv.wait()

    def qvproj(i, carry):
        for cc in range(QV_U):
            c = i * QV_U + cc
            r0 = pl.multiple_of(c * RC, RC)
            x = xa[pl.ds(r0, RC), :]
            for g in range(8):
                q = _dot(x, wqkv[:, g * 128:(g + 1) * 128]) * qscale
                v = _dot(x, wqkv[:, 2 * D + g * 128:2 * D + (g + 1) * 128])
                for jj in range(RC // 128):
                    j = c * (RC // 128) + jj
                    qT[g, j] = q[jj * 128:(jj + 1) * 128].T.astype(bf16)
                    vt = v[jj * 128:(jj + 1) * 128].T.astype(bf16)
                    for hh in range(4):
                        vT[g * 4 + hh, j] = vt[hh * DHA:(hh + 1) * DHA]
        return carry

    lax.fori_loop(0, NXC // QV_U, qvproj, 0)

    k32 = kbuf.bitcast(u32)
    q32 = qT.bitcast(u32)
    v32 = vT.bitcast(u32)
    NK = S // 128

    def q_tile(g, j, hh):
        q = _bc(q32[g, j, hh * 16:(hh + 1) * 16, :])
        parts = []
        if hh > 0:
            parts.append(jnp.zeros((hh * DHA, 128), bf16))
        parts.append(q)
        if hh < 3:
            parts.append(jnp.zeros(((3 - hh) * DHA, 128), bf16))
        return jnp.concatenate(parts, axis=0) if len(parts) > 1 else q

    def qk_tile(g, qm, c, s_w):
        k = _bc(k32[g, c * 64:(c + 1) * 64, :])
        s = _dot(k, qm)
        s_w[c * 128:(c + 1) * 128, :] = s
        return jnp.max(s.reshape(16, 8, 128), axis=0)

    def half(g, hh, gn, qn, s_w, s_r, m8_cur, zero):
        h = g * 4 + hh
        m = jnp.max(m8_cur, axis=0, keepdims=True)
        st = {"m8": None, "l": None, "acc": None}

        def do_qk(c):
            mt = qk_tile(gn, qn, c, s_w)
            st["m8"] = mt if st["m8"] is None else jnp.maximum(st["m8"], mt)

        def do_pv(t):
            if zero is None:
                s = s_r[t * 128:(t + 1) * 128, :]
            else:
                s = s_r[pl.ds(pl.multiple_of(zero + t * 128, 128), 128), :]
            p = jnp.exp2(s - m)
            lt = jnp.sum(p.reshape(16, 8, 128), axis=0)
            st["l"] = lt if st["l"] is None else st["l"] + lt
            pv = _dot(_bc(v32[h, t]), p.astype(bf16))
            st["acc"] = pv if st["acc"] is None else st["acc"] + pv

        for c in range(NK + LAG):
            if A2_PV_FIRST and c >= LAG:
                do_pv(c - LAG)
            if c < NK:
                do_qk(c)
            if not A2_PV_FIRST and c >= LAG:
                do_pv(c - LAG)
        m8, l, acc = st["m8"], st["l"], st["acc"]
        return acc, l, m8

    q0 = q_tile(0, 0, 0)
    m8 = None
    for c in range(NK):
        mt = qk_tile(0, q0, c, sa)
        m8 = mt if m8 is None else jnp.maximum(m8, mt)
    m8_first = m8

    cp_awo = pltpu.make_async_copy(awo_hbm, awo, sem_a.at[2])
    cp_raw = []
    for i, w_hbm in enumerate((bwq_hbm, bwk_hbm, bwv_hbm)):
        w32 = w_hbm.bitcast(u32)
        for hp in range(HB // 2):
            cp_raw.append(pltpu.make_async_copy(w32.at[:, hp, :], wbuf.at[i, pl.ds(hp * D, D), :],
                                                sem_raw.at[i * 16 + hp]))
    cp_wo = [pltpu.make_async_copy(bwo_hbm.at[:, pl.ds(n * 128, 128)], wo.at[n], sem_wo.at[n])
             for n in range(D // 128)]
    cp_xb = pltpu.make_async_copy(bx_hbm, xb, sem_b.at[0])
    cp_mem = pltpu.make_async_copy(bmem_hbm, mem0, sem_b.at[1])

    def repack_group(units):
        vals = []
        for wi, hp, blk in units:
            base = pl.multiple_of(hp * D + blk * 16, 16)
            vals.append((wbuf[wi, pl.ds(base, 8, stride=2), :], wbuf[wi, pl.ds(base + 1, 8, stride=2), :]))
        for (wi, hp, blk), (ve, vo) in zip(units, vals):
            r = pl.multiple_of(2 * hp * (D // 2) + blk * 8, 8)
            wbuf[3 + wi, pl.ds(r, 8), :] = (ve & jnp.uint32(0xFFFF)) | (vo << 16)
            wbuf[3 + wi, pl.ds(r + D // 2, 8), :] = (ve >> 16) | (vo & jnp.uint32(0xFFFF0000))

    JU = A2_JU
    NJ = 16 // JU
    NIT = 8 * NJ
    NR = 4 * JU

    def normalise(acc, l):
        return acc * (1.0 / jnp.sum(l, axis=0, keepdims=True))

    def store_tile(it, outs):
        ot = jnp.concatenate(outs, axis=0)
        g = it // NJ
        j = JU * (it % NJ) + (JU - 1)
        obuf[g, pl.ds(pl.multiple_of(j * 128, 128), 128), :] = ot.T.astype(bf16)

    def a2_body(it, carry):
        m8, prev_outs, prev_acc, prev_l = carry
        g = it // NJ
        jj = it % NJ

        @pl.when(it == 1)
        def _():
            cp_awo.start()
            for cp in cp_raw:
                cp.start()

        @pl.when(it == 4)
        def _():
            for cp in cp_wo:
                cp.start()
            cp_xb.start()
            cp_mem.start()

        store_tile(jnp.maximum(it - 1, 0), list(prev_outs) + [normalise(prev_acc, prev_l)])

        zero = (it * (it + 1)) & 1
        outs = []
        for r in range(NR):
            j = JU * jj + r // 4
            hh = r % 4
            s_r, s_w = (sa, sb) if r % 2 == 0 else (sb, sa)
            if r < NR - 1:
                gn = g
                qn = q_tile(g, JU * jj + (r + 1) // 4, (r + 1) % 4)
            else:
                itn = jnp.minimum(it + 1, NIT - 1)
                gn = itn // NJ
                qn = q_tile(gn, JU * (itn % NJ), 0)
            acc, l, m8 = half(g, hh, gn, qn, s_w, s_r, m8, None if r == 0 else zero)
            if r == NR - 1:
                return m8, tuple(outs), acc, l
            outs.append(normalise(acc, l))
            if hh == 3:
                ot = jnp.concatenate(outs, axis=0)
                outs = []
                obuf[g, pl.ds(pl.multiple_of(j * 128, 128), 128), :] = ot.T.astype(bf16)

    z32 = jnp.zeros((DHA, 128), f32)
    _, last_outs, last_acc, last_l = lax.fori_loop(
        0, NIT, a2_body, (m8_first, (z32, z32, z32), z32, jnp.ones((8, 128), f32)))
    store_tile(jnp.int32(NIT - 1), list(last_outs) + [normalise(last_acc, last_l)])

    cp_awo.wait()
    for cp in cp_raw:
        cp.wait()

    NOI = NXC // PROJ_U
    RBLK = (D // 16) // NOI

    def oproj(i, carry):
        units = [(wi, hp, jb) for jb in range(RBLK) for wi in range(3) for hp in range(HB // 2)]
        per_dot = -(-len(units) // (PROJ_U * 8))
        for cc in range(PROJ_U):
            r0 = pl.multiple_of((i * PROJ_U + cc) * RC, RC)
            o = jnp.concatenate([obuf[g, pl.ds(r0, RC), :] for g in range(8)], axis=1)
            for n in range(8):
                outa[pl.ds(r0, RC), n * 128:(n + 1) * 128] = _dot(o, awo[:, n * 128:(n + 1) * 128]).astype(bf16)
                mine, units = units[:per_dot], units[per_dot:]
                for q0 in range(0, len(mine), RP_G):
                    repack_group([(wi, hp, i * RBLK + jb) for wi, hp, jb in mine[q0:q0 + RP_G]])
        return carry

    lax.fori_loop(0, NOI, oproj, 0)
    cp_outa = pltpu.make_async_copy(outa, out_hbm.at[:, pl.ds(0, D)], sem_out.at[0])
    cp_outa.start()

    for cp in cp_wo:
        cp.wait()
    cp_xb.wait()
    cp_mem.wait()
    wo32 = wo.bitcast(u32)
    bscale = DHB ** -0.5
    L = MEM + SEG
    row = lax.broadcasted_iota(jnp.int32, (2 * L, 2 * L), 0)
    col = lax.broadcasted_iota(jnp.int32, (2 * L, 2 * L), 1)
    same = (row < L) == (col < L)
    r_in = jnp.where(row < L, row, row - L)
    c_in = jnp.where(col < L, col, col - L)
    keep = same & ((r_in < MEM) | (r_in >= c_in))
    fill = jnp.where(same, -1e9, -jnp.inf).astype(f32)
    LQ, LP = B_LQ, B_LP
    NP = HB // 2

    def qk_soft(q, k):
        s = _dot_t(q, k)
        s = jnp.where(keep, s * bscale, fill)
        m = jnp.max(s, axis=-1, keepdims=True)
        p = jnp.exp(s - m)
        l = jnp.sum(p, axis=-1, keepdims=True)
        return (p / l).astype(bf16)

    def step(hmat, blocks, finish_o):
        qs, ks, vs, ps, o_list = {}, {}, {}, {}, [None] * HB
        accs = [None] * 8

        def do_proj(pr):
            parts = {}
            todo = [(name, wi, cref, h) for h in (2 * pr, 2 * pr + 1)
                    for name, wi, cref in (("q", 3, cq), ("k", 4, ck), ("v", 5, cv))]
            if pr < B_SPLIT:
                acc = [None] * len(todo)
                for k0, k1 in B_KSPLIT:
                    for t, (_, wi, _, h) in enumerate(todo):
                        w = _bc(wbuf[wi, h * (D // 2) + k0 // 2:h * (D // 2) + k1 // 2, :])
                        r = _dot(hmat[:, k0:k1], w)
                        if acc[t] is not None:
                            r = r + acc[t]
                        acc[t] = r
                for (name, wi, cref, h), r in zip(todo, acc):
                    parts[name, h] = blocks(cref, h, r)
            else:
                for name, wi, cref, h in todo:
                    parts[name, h] = blocks(cref, h, _dot(hmat, _bc(wbuf[wi, h * (D // 2):(h + 1) * (D // 2), :])))
            for name, dst in (("q", qs), ("k", ks), ("v", vs)):
                dst[pr] = jnp.concatenate([parts[name, 2 * pr], parts[name, 2 * pr + 1]], axis=0).astype(bf16)

        def do_wo(g):
            og = jnp.concatenate(o_list[4 * g:4 * g + 4], axis=1)
            for n in range(8):
                r = _dot(og, _bc(wo32[n, g * 256:(g + 1) * 256, :]))
                accs[n] = r if accs[n] is None else accs[n] + r

        g_next = 0
        for i in range(NP + LP):
            if i < NP:
                do_proj(i)
            else:
                for _ in range(B_WG):
                    do_wo(g_next)
                    g_next += 1
            if 0 <= i - LQ < NP:
                ps[i - LQ] = qk_soft(qs.pop(i - LQ), ks.pop(i - LQ))
            if 0 <= i - LP < NP:
                pr = i - LP
                o = _dot(ps.pop(pr), vs.pop(pr))
                o_list[2 * pr] = finish_o(2 * pr, o[0:L])
                o_list[2 * pr + 1] = finish_o(2 * pr + 1, o[L:2 * L])
        while g_next < 8:
            do_wo(g_next)
            g_next += 1
        return jnp.concatenate(accs, axis=1)

    def dstep(d, mem):
        base = pl.multiple_of(d * 64, 64)
        ha = jnp.concatenate([mem, xb[pl.ds(base, 40), :].astype(f32)], axis=0).astype(bf16)

        def blk_a(cref, h, v):
            cref[h] = v[40:48]
            return v[0:40]

        def fin_a(h, o):
            co[h] = o[32:40]
            return o[0:32].astype(bf16)

        y = step(ha, blk_a, fin_a).astype(bf16)
        outb[pl.ds(base, 24), :] = y[8:32]
        mem1 = y[0:8].astype(f32)
        hb = jnp.concatenate([mem1, xb[pl.ds(base + 40, 24), :].astype(f32)], axis=0).astype(bf16)

        def asm_b(cref, h, v):
            return jnp.concatenate([v[0:8], cref[h], v[8:32]], axis=0)

        def fin_b(h, o):
            return jnp.concatenate([o[0:8], co[h], o[8:40]], axis=0).astype(bf16)

        y = step(hb, asm_b, fin_b).astype(bf16)
        outb[pl.ds(base + 24, 40), :] = y[8:48]
        rows = pl.ds(base, 64)
        pltpu.make_async_copy(outb.at[rows, :], out_hbm.at[rows, pl.ds(D, D)], sem_ob.at[d]).start()
        return y[0:8].astype(f32)

    def dstep_n(i, mem):
        for r in range(B_U):
            mem = dstep(i * B_U + r, mem)
        return mem

    lax.fori_loop(0, S // (2 * SEG) // B_U, dstep_n, mem0[...].astype(f32))

    cp_outa.wait()

    def wait_out(d, carry):
        rows = pl.ds(pl.multiple_of(d * 64, 64), 64)
        pltpu.make_async_copy(outb.at[rows, :], out_hbm.at[rows, pl.ds(D, D)], sem_ob.at[d]).wait()
        return carry

    lax.fori_loop(0, S // (2 * SEG), wait_out, 0)


@functools.partial(jax.jit, static_argnames=("B_seg_len",))
def pallas_concat_heads__softmax_full_mha__memory_aug_recurrent_mem_tr__prompt_kernel(
    A_x: jax.Array,
    A_wqkv: jax.Array,
    A_wo: jax.Array,
    B_x: jax.Array,
    B_mem0: jax.Array,
    B_Wq: jax.Array,
    B_Wk: jax.Array,
    B_Wv: jax.Array,
    B_Wo: jax.Array,
    B_seg_len: int,
):
    assert A_x.shape == (1, S, D) and B_x.shape == (1, S, D) and B_mem0.shape == (1, MEM, D)
    assert B_Wq.shape == (D, HB, DHB) and B_Wo.shape == (HB, DHB, D) and B_seg_len == SEG
    any_spec = pl.BlockSpec(memory_space=pl.ANY)
    scratch = [
        pltpu.VMEM((S, D), bf16),
        pltpu.VMEM((D, 3 * D), bf16),
        pltpu.VMEM((D, D), bf16),
        pltpu.VMEM((8, S, 128), bf16),
        pltpu.VMEM((8, 16, 128, 128), bf16),
        pltpu.VMEM((HA, 16, DHA, 128), bf16),
        pltpu.VMEM((S, 128), f32),
        pltpu.VMEM((S, 128), f32),
        pltpu.VMEM((8, S, 128), bf16),
        pltpu.VMEM((S, D), bf16),
        pltpu.VMEM((S, D), bf16),
        pltpu.VMEM((MEM, D), bf16),
        pltpu.VMEM((6, HB * D // 2, 128), u32),
        pltpu.VMEM((8, HB * DHB, 128), bf16),
        pltpu.VMEM((S, D), bf16),
        pltpu.VMEM((HB, 8, 128), f32),
        pltpu.VMEM((HB, 8, 128), f32),
        pltpu.VMEM((HB, 8, 128), f32),
        pltpu.VMEM((HB, 8, 128), f32),
        pltpu.SemaphoreType.DMA((4,)),
        pltpu.SemaphoreType.DMA((3,)),
        pltpu.SemaphoreType.DMA((8,)),
        pltpu.SemaphoreType.DMA((2,)),
        pltpu.SemaphoreType.DMA((48,)),
        pltpu.SemaphoreType.DMA((8,)),
        pltpu.SemaphoreType.DMA((1,)),
        pltpu.SemaphoreType.DMA((32,)),
    ]
    out = pl.pallas_call(
        _kernel,
        out_shape=jax.ShapeDtypeStruct((S, 2 * D), bf16),
        in_specs=[any_spec] * 9,
        out_specs=any_spec,
        scratch_shapes=scratch,
        compiler_params=pltpu.CompilerParams(vmem_limit_bytes=124 * 1024 * 1024),
        name="mha_rmt_fused",
    )(A_x.reshape(S, D), A_wqkv, A_wo, B_x.reshape(S, D), B_mem0.reshape(MEM, D),
      B_Wq, B_Wk, B_Wv, B_Wo.reshape(HB * DHB, D))
    return out.reshape(1, S, 2 * D)
```

```python
import functools

import jax
import jax.numpy as jnp
from jax import lax
import jax.experimental.pallas as pl
import jax.experimental.pallas.tpu as pltpu

bf16 = jnp.bfloat16
f32 = jnp.float32
u32 = jnp.uint32

S = 2048
D = 1024
HA = 32
DHA = 32
HB = 32
DHB = 128
MEM = 8
SEG = 32
LOG2E = 1.4426950408889634
A2_JU = 8
KG0 = 3
QV_U = 4
RP_G = 4
PROJ_U = 4
B_U = 2
B_SPLIT = 1
B_KSPLIT = ((0, 128), (128, 256), (256, 384), (384, 512), (512, 1024))
B_WG = 1
B_LQ = 2
B_LP = 6
A2_PV_FIRST = False
LAG = 9


def _dot(a, b):
    return jnp.dot(a, b, preferred_element_type=f32)


def _dot_t(a, b):
    return lax.dot_general(a, b, (((1,), (1,)), ((), ())), preferred_element_type=f32)


def _bc(x):
    return pltpu.bitcast(x, bf16)


def _kernel(ax_hbm, awqkv_hbm, awo_hbm, bx_hbm, bmem_hbm, bwq_hbm, bwk_hbm, bwv_hbm, bwo_hbm,
            out_hbm,
            xa, wqkv, awo, kbuf, qT, vT, sa, sb, obuf, outa,
            xb, mem0, wbuf, wo, outb, cq, ck, cv, co,
            sem_w, sem_a, sem_x, sem_b, sem_raw, sem_wo, sem_out, sem_ob):
    RC = 256
    NXC = S // RC

    def w_copy(col0, ncol, sem):
        return pltpu.make_async_copy(awqkv_hbm.at[:, pl.ds(col0, ncol)], wqkv.at[:, pl.ds(col0, ncol)], sem)

    cp_wk0 = w_copy(D, KG0 * 128, sem_w.at[0])
    cp_wk1 = w_copy(D + KG0 * 128, (8 - KG0) * 128, sem_w.at[1])
    cp_wq = w_copy(0, D, sem_w.at[2])
    cp_wv = w_copy(2 * D, D, sem_w.at[3])
    cp_x = [pltpu.make_async_copy(ax_hbm.at[pl.ds(c * RC, RC), :], xa.at[pl.ds(c * RC, RC), :], sem_x.at[c])
            for c in range(NXC)]
    cp_wk0.start(priority=0)
    cp_x[0].start(priority=0)
    cp_x[1].start(priority=0)
    cp_wk1.start(priority=1)

    qscale = (DHA ** -0.5) * LOG2E

    def kproj_chunks(r0s, groups):
        for r0 in r0s:
            x = xa[pl.ds(r0, RC), :]
            for g in groups:
                w = wqkv[:, D + g * 128:D + (g + 1) * 128]
                kbuf[g, pl.ds(r0, RC), :] = _dot(x, w).astype(bf16)

    cp_wk0.wait()
    cp_x[0].wait()
    cp_x[1].wait()
    kproj_chunks((0, RC), range(0, KG0))
    cp_wk1.wait()
    for c in range(2, NXC):
        cp_x[c].start(priority=0)
    cp_wq.start(priority=1)
    cp_wv.start(priority=1)
    kproj_chunks((0, RC), range(KG0, 8))

    def kproj(i, carry):
        r0s = [pl.multiple_of((2 * i + cc) * RC, RC) for cc in range(2)]
        for cc in range(2):
            pltpu.make_async_copy(ax_hbm.at[pl.ds(r0s[cc], RC), :], xa.at[pl.ds(r0s[cc], RC), :],
                                  sem_x.at[2 * i + cc]).wait()
        kproj_chunks(r0s, range(8))
        return carry

    lax.fori_loop(1, NXC // 2, kproj, 0)
    cp_wq.wait()
    cp_wv.wait()

    def qvproj(i, carry):
        for cc in range(QV_U):
            c = i * QV_U + cc
            r0 = pl.multiple_of(c * RC, RC)
            x = xa[pl.ds(r0, RC), :]
            for g in range(8):
                q = _dot(x, wqkv[:, g * 128:(g + 1) * 128]) * qscale
                v = _dot(x, wqkv[:, 2 * D + g * 128:2 * D + (g + 1) * 128])
                for jj in range(RC // 128):
                    j = c * (RC // 128) + jj
                    qT[g, j] = q[jj * 128:(jj + 1) * 128].T.astype(bf16)
                    vt = v[jj * 128:(jj + 1) * 128].T.astype(bf16)
                    for hh in range(4):
                        vT[g * 4 + hh, j] = vt[hh * DHA:(hh + 1) * DHA]
        return carry

    lax.fori_loop(0, NXC // QV_U, qvproj, 0)

    k32 = kbuf.bitcast(u32)
    q32 = qT.bitcast(u32)
    v32 = vT.bitcast(u32)
    NK = S // 128

    def q_tile(g, j, hh):
        q = _bc(q32[g, j, hh * 16:(hh + 1) * 16, :])
        parts = []
        if hh > 0:
            parts.append(jnp.zeros((hh * DHA, 128), bf16))
        parts.append(q)
        if hh < 3:
            parts.append(jnp.zeros(((3 - hh) * DHA, 128), bf16))
        return jnp.concatenate(parts, axis=0) if len(parts) > 1 else q

    def qk_tile(g, qm, c, s_w):
        k = _bc(k32[g, c * 64:(c + 1) * 64, :])
        s = _dot(k, qm)
        s_w[c * 128:(c + 1) * 128, :] = s
        return jnp.max(s.reshape(16, 8, 128), axis=0)

    def half(g, hh, gn, qn, s_w, s_r, m8_cur, zero):
        h = g * 4 + hh
        m = jnp.max(m8_cur, axis=0, keepdims=True)
        st = {"m8": None, "l": None, "acc": None}

        def do_qk(c):
            mt = qk_tile(gn, qn, c, s_w)
            st["m8"] = mt if st["m8"] is None else jnp.maximum(st["m8"], mt)

        def do_pv(t):
            if zero is None:
                s = s_r[t * 128:(t + 1) * 128, :]
            else:
                s = s_r[pl.ds(pl.multiple_of(zero + t * 128, 128), 128), :]
            p = jnp.exp2(s - m)
            lt = jnp.sum(p.reshape(16, 8, 128), axis=0)
            st["l"] = lt if st["l"] is None else st["l"] + lt
            pv = _dot(_bc(v32[h, t]), p.astype(bf16))
            st["acc"] = pv if st["acc"] is None else st["acc"] + pv

        for c in range(NK + LAG):
            if A2_PV_FIRST and c >= LAG:
                do_pv(c - LAG)
            if c < NK:
                do_qk(c)
            if not A2_PV_FIRST and c >= LAG:
                do_pv(c - LAG)
        m8, l, acc = st["m8"], st["l"], st["acc"]
        return acc, l, m8

    q0 = q_tile(0, 0, 0)
    m8 = None
    for c in range(NK):
        mt = qk_tile(0, q0, c, sa)
        m8 = mt if m8 is None else jnp.maximum(m8, mt)
    m8_first = m8

    cp_awo = pltpu.make_async_copy(awo_hbm, awo, sem_a.at[2])
    cp_raw = []
    for i, w_hbm in enumerate((bwq_hbm, bwk_hbm, bwv_hbm)):
        w32 = w_hbm.bitcast(u32)
        for hp in range(HB // 2):
            cp_raw.append(pltpu.make_async_copy(w32.at[:, hp, :], wbuf.at[i, pl.ds(hp * D, D), :],
                                                sem_raw.at[i * 16 + hp]))
    cp_wo = [pltpu.make_async_copy(bwo_hbm.at[:, pl.ds(n * 128, 128)], wo.at[n], sem_wo.at[n])
             for n in range(D // 128)]
    cp_xb = pltpu.make_async_copy(bx_hbm, xb, sem_b.at[0])
    cp_mem = pltpu.make_async_copy(bmem_hbm, mem0, sem_b.at[1])

    def repack_group(units):
        vals = []
        for wi, hp, blk in units:
            base = pl.multiple_of(hp * D + blk * 16, 16)
            vals.append((wbuf[wi, pl.ds(base, 8, stride=2), :], wbuf[wi, pl.ds(base + 1, 8, stride=2), :]))
        for (wi, hp, blk), (ve, vo) in zip(units, vals):
            r = pl.multiple_of(2 * hp * (D // 2) + blk * 8, 8)
            wbuf[3 + wi, pl.ds(r, 8), :] = (ve & jnp.uint32(0xFFFF)) | (vo << 16)
            wbuf[3 + wi, pl.ds(r + D // 2, 8), :] = (ve >> 16) | (vo & jnp.uint32(0xFFFF0000))

    JU = A2_JU
    NJ = 16 // JU
    NIT = 8 * NJ
    NR = 4 * JU

    def normalise(acc, l):
        return acc * (1.0 / jnp.sum(l, axis=0, keepdims=True))

    def store_tile(it, outs):
        ot = jnp.concatenate(outs, axis=0)
        g = it // NJ
        j = JU * (it % NJ) + (JU - 1)
        obuf[g, pl.ds(pl.multiple_of(j * 128, 128), 128), :] = ot.T.astype(bf16)

    def a2_body(it, carry):
        m8, prev_outs, prev_acc, prev_l = carry
        g = it // NJ
        jj = it % NJ

        @pl.when(it == 1)
        def _():
            cp_awo.start()
            for cp in cp_raw:
                cp.start()

        @pl.when(it == 4)
        def _():
            for cp in cp_wo:
                cp.start()
            cp_xb.start()
            cp_mem.start()

        store_tile(jnp.maximum(it - 1, 0), list(prev_outs) + [normalise(prev_acc, prev_l)])

        zero = (it * (it + 1)) & 1
        outs = []
        for r in range(NR):
            j = JU * jj + r // 4
            hh = r % 4
            s_r, s_w = (sa, sb) if r % 2 == 0 else (sb, sa)
            if r < NR - 1:
                gn = g
                qn = q_tile(g, JU * jj + (r + 1) // 4, (r + 1) % 4)
            else:
                itn = jnp.minimum(it + 1, NIT - 1)
                gn = itn // NJ
                qn = q_tile(gn, JU * (itn % NJ), 0)
            acc, l, m8 = half(g, hh, gn, qn, s_w, s_r, m8, None if r == 0 else zero)
            if r == NR - 1:
                return m8, tuple(outs), acc, l
            outs.append(normalise(acc, l))
            if hh == 3:
                ot = jnp.concatenate(outs, axis=0)
                outs = []
                obuf[g, pl.ds(pl.multiple_of(j * 128, 128), 128), :] = ot.T.astype(bf16)

    z32 = jnp.zeros((DHA, 128), f32)
    _, last_outs, last_acc, last_l = lax.fori_loop(
        0, NIT, a2_body, (m8_first, (z32, z32, z32), z32, jnp.ones((8, 128), f32)))
    store_tile(jnp.int32(NIT - 1), list(last_outs) + [normalise(last_acc, last_l)])

    cp_awo.wait()
    for cp in cp_raw:
        cp.wait()

    NOI = NXC // PROJ_U
    RBLK = (D // 16) // NOI

    def oproj(i, carry):
        units = [(wi, hp, jb) for jb in range(RBLK) for wi in range(3) for hp in range(HB // 2)]
        per_dot = -(-len(units) // (PROJ_U * 8))
        for cc in range(PROJ_U):
            r0 = pl.multiple_of((i * PROJ_U + cc) * RC, RC)
            o = jnp.concatenate([obuf[g, pl.ds(r0, RC), :] for g in range(8)], axis=1)
            for n in range(8):
                outa[pl.ds(r0, RC), n * 128:(n + 1) * 128] = _dot(o, awo[:, n * 128:(n + 1) * 128]).astype(bf16)
                mine, units = units[:per_dot], units[per_dot:]
                for q0 in range(0, len(mine), RP_G):
                    repack_group([(wi, hp, i * RBLK + jb) for wi, hp, jb in mine[q0:q0 + RP_G]])
        return carry

    lax.fori_loop(0, NOI, oproj, 0)
    cp_outa = pltpu.make_async_copy(outa, out_hbm.at[:, pl.ds(0, D)], sem_out.at[0])
    cp_outa.start()

    for cp in cp_wo:
        cp.wait()
    cp_xb.wait()
    cp_mem.wait()
    wo32 = wo.bitcast(u32)
    bscale = DHB ** -0.5
    L = MEM + SEG
    row = lax.broadcasted_iota(jnp.int32, (2 * L, 2 * L), 0)
    col = lax.broadcasted_iota(jnp.int32, (2 * L, 2 * L), 1)
    same = (row < L) == (col < L)
    r_in = jnp.where(row < L, row, row - L)
    c_in = jnp.where(col < L, col, col - L)
    keep = same & ((r_in < MEM) | (r_in >= c_in))
    fill = jnp.where(same, -1e9, -jnp.inf).astype(f32)
    LQ, LP = B_LQ, B_LP
    NP = HB // 2

    def qk_soft(q, k):
        s = _dot_t(q, k)
        s = jnp.where(keep, s * bscale, fill)
        m = jnp.max(s, axis=-1, keepdims=True)
        p = jnp.exp(s - m)
        l = jnp.sum(p, axis=-1, keepdims=True)
        return (p / l).astype(bf16)

    def step(hmat, blocks, finish_o):
        qs, ks, vs, ps, o_list = {}, {}, {}, {}, [None] * HB
        accs = [None] * 8

        def do_proj(pr):
            parts = {}
            todo = [(name, wi, cref, h) for h in (2 * pr, 2 * pr + 1)
                    for name, wi, cref in (("q", 3, cq), ("k", 4, ck), ("v", 5, cv))]
            if pr < B_SPLIT:
                acc = [None] * len(todo)
                for k0, k1 in B_KSPLIT:
                    for t, (_, wi, _, h) in enumerate(todo):
                        w = _bc(wbuf[wi, h * (D // 2) + k0 // 2:h * (D // 2) + k1 // 2, :])
                        r = _dot(hmat[:, k0:k1], w)
                        if acc[t] is not None:
                            r = r + acc[t]
                        acc[t] = r
                for (name, wi, cref, h), r in zip(todo, acc):
                    parts[name, h] = blocks(cref, h, r)
            else:
                for name, wi, cref, h in todo:
                    parts[name, h] = blocks(cref, h, _dot(hmat, _bc(wbuf[wi, h * (D // 2):(h + 1) * (D // 2), :])))
            for name, dst in (("q", qs), ("k", ks), ("v", vs)):
                dst[pr] = jnp.concatenate([parts[name, 2 * pr], parts[name, 2 * pr + 1]], axis=0).astype(bf16)

        def do_wo(g):
            og = jnp.concatenate(o_list[4 * g:4 * g + 4], axis=1)
            for n in range(8):
                r = _dot(og, _bc(wo32[n, g * 256:(g + 1) * 256, :]))
                accs[n] = r if accs[n] is None else accs[n] + r

        g_next = 0
        for i in range(NP + LP):
            if i < NP:
                do_proj(i)
            else:
                for _ in range(B_WG):
                    do_wo(g_next)
                    g_next += 1
            if 0 <= i - LQ < NP:
                ps[i - LQ] = qk_soft(qs.pop(i - LQ), ks.pop(i - LQ))
            if 0 <= i - LP < NP:
                pr = i - LP
                o = _dot(ps.pop(pr), vs.pop(pr))
                o_list[2 * pr] = finish_o(2 * pr, o[0:L])
                o_list[2 * pr + 1] = finish_o(2 * pr + 1, o[L:2 * L])
        while g_next < 8:
            do_wo(g_next)
            g_next += 1
        return jnp.concatenate(accs, axis=1)

    def dstep(d, mem):
        base = pl.multiple_of(d * 64, 64)
        ha = jnp.concatenate([mem, xb[pl.ds(base, 40), :].astype(f32)], axis=0).astype(bf16)

        def blk_a(cref, h, v):
            cref[h] = v[40:48]
            return v[0:40]

        def fin_a(h, o):
            co[h] = o[32:40]
            return o[0:32].astype(bf16)

        y = step(ha, blk_a, fin_a).astype(bf16)
        outb[pl.ds(base, 24), :] = y[8:32]
        mem1 = y[0:8].astype(f32)
        hb = jnp.concatenate([mem1, xb[pl.ds(base + 40, 24), :].astype(f32)], axis=0).astype(bf16)

        def asm_b(cref, h, v):
            return jnp.concatenate([v[0:8], cref[h], v[8:32]], axis=0)

        def fin_b(h, o):
            return jnp.concatenate([o[0:8], co[h], o[8:40]], axis=0).astype(bf16)

        y = step(hb, asm_b, fin_b).astype(bf16)
        outb[pl.ds(base + 24, 40), :] = y[8:48]
        rows = pl.ds(base, 64)
        pltpu.make_async_copy(outb.at[rows, :], out_hbm.at[rows, pl.ds(D, D)], sem_ob.at[d]).start()
        return y[0:8].astype(f32)

    def dstep_n(i, mem):
        for r in range(B_U):
            mem = dstep(i * B_U + r, mem)
        return mem

    lax.fori_loop(0, S // (2 * SEG) // B_U, dstep_n, mem0[...].astype(f32))

    cp_outa.wait()

    def wait_out(d, carry):
        rows = pl.ds(pl.multiple_of(d * 64, 64), 64)
        pltpu.make_async_copy(outb.at[rows, :], out_hbm.at[rows, pl.ds(D, D)], sem_ob.at[d]).wait()
        return carry

    lax.fori_loop(0, S // (2 * SEG), wait_out, 0)


@functools.partial(jax.jit, static_argnames=("B_seg_len",))
def pallas_concat_heads__softmax_full_mha__memory_aug_recurrent_mem_tr__prompt_kernel(
    A_x: jax.Array,
    A_wqkv: jax.Array,
    A_wo: jax.Array,
    B_x: jax.Array,
    B_mem0: jax.Array,
    B_Wq: jax.Array,
    B_Wk: jax.Array,
    B_Wv: jax.Array,
    B_Wo: jax.Array,
    B_seg_len: int,
):
    assert A_x.shape == (1, S, D) and B_x.shape == (1, S, D) and B_mem0.shape == (1, MEM, D)
    assert B_Wq.shape == (D, HB, DHB) and B_Wo.shape == (HB, DHB, D) and B_seg_len == SEG
    any_spec = pl.BlockSpec(memory_space=pl.ANY)
    scratch = [
        pltpu.VMEM((S, D), bf16),
        pltpu.VMEM((D, 3 * D), bf16),
        pltpu.VMEM((D, D), bf16),
        pltpu.VMEM((8, S, 128), bf16),
        pltpu.VMEM((8, 16, 128, 128), bf16),
        pltpu.VMEM((HA, 16, DHA, 128), bf16),
        pltpu.VMEM((S, 128), f32),
        pltpu.VMEM((S, 128), f32),
        pltpu.VMEM((8, S, 128), bf16),
        pltpu.VMEM((S, D), bf16),
        pltpu.VMEM((S, D), bf16),
        pltpu.VMEM((MEM, D), bf16),
        pltpu.VMEM((6, HB * D // 2, 128), u32),
        pltpu.VMEM((8, HB * DHB, 128), bf16),
        pltpu.VMEM((S, D), bf16),
        pltpu.VMEM((HB, 8, 128), f32),
        pltpu.VMEM((HB, 8, 128), f32),
        pltpu.VMEM((HB, 8, 128), f32),
        pltpu.VMEM((HB, 8, 128), f32),
        pltpu.SemaphoreType.DMA((4,)),
        pltpu.SemaphoreType.DMA((3,)),
        pltpu.SemaphoreType.DMA((8,)),
        pltpu.SemaphoreType.DMA((2,)),
        pltpu.SemaphoreType.DMA((48,)),
        pltpu.SemaphoreType.DMA((8,)),
        pltpu.SemaphoreType.DMA((1,)),
        pltpu.SemaphoreType.DMA((32,)),
    ]
    out = pl.pallas_call(
        _kernel,
        out_shape=jax.ShapeDtypeStruct((S, 2 * D), bf16),
        in_specs=[any_spec] * 9,
        out_specs=any_spec,
        scratch_shapes=scratch,
        compiler_params=pltpu.CompilerParams(vmem_limit_bytes=124 * 1024 * 1024),
        name="mha_rmt_fused",
    )(A_x.reshape(S, D), A_wqkv, A_wo, B_x.reshape(S, D), B_mem0.reshape(MEM, D),
      B_Wq, B_Wk, B_Wv, B_Wo.reshape(HB * DHB, D))
    return out.reshape(1, S, 2 * D)
```

```python
import functools

import jax
import jax.numpy as jnp
from jax import lax
import jax.experimental.pallas as pl
import jax.experimental.pallas.tpu as pltpu

bf16 = jnp.bfloat16
f32 = jnp.float32
u32 = jnp.uint32

S = 2048
D = 1024
HA = 32
DHA = 32
HB = 32
DHB = 128
MEM = 8
SEG = 32
LOG2E = 1.4426950408889634

KG0 = 3
QV_U = 4
PROJ_U = 4
RP_G = 6
A2_JU = 8
LAG = 9
B_U = 2
B_LQ = 2
B_LP = 6
B_KSPLIT = ((0, 128), (128, 256), (256, 384), (384, 512), (512, 1024))


def _dot(a, b):
    return jnp.dot(a, b, preferred_element_type=f32)


def _dot_t(a, b):
    return lax.dot_general(a, b, (((1,), (1,)), ((), ())), preferred_element_type=f32)


def _bc(x):
    return pltpu.bitcast(x, bf16)


def _kernel(ax_hbm, awqkv_hbm, awo_hbm, bx_hbm, bmem_hbm, bwq_hbm, bwk_hbm, bwv_hbm, bwo_hbm,
            out_hbm,
            xa, wqkv, awo, kbuf, qT, vT, sa, sb, obuf, outa,
            xb, mem0, wbuf, wo, outb, cq, ck, cv, co,
            sem_w, sem_a, sem_x, sem_b, sem_raw, sem_wo, sem_out, sem_ob):
    RC = 256
    NXC = S // RC

    def w_copy(col0, ncol, sem):
        return pltpu.make_async_copy(awqkv_hbm.at[:, pl.ds(col0, ncol)], wqkv.at[:, pl.ds(col0, ncol)], sem)

    cp_wk0 = w_copy(D, KG0 * 128, sem_w.at[0])
    cp_wk1 = w_copy(D + KG0 * 128, (8 - KG0) * 128, sem_w.at[1])
    cp_wq = w_copy(0, D, sem_w.at[2])
    cp_wv = w_copy(2 * D, D, sem_w.at[3])
    cp_x = [pltpu.make_async_copy(ax_hbm.at[pl.ds(c * RC, RC), :], xa.at[pl.ds(c * RC, RC), :], sem_x.at[c])
            for c in range(NXC)]
    cp_wk0.start(priority=0)
    cp_x[0].start(priority=0)
    cp_x[1].start(priority=0)
    cp_wk1.start(priority=1)

    qscale = (DHA ** -0.5) * LOG2E

    def kproj_chunks(r0s, groups):
        for r0 in r0s:
            x = xa[pl.ds(r0, RC), :]
            for g in groups:
                w = wqkv[:, D + g * 128:D + (g + 1) * 128]
                kbuf[g, pl.ds(r0, RC), :] = _dot(x, w).astype(bf16)

    cp_wk0.wait()
    cp_x[0].wait()
    cp_x[1].wait()
    kproj_chunks((0, RC), range(0, KG0))
    cp_wk1.wait()
    for c in range(2, NXC):
        cp_x[c].start(priority=0)
    cp_wq.start(priority=1)
    cp_wv.start(priority=1)
    kproj_chunks((0, RC), range(KG0, 8))

    def kproj(i, carry):
        r0s = [pl.multiple_of((2 * i + cc) * RC, RC) for cc in range(2)]
        for cc in range(2):
            pltpu.make_async_copy(ax_hbm.at[pl.ds(r0s[cc], RC), :], xa.at[pl.ds(r0s[cc], RC), :],
                                  sem_x.at[2 * i + cc]).wait()
        kproj_chunks(r0s, range(8))
        return carry

    lax.fori_loop(1, NXC // 2, kproj, 0)
    cp_wq.wait()
    cp_wv.wait()

    def qvproj(i, carry):
        for cc in range(QV_U):
            c = i * QV_U + cc
            r0 = pl.multiple_of(c * RC, RC)
            x = xa[pl.ds(r0, RC), :]
            for g in range(8):
                q = _dot(x, wqkv[:, g * 128:(g + 1) * 128]) * qscale
                v = _dot(x, wqkv[:, 2 * D + g * 128:2 * D + (g + 1) * 128])
                for jj in range(RC // 128):
                    j = c * (RC // 128) + jj
                    qT[g, j] = q[jj * 128:(jj + 1) * 128].T.astype(bf16)
                    vt = v[jj * 128:(jj + 1) * 128].T.astype(bf16)
                    for hh in range(4):
                        vT[g * 4 + hh, j] = vt[hh * DHA:(hh + 1) * DHA]
        return carry

    lax.fori_loop(0, NXC // QV_U, qvproj, 0)

    k32 = kbuf.bitcast(u32)
    q32 = qT.bitcast(u32)
    v32 = vT.bitcast(u32)
    NK = S // 128

    def q_tile(g, j, hh):
        q = _bc(q32[g, j, hh * 16:(hh + 1) * 16, :])
        parts = []
        if hh > 0:
            parts.append(jnp.zeros((hh * DHA, 128), bf16))
        parts.append(q)
        if hh < 3:
            parts.append(jnp.zeros(((3 - hh) * DHA, 128), bf16))
        return jnp.concatenate(parts, axis=0) if len(parts) > 1 else q

    def qk_tile(g, qm, c, s_w):
        k = _bc(k32[g, c * 64:(c + 1) * 64, :])
        s = _dot(k, qm)
        s_w[c * 128:(c + 1) * 128, :] = s
        return jnp.max(s.reshape(16, 8, 128), axis=0)

    def half(g, hh, gn, qn, s_w, s_r, m8_cur, zero):
        h = g * 4 + hh
        m = jnp.max(m8_cur, axis=0, keepdims=True)
        st = {"m8": None, "l": None, "acc": None}

        def do_qk(c):
            mt = qk_tile(gn, qn, c, s_w)
            st["m8"] = mt if st["m8"] is None else jnp.maximum(st["m8"], mt)

        def do_pv(t):
            if zero is None:
                s = s_r[t * 128:(t + 1) * 128, :]
            else:
                s = s_r[pl.ds(pl.multiple_of(zero + t * 128, 128), 128), :]
            p = jnp.exp2(s - m)
            lt = jnp.sum(p.reshape(16, 8, 128), axis=0)
            st["l"] = lt if st["l"] is None else st["l"] + lt
            pv = _dot(_bc(v32[h, t]), p.astype(bf16))
            st["acc"] = pv if st["acc"] is None else st["acc"] + pv

        for c in range(NK + LAG):
            if c < NK:
                do_qk(c)
            if c >= LAG:
                do_pv(c - LAG)
        m8, l, acc = st["m8"], st["l"], st["acc"]
        return acc, l, m8

    q0 = q_tile(0, 0, 0)
    m8 = None
    for c in range(NK):
        mt = qk_tile(0, q0, c, sa)
        m8 = mt if m8 is None else jnp.maximum(m8, mt)
    m8_first = m8

    cp_awo = pltpu.make_async_copy(awo_hbm, awo, sem_a.at[0])
    cp_raw = []
    for i, w_hbm in enumerate((bwq_hbm, bwk_hbm, bwv_hbm)):
        w32 = w_hbm.bitcast(u32)
        for hp in range(HB // 2):
            cp_raw.append(pltpu.make_async_copy(w32.at[:, hp, :], wbuf.at[i, pl.ds(hp * D, D), :],
                                                sem_raw.at[i * 16 + hp]))
    cp_wo = [pltpu.make_async_copy(bwo_hbm.at[:, pl.ds(n * 128, 128)], wo.at[n], sem_wo.at[n])
             for n in range(D // 128)]
    cp_xb = pltpu.make_async_copy(bx_hbm, xb, sem_b.at[0])
    cp_mem = pltpu.make_async_copy(bmem_hbm, mem0, sem_b.at[1])

    def repack_group(units):
        vals = []
        for wi, hp, blk in units:
            base = pl.multiple_of(hp * D + blk * 16, 16)
            vals.append((wbuf[wi, pl.ds(base, 8, stride=2), :], wbuf[wi, pl.ds(base + 1, 8, stride=2), :]))
        for (wi, hp, blk), (ve, vo) in zip(units, vals):
            r = pl.multiple_of(2 * hp * (D // 2) + blk * 8, 8)
            wbuf[3 + wi, pl.ds(r, 8), :] = (ve & jnp.uint32(0xFFFF)) | (vo << 16)
            wbuf[3 + wi, pl.ds(r + D // 2, 8), :] = (ve >> 16) | (vo & jnp.uint32(0xFFFF0000))

    JU = A2_JU
    NJ = 16 // JU
    NIT = 8 * NJ
    NR = 4 * JU

    def normalise(acc, l):
        return acc * (1.0 / jnp.sum(l, axis=0, keepdims=True))

    def store_tile(it, outs):
        ot = jnp.concatenate(outs, axis=0)
        g = it // NJ
        j = JU * (it % NJ) + (JU - 1)
        obuf[g, pl.ds(pl.multiple_of(j * 128, 128), 128), :] = ot.T.astype(bf16)

    def a2_body(it, carry):
        m8, prev_outs, prev_acc, prev_l = carry
        g = it // NJ
        jj = it % NJ

        @pl.when(it == 1)
        def _():
            cp_awo.start()
            for cp in cp_raw:
                cp.start()

        @pl.when(it == 4)
        def _():
            for cp in cp_wo:
                cp.start()
            cp_xb.start()
            cp_mem.start()

        store_tile(jnp.maximum(it - 1, 0), list(prev_outs) + [normalise(prev_acc, prev_l)])

        zero = (it * (it + 1)) & 1
        outs = []
        for r in range(NR):
            j = JU * jj + r // 4
            hh = r % 4
            s_r, s_w = (sa, sb) if r % 2 == 0 else (sb, sa)
            if r < NR - 1:
                gn = g
                qn = q_tile(g, JU * jj + (r + 1) // 4, (r + 1) % 4)
            else:
                itn = jnp.minimum(it + 1, NIT - 1)
                gn = itn // NJ
                qn = q_tile(gn, JU * (itn % NJ), 0)
            acc, l, m8 = half(g, hh, gn, qn, s_w, s_r, m8, None if r == 0 else zero)
            if r == NR - 1:
                return m8, tuple(outs), acc, l
            outs.append(normalise(acc, l))
            if hh == 3:
                ot = jnp.concatenate(outs, axis=0)
                outs = []
                obuf[g, pl.ds(pl.multiple_of(j * 128, 128), 128), :] = ot.T.astype(bf16)

    z32 = jnp.zeros((DHA, 128), f32)
    _, last_outs, last_acc, last_l = lax.fori_loop(
        0, NIT, a2_body, (m8_first, (z32, z32, z32), z32, jnp.ones((8, 128), f32)))
    store_tile(jnp.int32(NIT - 1), list(last_outs) + [normalise(last_acc, last_l)])

    cp_awo.wait()
    for cp in cp_raw:
        cp.wait()

    NOI = NXC // PROJ_U
    RBLK = (D // 16) // NOI

    def oproj(i, carry):
        units = [(wi, hp, jb) for jb in range(RBLK) for wi in range(3) for hp in range(HB // 2)]
        per_dot = -(-len(units) // (PROJ_U * 8))
        for cc in range(PROJ_U):
            r0 = pl.multiple_of((i * PROJ_U + cc) * RC, RC)
            o = jnp.concatenate([obuf[g, pl.ds(r0, RC), :] for g in range(8)], axis=1)
            for n in range(8):
                outa[pl.ds(r0, RC), n * 128:(n + 1) * 128] = _dot(o, awo[:, n * 128:(n + 1) * 128]).astype(bf16)
                mine, units = units[:per_dot], units[per_dot:]
                for q0 in range(0, len(mine), RP_G):
                    repack_group([(wi, hp, i * RBLK + jb) for wi, hp, jb in mine[q0:q0 + RP_G]])
        return carry

    lax.fori_loop(0, NOI, oproj, 0)
    cp_outa = pltpu.make_async_copy(outa, out_hbm.at[:, pl.ds(0, D)], sem_out.at[0])
    cp_outa.start()

    for cp in cp_wo:
        cp.wait()
    cp_xb.wait()
    cp_mem.wait()
    wo32 = wo.bitcast(u32)
    bscale = DHB ** -0.5
    L = MEM + SEG
    row = lax.broadcasted_iota(jnp.int32, (2 * L, 2 * L), 0)
    col = lax.broadcasted_iota(jnp.int32, (2 * L, 2 * L), 1)
    same = (row < L) == (col < L)
    r_in = jnp.where(row < L, row, row - L)
    c_in = jnp.where(col < L, col, col - L)
    keep = same & ((r_in < MEM) | (r_in >= c_in))
    fill = jnp.where(same, -1e9, -jnp.inf).astype(f32)
    LQ, LP = B_LQ, B_LP
    NP = HB // 2

    def qk_soft(q, k):
        s = _dot_t(q, k)
        s = jnp.where(keep, s * bscale, fill)
        m = jnp.max(s, axis=-1, keepdims=True)
        p = jnp.exp(s - m)
        l = jnp.sum(p, axis=-1, keepdims=True)
        return (p / l).astype(bf16)

    def step(hmat, blocks, finish_o):
        qs, ks, vs, ps, o_list = {}, {}, {}, {}, [None] * HB
        accs = [None] * 8

        def do_proj(pr):
            parts = {}
            todo = [(name, wi, cref, h) for h in (2 * pr, 2 * pr + 1)
                    for name, wi, cref in (("q", 3, cq), ("k", 4, ck), ("v", 5, cv))]
            if pr == 0:
                acc = [None] * len(todo)
                for k0, k1 in B_KSPLIT:
                    for t, (_, wi, _, h) in enumerate(todo):
                        w = _bc(wbuf[wi, h * (D // 2) + k0 // 2:h * (D // 2) + k1 // 2, :])
                        r = _dot(hmat[:, k0:k1], w)
                        if acc[t] is not None:
                            r = r + acc[t]
                        acc[t] = r
                for (name, wi, cref, h), r in zip(todo, acc):
                    parts[name, h] = blocks(cref, h, r)
            else:
                for name, wi, cref, h in todo:
                    parts[name, h] = blocks(cref, h, _dot(hmat, _bc(wbuf[wi, h * (D // 2):(h + 1) * (D // 2), :])))
            for name, dst in (("q", qs), ("k", ks), ("v", vs)):
                dst[pr] = jnp.concatenate([parts[name, 2 * pr], parts[name, 2 * pr + 1]], axis=0).astype(bf16)

        def do_wo(g):
            og = jnp.concatenate(o_list[4 * g:4 * g + 4], axis=1)
            for n in range(8):
                r = _dot(og, _bc(wo32[n, g * 256:(g + 1) * 256, :]))
                accs[n] = r if accs[n] is None else accs[n] + r

        g_next = 0
        for i in range(NP + LP):
            if i < NP:
                do_proj(i)
            else:
                do_wo(g_next)
                g_next += 1
            if 0 <= i - LQ < NP:
                ps[i - LQ] = qk_soft(qs.pop(i - LQ), ks.pop(i - LQ))
            if 0 <= i - LP < NP:
                pr = i - LP
                o = _dot(ps.pop(pr), vs.pop(pr))
                o_list[2 * pr] = finish_o(2 * pr, o[0:L])
                o_list[2 * pr + 1] = finish_o(2 * pr + 1, o[L:2 * L])
        while g_next < 8:
            do_wo(g_next)
            g_next += 1
        return jnp.concatenate(accs, axis=1)

    def dstep(d, mem):
        base = pl.multiple_of(d * 64, 64)
        ha = jnp.concatenate([mem, xb[pl.ds(base, 40), :].astype(f32)], axis=0).astype(bf16)

        def blk_a(cref, h, v):
            cref[h] = v[40:48]
            return v[0:40]

        def fin_a(h, o):
            co[h] = o[32:40]
            return o[0:32].astype(bf16)

        y = step(ha, blk_a, fin_a).astype(bf16)
        outb[pl.ds(base, 24), :] = y[8:32]
        mem1 = y[0:8].astype(f32)
        hb = jnp.concatenate([mem1, xb[pl.ds(base + 40, 24), :].astype(f32)], axis=0).astype(bf16)

        def asm_b(cref, h, v):
            return jnp.concatenate([v[0:8], cref[h], v[8:32]], axis=0)

        def fin_b(h, o):
            return jnp.concatenate([o[0:8], co[h], o[8:40]], axis=0).astype(bf16)

        y = step(hb, asm_b, fin_b).astype(bf16)
        outb[pl.ds(base + 24, 40), :] = y[8:48]
        rows = pl.ds(base, 64)
        pltpu.make_async_copy(outb.at[rows, :], out_hbm.at[rows, pl.ds(D, D)], sem_ob.at[d]).start()
        return y[0:8].astype(f32)

    def dstep_n(i, mem):
        for r in range(B_U):
            mem = dstep(i * B_U + r, mem)
        return mem

    lax.fori_loop(0, S // (2 * SEG) // B_U, dstep_n, mem0[...].astype(f32))

    cp_outa.wait()

    def wait_out(d, carry):
        rows = pl.ds(pl.multiple_of(d * 64, 64), 64)
        pltpu.make_async_copy(outb.at[rows, :], out_hbm.at[rows, pl.ds(D, D)], sem_ob.at[d]).wait()
        return carry

    lax.fori_loop(0, S // (2 * SEG), wait_out, 0)


@functools.partial(jax.jit, static_argnames=("B_seg_len",))
def pallas_concat_heads__softmax_full_mha__memory_aug_recurrent_mem_tr__prompt_kernel(
    A_x: jax.Array,
    A_wqkv: jax.Array,
    A_wo: jax.Array,
    B_x: jax.Array,
    B_mem0: jax.Array,
    B_Wq: jax.Array,
    B_Wk: jax.Array,
    B_Wv: jax.Array,
    B_Wo: jax.Array,
    B_seg_len: int,
):
    assert A_x.shape == (1, S, D) and B_x.shape == (1, S, D) and B_mem0.shape == (1, MEM, D)
    assert B_Wq.shape == (D, HB, DHB) and B_Wo.shape == (HB, DHB, D) and B_seg_len == SEG
    any_spec = pl.BlockSpec(memory_space=pl.ANY)
    scratch = [
        pltpu.VMEM((S, D), bf16),
        pltpu.VMEM((D, 3 * D), bf16),
        pltpu.VMEM((D, D), bf16),
        pltpu.VMEM((8, S, 128), bf16),
        pltpu.VMEM((8, 16, 128, 128), bf16),
        pltpu.VMEM((HA, 16, DHA, 128), bf16),
        pltpu.VMEM((S, 128), f32),
        pltpu.VMEM((S, 128), f32),
        pltpu.VMEM((8, S, 128), bf16),
        pltpu.VMEM((S, D), bf16),
        pltpu.VMEM((S, D), bf16),
        pltpu.VMEM((MEM, D), bf16),
        pltpu.VMEM((6, HB * D // 2, 128), u32),
        pltpu.VMEM((8, HB * DHB, 128), bf16),
        pltpu.VMEM((S, D), bf16),
        pltpu.VMEM((HB, 8, 128), f32),
        pltpu.VMEM((HB, 8, 128), f32),
        pltpu.VMEM((HB, 8, 128), f32),
        pltpu.VMEM((HB, 8, 128), f32),
        pltpu.SemaphoreType.DMA((4,)),
        pltpu.SemaphoreType.DMA((1,)),
        pltpu.SemaphoreType.DMA((8,)),
        pltpu.SemaphoreType.DMA((2,)),
        pltpu.SemaphoreType.DMA((48,)),
        pltpu.SemaphoreType.DMA((8,)),
        pltpu.SemaphoreType.DMA((1,)),
        pltpu.SemaphoreType.DMA((32,)),
    ]
    out = pl.pallas_call(
        _kernel,
        out_shape=jax.ShapeDtypeStruct((S, 2 * D), bf16),
        in_specs=[any_spec] * 9,
        out_specs=any_spec,
        scratch_shapes=scratch,
        compiler_params=pltpu.CompilerParams(vmem_limit_bytes=124 * 1024 * 1024),
        name="mha_rmt_fused",
    )(A_x.reshape(S, D), A_wqkv, A_wo, B_x.reshape(S, D), B_mem0.reshape(MEM, D),
      B_Wq, B_Wk, B_Wv, B_Wo.reshape(HB * DHB, D))
    return out.reshape(1, S, 2 * D)
```

```python
import functools

import jax
import jax.numpy as jnp
from jax import lax
import jax.experimental.pallas as pl
import jax.experimental.pallas.tpu as pltpu

bf16 = jnp.bfloat16
f32 = jnp.float32
u32 = jnp.uint32

S = 2048
D = 1024
HA = 32
DHA = 32
HB = 32
DHB = 128
MEM = 8
SEG = 32
LOG2E = 1.4426950408889634

KG0 = 3
QV_U = 4
PROJ_U = 4
RP_G = 6
A2_JU = 8
LAG = 9
B_U = 2
B_LQ = 2
B_LP = 6
B_KSPLIT = ((0, 128), (128, 256), (256, 384), (384, 512), (512, 1024))


def _dot(a, b):
    return jnp.dot(a, b, preferred_element_type=f32)


def _dot_t(a, b):
    return lax.dot_general(a, b, (((1,), (1,)), ((), ())), preferred_element_type=f32)


def _bc(x):
    return pltpu.bitcast(x, bf16)


def _kernel(ax_hbm, awqkv_hbm, awo_hbm, bx_hbm, bmem_hbm, bwq_hbm, bwk_hbm, bwv_hbm, bwo_hbm,
            out_hbm,
            xa, wqkv, awo, kbuf, qT, vT, sa, sb, obuf, outa,
            xb, mem0, wbuf, wo, outb, cq, ck, cv, co,
            sem_w, sem_a, sem_x, sem_b, sem_raw, sem_wo, sem_out, sem_ob):
    RC = 256
    NXC = S // RC

    def w_copy(col0, ncol, sem):
        return pltpu.make_async_copy(awqkv_hbm.at[:, pl.ds(col0, ncol)], wqkv.at[:, pl.ds(col0, ncol)], sem)

    cp_wk0 = w_copy(D, KG0 * 128, sem_w.at[0])
    cp_wk1 = w_copy(D + KG0 * 128, (8 - KG0) * 128, sem_w.at[1])
    cp_wq = w_copy(0, D, sem_w.at[2])
    cp_wv = w_copy(2 * D, D, sem_w.at[3])
    cp_x = [pltpu.make_async_copy(ax_hbm.at[pl.ds(c * RC, RC), :], xa.at[pl.ds(c * RC, RC), :], sem_x.at[c])
            for c in range(NXC)]
    cp_wk0.start(priority=0)
    cp_x[0].start(priority=0)
    cp_x[1].start(priority=0)
    cp_wk1.start(priority=1)

    qscale = (DHA ** -0.5) * LOG2E

    def kproj_chunks(r0s, groups):
        for r0 in r0s:
            x = xa[pl.ds(r0, RC), :]
            for g in groups:
                w = wqkv[:, D + g * 128:D + (g + 1) * 128]
                kbuf[g, pl.ds(r0, RC), :] = _dot(x, w).astype(bf16)

    cp_wk0.wait()
    cp_x[0].wait()
    cp_x[1].wait()
    kproj_chunks((0, RC), range(0, KG0))
    cp_wk1.wait()
    for c in range(2, NXC):
        cp_x[c].start(priority=0)
    cp_wq.start(priority=1)
    cp_wv.start(priority=1)
    kproj_chunks((0, RC), range(KG0, 8))

    def kproj(i, carry):
        r0s = [pl.multiple_of((2 * i + cc) * RC, RC) for cc in range(2)]
        for cc in range(2):
            pltpu.make_async_copy(ax_hbm.at[pl.ds(r0s[cc], RC), :], xa.at[pl.ds(r0s[cc], RC), :],
                                  sem_x.at[2 * i + cc]).wait()
        kproj_chunks(r0s, range(8))
        return carry

    lax.fori_loop(1, NXC // 2, kproj, 0)
    cp_wq.wait()
    cp_wv.wait()

    def qvproj(i, carry):
        for cc in range(QV_U):
            c = i * QV_U + cc
            r0 = pl.multiple_of(c * RC, RC)
            x = xa[pl.ds(r0, RC), :]
            for g in range(8):
                q = _dot(x, wqkv[:, g * 128:(g + 1) * 128]) * qscale
                v = _dot(x, wqkv[:, 2 * D + g * 128:2 * D + (g + 1) * 128])
                for jj in range(RC // 128):
                    j = c * (RC // 128) + jj
                    qT[g, j] = q[jj * 128:(jj + 1) * 128].T.astype(bf16)
                    vt = v[jj * 128:(jj + 1) * 128].T.astype(bf16)
                    for hh in range(4):
                        vT[g * 4 + hh, j] = vt[hh * DHA:(hh + 1) * DHA]
        return carry

    lax.fori_loop(0, NXC // QV_U, qvproj, 0)

    k32 = kbuf.bitcast(u32)
    q32 = qT.bitcast(u32)
    v32 = vT.bitcast(u32)
    NK = S // 128

    def q_tile(g, j, hh):
        q = _bc(q32[g, j, hh * 16:(hh + 1) * 16, :])
        parts = []
        if hh > 0:
            parts.append(jnp.zeros((hh * DHA, 128), bf16))
        parts.append(q)
        if hh < 3:
            parts.append(jnp.zeros(((3 - hh) * DHA, 128), bf16))
        return jnp.concatenate(parts, axis=0) if len(parts) > 1 else q

    def qk_tile(g, qm, c, s_w):
        k = _bc(k32[g, c * 64:(c + 1) * 64, :])
        s = _dot(k, qm)
        s_w[c * 128:(c + 1) * 128, :] = s
        return jnp.max(s.reshape(16, 8, 128), axis=0)

    def half(g, hh, gn, qn, s_w, s_r, m8_cur, zero):
        h = g * 4 + hh
        m = jnp.max(m8_cur, axis=0, keepdims=True)
        st = {"m8": None, "l": None, "acc": None}

        def do_qk(c):
            mt = qk_tile(gn, qn, c, s_w)
            st["m8"] = mt if st["m8"] is None else jnp.maximum(st["m8"], mt)

        def do_pv(t):
            if zero is None:
                s = s_r[t * 128:(t + 1) * 128, :]
            else:
                s = s_r[pl.ds(pl.multiple_of(zero + t * 128, 128), 128), :]
            p = jnp.exp2(s - m)
            lt = jnp.sum(p.reshape(16, 8, 128), axis=0)
            st["l"] = lt if st["l"] is None else st["l"] + lt
            pv = _dot(_bc(v32[h, t]), p.astype(bf16))
            st["acc"] = pv if st["acc"] is None else st["acc"] + pv

        for c0 in range(0, NK + LAG, 2):
            for c in (c0, c0 + 1):
                if c < NK:
                    do_qk(c)
            for c in (c0, c0 + 1):
                if LAG <= c < NK + LAG:
                    do_pv(c - LAG)
        m8, l, acc = st["m8"], st["l"], st["acc"]
        return acc, l, m8

    q0 = q_tile(0, 0, 0)
    m8 = None
    for c in range(NK):
        mt = qk_tile(0, q0, c, sa)
        m8 = mt if m8 is None else jnp.maximum(m8, mt)
    m8_first = m8

    cp_awo = pltpu.make_async_copy(awo_hbm, awo, sem_a.at[0])
    cp_raw = []
    for i, w_hbm in enumerate((bwq_hbm, bwk_hbm, bwv_hbm)):
        w32 = w_hbm.bitcast(u32)
        for hp in range(HB // 2):
            cp_raw.append(pltpu.make_async_copy(w32.at[:, hp, :], wbuf.at[i, pl.ds(hp * D, D), :],
                                                sem_raw.at[i * 16 + hp]))
    cp_wo = [pltpu.make_async_copy(bwo_hbm.at[:, pl.ds(n * 128, 128)], wo.at[n], sem_wo.at[n])
             for n in range(D // 128)]
    cp_xb = pltpu.make_async_copy(bx_hbm, xb, sem_b.at[0])
    cp_mem = pltpu.make_async_copy(bmem_hbm, mem0, sem_b.at[1])

    def repack_group(units):
        vals = []
        for wi, hp, blk in units:
            base = pl.multiple_of(hp * D + blk * 16, 16)
            vals.append((wbuf[wi, pl.ds(base, 8, stride=2), :], wbuf[wi, pl.ds(base + 1, 8, stride=2), :]))
        for (wi, hp, blk), (ve, vo) in zip(units, vals):
            r = pl.multiple_of(2 * hp * (D // 2) + blk * 8, 8)
            wbuf[3 + wi, pl.ds(r, 8), :] = (ve & jnp.uint32(0xFFFF)) | (vo << 16)
            wbuf[3 + wi, pl.ds(r + D // 2, 8), :] = (ve >> 16) | (vo & jnp.uint32(0xFFFF0000))

    JU = A2_JU
    NJ = 16 // JU
    NIT = 8 * NJ
    NR = 4 * JU

    def normalise(acc, l):
        return acc * (1.0 / jnp.sum(l, axis=0, keepdims=True))

    def store_tile(it, outs):
        ot = jnp.concatenate(outs, axis=0)
        g = it // NJ
        j = JU * (it % NJ) + (JU - 1)
        obuf[g, pl.ds(pl.multiple_of(j * 128, 128), 128), :] = ot.T.astype(bf16)

    def a2_body(it, carry):
        m8, prev_outs, prev_acc, prev_l = carry
        g = it // NJ
        jj = it % NJ

        @pl.when(it == 1)
        def _():
            cp_awo.start()
            for cp in cp_raw:
                cp.start()

        @pl.when(it == 4)
        def _():
            for cp in cp_wo:
                cp.start()
            cp_xb.start()
            cp_mem.start()

        store_tile(jnp.maximum(it - 1, 0), list(prev_outs) + [normalise(prev_acc, prev_l)])

        zero = (it * (it + 1)) & 1
        outs = []
        for r in range(NR):
            j = JU * jj + r // 4
            hh = r % 4
            s_r, s_w = (sa, sb) if r % 2 == 0 else (sb, sa)
            if r < NR - 1:
                gn = g
                qn = q_tile(g, JU * jj + (r + 1) // 4, (r + 1) % 4)
            else:
                itn = jnp.minimum(it + 1, NIT - 1)
                gn = itn // NJ
                qn = q_tile(gn, JU * (itn % NJ), 0)
            acc, l, m8 = half(g, hh, gn, qn, s_w, s_r, m8, None if r == 0 else zero)
            if r == NR - 1:
                return m8, tuple(outs), acc, l
            outs.append(normalise(acc, l))
            if hh == 3:
                ot = jnp.concatenate(outs, axis=0)
                outs = []
                obuf[g, pl.ds(pl.multiple_of(j * 128, 128), 128), :] = ot.T.astype(bf16)

    z32 = jnp.zeros((DHA, 128), f32)
    _, last_outs, last_acc, last_l = lax.fori_loop(
        0, NIT, a2_body, (m8_first, (z32, z32, z32), z32, jnp.ones((8, 128), f32)))
    store_tile(jnp.int32(NIT - 1), list(last_outs) + [normalise(last_acc, last_l)])

    cp_awo.wait()
    for cp in cp_raw:
        cp.wait()

    NOI = NXC // PROJ_U
    RBLK = (D // 16) // NOI

    def oproj(i, carry):
        units = [(wi, hp, jb) for jb in range(RBLK) for wi in range(3) for hp in range(HB // 2)]
        per_dot = -(-len(units) // (PROJ_U * 8))
        for cc in range(PROJ_U):
            r0 = pl.multiple_of((i * PROJ_U + cc) * RC, RC)
            o = jnp.concatenate([obuf[g, pl.ds(r0, RC), :] for g in range(8)], axis=1)
            for n in range(8):
                outa[pl.ds(r0, RC), n * 128:(n + 1) * 128] = _dot(o, awo[:, n * 128:(n + 1) * 128]).astype(bf16)
                mine, units = units[:per_dot], units[per_dot:]
                for q0 in range(0, len(mine), RP_G):
                    repack_group([(wi, hp, i * RBLK + jb) for wi, hp, jb in mine[q0:q0 + RP_G]])
        return carry

    lax.fori_loop(0, NOI, oproj, 0)
    cp_outa = pltpu.make_async_copy(outa, out_hbm.at[:, pl.ds(0, D)], sem_out.at[0])
    cp_outa.start()

    for cp in cp_wo:
        cp.wait()
    cp_xb.wait()
    cp_mem.wait()
    wo32 = wo.bitcast(u32)
    bscale = DHB ** -0.5
    L = MEM + SEG
    row = lax.broadcasted_iota(jnp.int32, (2 * L, 2 * L), 0)
    col = lax.broadcasted_iota(jnp.int32, (2 * L, 2 * L), 1)
    same = (row < L) == (col < L)
    r_in = jnp.where(row < L, row, row - L)
    c_in = jnp.where(col < L, col, col - L)
    keep = same & ((r_in < MEM) | (r_in >= c_in))
    fill = jnp.where(same, -1e9, -jnp.inf).astype(f32)
    LQ, LP = B_LQ, B_LP
    NP = HB // 2

    def qk_soft(q, k):
        s = _dot_t(q, k)
        s = jnp.where(keep, s * bscale, fill)
        m = jnp.max(s, axis=-1, keepdims=True)
        p = jnp.exp(s - m)
        l = jnp.sum(p, axis=-1, keepdims=True)
        return (p / l).astype(bf16)

    def step(hmat, blocks, finish_o):
        qs, ks, vs, ps, o_list = {}, {}, {}, {}, [None] * HB
        accs = [None] * 8

        def do_proj(pr):
            parts = {}
            todo = [(name, wi, cref, h) for h in (2 * pr, 2 * pr + 1)
                    for name, wi, cref in (("q", 3, cq), ("k", 4, ck), ("v", 5, cv))]
            if pr == 0:
                acc = [None] * len(todo)
                for k0, k1 in B_KSPLIT:
                    for t, (_, wi, _, h) in enumerate(todo):
                        w = _bc(wbuf[wi, h * (D // 2) + k0 // 2:h * (D // 2) + k1 // 2, :])
                        r = _dot(hmat[:, k0:k1], w)
                        if acc[t] is not None:
                            r = r + acc[t]
                        acc[t] = r
                for (name, wi, cref, h), r in zip(todo, acc):
                    parts[name, h] = blocks(cref, h, r)
            else:
                for name, wi, cref, h in todo:
                    parts[name, h] = blocks(cref, h, _dot(hmat, _bc(wbuf[wi, h * (D // 2):(h + 1) * (D // 2), :])))
            for name, dst in (("q", qs), ("k", ks), ("v", vs)):
                dst[pr] = jnp.concatenate([parts[name, 2 * pr], parts[name, 2 * pr + 1]], axis=0).astype(bf16)

        def do_wo(g):
            og = jnp.concatenate(o_list[4 * g:4 * g + 4], axis=1)
            for n in range(8):
                r = _dot(og, _bc(wo32[n, g * 256:(g + 1) * 256, :]))
                accs[n] = r if accs[n] is None else accs[n] + r

        g_next = 0
        for i in range(NP + LP):
            if i < NP:
                do_proj(i)
            else:
                do_wo(g_next)
                g_next += 1
            if 0 <= i - LQ < NP:
                ps[i - LQ] = qk_soft(qs.pop(i - LQ), ks.pop(i - LQ))
            if 0 <= i - LP < NP:
                pr = i - LP
                o = _dot(ps.pop(pr), vs.pop(pr))
                o_list[2 * pr] = finish_o(2 * pr, o[0:L])
                o_list[2 * pr + 1] = finish_o(2 * pr + 1, o[L:2 * L])
        while g_next < 8:
            do_wo(g_next)
            g_next += 1
        return jnp.concatenate(accs, axis=1)

    def dstep(d, mem):
        base = pl.multiple_of(d * 64, 64)
        ha = jnp.concatenate([mem, xb[pl.ds(base, 40), :].astype(f32)], axis=0).astype(bf16)

        def blk_a(cref, h, v):
            cref[h] = v[40:48]
            return v[0:40]

        def fin_a(h, o):
            co[h] = o[32:40]
            return o[0:32].astype(bf16)

        y = step(ha, blk_a, fin_a).astype(bf16)
        outb[pl.ds(base, 24), :] = y[8:32]
        mem1 = y[0:8].astype(f32)
        hb = jnp.concatenate([mem1, xb[pl.ds(base + 40, 24), :].astype(f32)], axis=0).astype(bf16)

        def asm_b(cref, h, v):
            return jnp.concatenate([v[0:8], cref[h], v[8:32]], axis=0)

        def fin_b(h, o):
            return jnp.concatenate([o[0:8], co[h], o[8:40]], axis=0).astype(bf16)

        y = step(hb, asm_b, fin_b).astype(bf16)
        outb[pl.ds(base + 24, 40), :] = y[8:48]
        rows = pl.ds(base, 64)
        pltpu.make_async_copy(outb.at[rows, :], out_hbm.at[rows, pl.ds(D, D)], sem_ob.at[d]).start()
        return y[0:8].astype(f32)

    def dstep_n(i, mem):
        for r in range(B_U):
            mem = dstep(i * B_U + r, mem)
        return mem

    lax.fori_loop(0, S // (2 * SEG) // B_U, dstep_n, mem0[...].astype(f32))

    cp_outa.wait()

    def wait_out(d, carry):
        rows = pl.ds(pl.multiple_of(d * 64, 64), 64)
        pltpu.make_async_copy(outb.at[rows, :], out_hbm.at[rows, pl.ds(D, D)], sem_ob.at[d]).wait()
        return carry

    lax.fori_loop(0, S // (2 * SEG), wait_out, 0)


@functools.partial(jax.jit, static_argnames=("B_seg_len",))
def pallas_concat_heads__softmax_full_mha__memory_aug_recurrent_mem_tr__prompt_kernel(
    A_x: jax.Array,
    A_wqkv: jax.Array,
    A_wo: jax.Array,
    B_x: jax.Array,
    B_mem0: jax.Array,
    B_Wq: jax.Array,
    B_Wk: jax.Array,
    B_Wv: jax.Array,
    B_Wo: jax.Array,
    B_seg_len: int,
):
    assert A_x.shape == (1, S, D) and B_x.shape == (1, S, D) and B_mem0.shape == (1, MEM, D)
    assert B_Wq.shape == (D, HB, DHB) and B_Wo.shape == (HB, DHB, D) and B_seg_len == SEG
    any_spec = pl.BlockSpec(memory_space=pl.ANY)
    scratch = [
        pltpu.VMEM((S, D), bf16),
        pltpu.VMEM((D, 3 * D), bf16),
        pltpu.VMEM((D, D), bf16),
        pltpu.VMEM((8, S, 128), bf16),
        pltpu.VMEM((8, 16, 128, 128), bf16),
        pltpu.VMEM((HA, 16, DHA, 128), bf16),
        pltpu.VMEM((S, 128), f32),
        pltpu.VMEM((S, 128), f32),
        pltpu.VMEM((8, S, 128), bf16),
        pltpu.VMEM((S, D), bf16),
        pltpu.VMEM((S, D), bf16),
        pltpu.VMEM((MEM, D), bf16),
        pltpu.VMEM((6, HB * D // 2, 128), u32),
        pltpu.VMEM((8, HB * DHB, 128), bf16),
        pltpu.VMEM((S, D), bf16),
        pltpu.VMEM((HB, 8, 128), f32),
        pltpu.VMEM((HB, 8, 128), f32),
        pltpu.VMEM((HB, 8, 128), f32),
        pltpu.VMEM((HB, 8, 128), f32),
        pltpu.SemaphoreType.DMA((4,)),
        pltpu.SemaphoreType.DMA((1,)),
        pltpu.SemaphoreType.DMA((8,)),
        pltpu.SemaphoreType.DMA((2,)),
        pltpu.SemaphoreType.DMA((48,)),
        pltpu.SemaphoreType.DMA((8,)),
        pltpu.SemaphoreType.DMA((1,)),
        pltpu.SemaphoreType.DMA((32,)),
    ]
    out = pl.pallas_call(
        _kernel,
        out_shape=jax.ShapeDtypeStruct((S, 2 * D), bf16),
        in_specs=[any_spec] * 9,
        out_specs=any_spec,
        scratch_shapes=scratch,
        compiler_params=pltpu.CompilerParams(vmem_limit_bytes=124 * 1024 * 1024),
        name="mha_rmt_fused",
    )(A_x.reshape(S, D), A_wqkv, A_wo, B_x.reshape(S, D), B_mem0.reshape(MEM, D),
      B_Wq, B_Wk, B_Wv, B_Wo.reshape(HB * DHB, D))
    return out.reshape(1, S, 2 * D)
```
